```python
import jax
import jax.numpy as jnp

def _softmax(x, axis=-1):
    return jax.nn.softmax(x, axis=axis)
def _gelu(x):
    return jax.nn.gelu(x, approximate=True)
def _silu(x):
    return jax.nn.silu(x)
def _sigmoid(x):
    return jax.nn.sigmoid(x)
def _layernorm(x, axis=-1, eps=1e-5):
    m = jnp.mean(x, axis=axis, keepdims=True)
    v = jnp.var(x, axis=axis, keepdims=True)
    return (x - m) / jnp.sqrt(v + eps)
def _scatter_add(tgt, idx, src, axis=0):
    return tgt.at[idx].add(src)
def _segment_sum(src, seg, n):
    return jax.ops.segment_sum(src, seg, n)
class _Rng:
    def __init__(self, key):
        self._k = key
    def _next(self):
        self._k, sub = jax.random.split(self._k)
        return sub
    def normal(self, shape):
        return jax.random.normal(self._next(), shape, dtype=jnp.bfloat16)
    def randint(self, lo, hi, shape):
        return jax.random.randint(self._next(), shape, lo, hi, dtype=jnp.int32)
    def uniform(self, shape, lo=0.0, hi=1.0):
        return jax.random.uniform(self._next(), shape, jnp.bfloat16, lo, hi)
    def permutation(self, n):
        return jax.random.permutation(self._next(), n)


kernel_name = 'concat_heads__gqa_block_cached__mha_block_cached__near_ridge'

def setup_inputs():
    _rng = _Rng(jax.random.key(int.from_bytes(__import__("os").urandom(4), "little")))
    _w = (lambda a: (lambda t: t.astype(jnp.bfloat16) if jnp.issubdtype(t.dtype, jnp.floating) else t)(jnp.asarray(a)))
    def _A_setup():
        B, Sq, D = 16, 160, 640
        Hq, Hkv, Sk, Dh = 32, 32, 512, 192
        assert Hq % Hkv == 0, (Hq, Hkv)
        return {
            "x": _w((lambda *s: _rng.normal(s) * 0.05)(B, Sq, D)),
            "k_cache": _w((lambda *s: _rng.normal(s) * 0.05)(B, Hkv, Sk, Dh)),
            "v_cache": _w((lambda *s: _rng.normal(s) * 0.05)(B, Hkv, Sk, Dh)),
            "wq": _w((lambda *s: _rng.normal(s) * 0.05)(D, Hq * Dh) * (D ** -0.5)),
            "wo": _w((lambda *s: _rng.normal(s) * 0.05)(Hq * Dh, D) * ((Hq * Dh) ** -0.5)),
        }
    _A_in = _A_setup()

    def _B_setup():
        B, Sq, D = 16, 160, 640
        H, Sk, Dh = 32, 512, 192
        return {
            "x": _w((lambda *s: _rng.normal(s) * 0.05)(B, Sq, D)),
            "k_cache": _w((lambda *s: _rng.normal(s) * 0.05)(B, H, Sk, Dh)),
            "v_cache": _w((lambda *s: _rng.normal(s) * 0.05)(B, H, Sk, Dh)),
            "wq": _w((lambda *s: _rng.normal(s) * 0.05)(D, H * Dh) * (D ** -0.5)),
            "wo": _w((lambda *s: _rng.normal(s) * 0.05)(H * Dh, D) * ((H * Dh) ** -0.5)),
        }
    _B_in = _B_setup()

    return {
        "A_x": _A_in["x"],
        "A_k_cache": _A_in["k_cache"],
        "A_v_cache": _A_in["v_cache"],
        "A_wq": _A_in["wq"],
        "A_wo": _A_in["wo"],
        "B_x": _B_in["x"],
        "B_k_cache": _B_in["k_cache"],
        "B_v_cache": _B_in["v_cache"],
        "B_wq": _B_in["wq"],
        "B_wo": _B_in["wo"],
    }

def reference(A_x, A_k_cache, A_v_cache, A_wq, A_wo, B_x, B_k_cache, B_v_cache, B_wq, B_wo):
    def _A_ref(x, k_cache, v_cache, wq, wo):
        B, Sq, D = x.shape
        Hq, Dh = 32, 192
        Hkv = k_cache.shape[1]
        rep = Hq // Hkv
        q = (lambda x, *d: x.transpose(*d))((x @ wq).reshape(B, Sq, Hq, Dh), 0, 2, 1, 3)
        k = jnp.repeat(k_cache, rep, axis=1)
        v = jnp.repeat(v_cache, rep, axis=1)
        scores = jnp.einsum("bhqd,bhkd->bhqk", q, k) * (Dh ** -0.5)
        p = _softmax(scores, axis=-1)
        o = jnp.einsum("bhqk,bhkd->bhqd", p, v)
        return (lambda x, *d: x.transpose(*d))(o, 0, 2, 1, 3).reshape(B, Sq, Hq * Dh) @ wo

    def _B_ref(x, k_cache, v_cache, wq, wo):
        B, Sq, D = x.shape
        H, Dh = 32, 192
        q = (lambda x, *d: x.transpose(*d))((x @ wq).reshape(B, Sq, H, Dh), 0, 2, 1, 3)
        scores = jnp.einsum("bhqd,bhkd->bhqk", q, k_cache) * (Dh ** -0.5)
        p = _softmax(scores, axis=-1)
        o = jnp.einsum("bhqk,bhkd->bhqd", p, v_cache)
        return (lambda x, *d: x.transpose(*d))(o, 0, 2, 1, 3).reshape(B, Sq, H * Dh) @ wo

    a = _A_ref(A_x, A_k_cache, A_v_cache, A_wq, A_wo)
    b = _B_ref(B_x, B_k_cache, B_v_cache, B_wq, B_wo)
    return jnp.concatenate([a, b], axis=-1)
```

```python
import functools
import math

import jax
import jax.numpy as jnp
import jax.experimental.pallas as pl
import jax.experimental.pallas.tpu as pltpu

_NN = (((1,), (0,)), ((), ()))
_NT = (((1,), (1,)), ((), ()))


def _pair_attention(x, wq, kt0, kt1, vt0, vt1, wo, *, scale):
    f32, bf16 = jnp.float32, jnp.bfloat16
    dh, sk = kt0.shape
    pad = 256 - dh
    q = jax.lax.dot_general(x, wq, _NN, preferred_element_type=f32)
    q = (q * scale).astype(bf16)
    zeros = jnp.zeros((pad, sk), bf16)
    ones = jnp.ones((pad, sk), bf16)
    s0 = jax.lax.dot_general(q[:, :256], jnp.concatenate([kt0, zeros], axis=0),
                             _NN, preferred_element_type=f32)
    s1 = jax.lax.dot_general(q[:, 128:], jnp.concatenate([zeros, kt1], axis=0),
                             _NN, preferred_element_type=f32)
    p0 = jnp.exp2(s0 - jnp.max(s0, axis=-1, keepdims=True)).astype(bf16)
    p1 = jnp.exp2(s1 - jnp.max(s1, axis=-1, keepdims=True)).astype(bf16)
    o0 = jax.lax.dot_general(p0, jnp.concatenate([vt0, ones], axis=0),
                             _NT, preferred_element_type=f32)
    o1 = jax.lax.dot_general(p1, jnp.concatenate([ones, vt1], axis=0),
                             _NT, preferred_element_type=f32)
    mid0 = o0[:, 128:]
    mid1 = o1[:, :128]
    lo = jax.lax.broadcasted_iota(jnp.int32, mid0.shape, 1) < 64
    r = 1.0 / jnp.where(lo, mid1, mid0)
    rr = pltpu.roll(r, 64, 1)
    o = jnp.concatenate([
        o0[:, :128] * jnp.where(lo, rr, r),
        jnp.where(lo, mid0, mid1) * rr,
        o1[:, 128:] * jnp.where(lo, r, rr),
    ], axis=1).astype(bf16)
    return jax.lax.dot_general(o, wo, _NN, preferred_element_type=f32)


def _kernel(ax, akt, avt, awq, awo, bx, bkt, bvt, bwq, bwo, out, acc,
            *, nb, scale, d):
    p = pl.program_id(0)
    g = pl.program_id(1)
    last = pl.num_programs(0) - 1

    for i in range(nb):
        b = g * nb + i
        for (x, kt, vt, wq, wo, col) in ((ax, akt, avt, awq, awo, 0),
                                         (bx, bkt, bvt, bwq, bwo, d)):
            y = _pair_attention(x[i], wq[...], kt[i, 0], kt[i, 1],
                                vt[i, 0], vt[i, 1], wo[...], scale=scale)

            @pl.when(p == 0)
            def _():
                acc[b, :, col:col + d] = y

            @pl.when(jnp.logical_and(p > 0, p < last))
            def _():
                acc[b, :, col:col + d] += y

            @pl.when(p == last)
            def _():
                out[i, :, col:col + d] = (acc[b, :, col:col + d] + y).astype(out.dtype)


@jax.jit
def pallas_concat_heads__gqa_block_cached__mha_block_cached__near_ridge_kernel(
    A_x: jax.Array,
    A_k_cache: jax.Array,
    A_v_cache: jax.Array,
    A_wq: jax.Array,
    A_wo: jax.Array,
    B_x: jax.Array,
    B_k_cache: jax.Array,
    B_v_cache: jax.Array,
    B_wq: jax.Array,
    B_wo: jax.Array,
):
    B, Sq, D = A_x.shape
    _, H, Sk, Dh = A_k_cache.shape
    nb = 1
    npairs = H // 2
    scale = (Dh ** -0.5) * math.log2(math.e)

    akt, avt, bkt, bvt = (jnp.swapaxes(t, 2, 3) for t in
                          (A_k_cache, A_v_cache, B_k_cache, B_v_cache))

    x_spec = pl.BlockSpec((nb, Sq, D), lambda p, g: (g, 0, 0))
    kv_spec = pl.BlockSpec((nb, 2, Dh, Sk), lambda p, g: (g, p, 0, 0))
    wq_spec = pl.BlockSpec((D, 2 * Dh), lambda p, g: (0, p))
    wo_spec = pl.BlockSpec((2 * Dh, D), lambda p, g: (p, 0))
    out_spec = pl.BlockSpec(
        (nb, Sq, 2 * D),
        lambda p, g: (jnp.where(p == npairs - 1, g, 0), 0, 0))
    branch_specs = [x_spec, kv_spec, kv_spec, wq_spec, wo_spec]

    return pl.pallas_call(
        functools.partial(_kernel, nb=nb, scale=scale, d=D),
        grid=(npairs, B // nb),
        in_specs=branch_specs + branch_specs,
        out_specs=out_spec,
        out_shape=jax.ShapeDtypeStruct((B, Sq, 2 * D), A_x.dtype),
        scratch_shapes=[pltpu.VMEM((B, Sq, 2 * D), jnp.float32)],
        compiler_params=pltpu.CompilerParams(
            dimension_semantics=("arbitrary", "arbitrary"),
            vmem_limit_bytes=100 * 1024 * 1024,
        ),
    )(A_x, akt, avt, A_wq, A_wo, B_x, bkt, bvt, B_wq, B_wo)
```

```python
import functools
import math

import jax
import jax.numpy as jnp
import jax.experimental.pallas as pl
import jax.experimental.pallas.tpu as pltpu

_NN = (((1,), (0,)), ((), ()))
_NT = (((1,), (1,)), ((), ()))
NB = 4
CH = 16
DEP = 2
INLINE_OUT = 1
NOBC = 1
bf16 = jnp.bfloat16
f32 = jnp.float32


def _dot(a, b, dims=_NN):
    return jax.lax.dot_general(a, b, dims, preferred_element_type=f32)


def _recip(l):
    r = pl.reciprocal(l, approx=True)
    return r * (2.0 - l * r)


def _softmax_terms(s):
    sq, sk = s.shape
    es, rs, toks = [], [], []
    for ci, c in enumerate(range(0, sq, CH)):
        sc = s[c:c + CH]
        m = jnp.max(sc, axis=-1, keepdims=True)
        m = jnp.broadcast_to(m, (CH, 128))
        if DEP and ci >= DEP:
            m = jnp.where(toks[ci - DEP] < 0.0, 0.0, m)
        e = [jnp.exp2(sc[:, k:k + 128] - m) for k in range(0, sk, 128)]
        t = (e[0] + e[1]) + (e[2] + e[3])
        toks.append(t)
        l = jnp.broadcast_to(jnp.sum(t, axis=-1, keepdims=True), (CH, 128))
        rs.append(_recip(l))
        es.append(jnp.concatenate(e, axis=1))
    return jnp.concatenate(es, axis=0), jnp.concatenate(rs, axis=0)


def _scores(q, kt0, kt1):
    dh, sk = kt0.shape
    zeros = jnp.zeros((256 - dh, sk), bf16)
    s0 = _dot(q[0], jnp.concatenate([kt0, zeros], axis=0))
    s1 = _dot(q[1], jnp.concatenate([zeros, kt1], axis=0))
    return s0, s1


def _attend(s0, s1, vt0, vt1):
    sq = s0.shape[0]
    e0, r0 = _softmax_terms(s0)
    e1, r1 = _softmax_terms(s1)
    lo = jax.lax.broadcasted_iota(jnp.int32, (sq, 128), 1) < 64
    mid_t = jnp.concatenate([_dot(vt0[128:], e0[:128].astype(bf16), _NT),
                             _dot(vt1[:64], e1[:128].astype(bf16), _NT)], axis=0)
    tail = _dot(jnp.concatenate([e0[128:], e1[128:]], axis=0).astype(bf16),
                jnp.concatenate([vt0[128:], vt1[:64]], axis=0), _NT)
    o_lo = _dot(e0.astype(bf16), vt0[:128], _NT)
    o_hi = _dot(e1.astype(bf16), vt1[64:], _NT)
    nt = sq - 128
    lo_t = jax.lax.broadcasted_iota(jnp.int32, (nt, 128), 1) < 64
    mid = jnp.concatenate(
        [mid_t.T, jnp.where(lo_t, tail[:nt], tail[nt:])], axis=0)
    return jnp.concatenate([
        o_lo * r0,
        mid * jnp.where(lo, r0, r1),
        o_hi * r1,
    ], axis=1).astype(bf16)


def _kernel(ax, akt, avt, awq, awo, bx, bkt, bvt, bwq, bwo, out,
            xbuf, kvbuf, wqbuf, wobuf, acc, obuf,
            xsem, kvsem, wsem, osem,
            *, nb, scale, d, sq, nbatch, npairs, dh):
    ng = nbatch // nb
    n = 2 * nb
    xs, wqs, wos = (ax, bx), (awq, bwq), (awo, bwo)
    kvs = (akt, avt, bkt, bvt)

    def kv_start(pp, gg, slot):
        for t in range(4):
            pltpu.make_async_copy(kvs[t].at[pl.ds(gg * nb, nb), pl.ds(2 * pp, 2)],
                                  kvbuf.at[slot, t], kvsem.at[slot]).start()

    def kv_wait(slot):
        pltpu.make_async_copy(kvbuf.at[slot], kvbuf.at[slot], kvsem.at[slot]).wait()

    def w_copies(pp):
        slot = pp % 2
        col = pl.multiple_of(pp * (2 * dh), 128)
        cs = []
        for j in range(2):
            cs.append(pltpu.make_async_copy(wqs[j].at[:, pl.ds(col, 2 * dh)], wqbuf.at[slot, j], wsem.at[slot, j]))
        for j in range(2):
            cs.append(pltpu.make_async_copy(wos[j].at[pl.ds(col, 2 * dh), :], wobuf.at[slot, j], wsem.at[slot, 2 + j]))
        return cs

    def x_start(gg):
        for j in range(2):
            pltpu.make_async_copy(xs[j].at[pl.ds(gg * nb, nb)], xbuf.at[gg, j], xsem.at[gg]).start()

    def x_wait(gg):
        pltpu.make_async_copy(xbuf.at[gg], xbuf.at[gg], xsem.at[gg]).wait()

    def out_copy(b):
        return pltpu.make_async_copy(obuf.at[b], out.at[b], osem)

    x_start(0)
    for c in w_copies(0):
        c.start()
    kv_start(0, 0, 0)
    for gg in range(1, ng):
        x_start(gg)

    def step_body(p, g, wslot):
        step = p * ng + g
        slot = step % 2
        first = p == 0
        last = p == npairs - 1

        @pl.when(first)
        def _():
            x_wait(g)

        kv_wait(slot)
        gn = jnp.where(g + 1 < ng, g + 1, 0)
        pn = jnp.where(g + 1 < ng, p, jnp.minimum(p + 1, npairs - 1))
        kv_start(pn, gn, 1 - slot)

        q = {}
        o = {}

        def qproj(u):
            j, i = u % 2, u // 2
            qf = _dot(xbuf[g, j, i], wqbuf[wslot, j]) * scale
            q[u] = (qf[:, :256].astype(bf16), qf[:, 128:].astype(bf16))

        def oproj(u):
            j, i = u % 2, u // 2
            y = _dot(o.pop(u), wobuf[wslot, j])
            b = g * nb + i
            prev = acc[b, :, j * d:(j + 1) * d]
            y = y + jnp.where(first, 0.0, prev)
            acc[b, :, j * d:(j + 1) * d] = y
            if INLINE_OUT:
                obuf[b, :, j * d:(j + 1) * d] = y.astype(bf16)
                if j == 1:
                    @pl.when(last)
                    def _():
                        out_copy(b).start()

        qproj(0)
        qproj(1)
        for u in range(n):
            j, i = u % 2, u // 2
            s0, s1 = _scores(q.pop(u), kvbuf[slot, 2 * j, i, 0], kvbuf[slot, 2 * j, i, 1])
            if u >= 2:
                oproj(u - 2)
            if u + 2 < n:
                qproj(u + 2)
            o[u] = _attend(s0, s1, kvbuf[slot, 2 * j + 1, i, 0], kvbuf[slot, 2 * j + 1, i, 1])
        oproj(n - 2)
        oproj(n - 1)

        if not INLINE_OUT:
            @pl.when(last)
            def _():
                for i in range(nb):
                    b = g * nb + i
                    obuf[b] = acc[b].astype(bf16)
                    out_copy(b).start()

    def pair_body(p, carry):
        for c in w_copies(p):
            c.wait()

        @pl.when(p + 1 < npairs)
        def _():
            for c in w_copies(p + 1):
                c.start()

        wslot = p % 2

        def group_body(g, carry):
            step_body(p, g, wslot)
            return carry

        return jax.lax.fori_loop(0, ng, group_body, carry)

    jax.lax.fori_loop(0, npairs, pair_body, 0)

    kv_wait((npairs * ng) % 2)
    pltpu.make_async_copy(obuf, obuf, osem).wait()


@jax.jit
def pallas_concat_heads__gqa_block_cached__mha_block_cached__near_ridge_kernel(
    A_x, A_k_cache, A_v_cache, A_wq, A_wo, B_x, B_k_cache, B_v_cache, B_wq, B_wo,
):
    B, Sq, D = A_x.shape
    _, H, Sk, Dh = A_k_cache.shape
    nb = NB
    npairs = H // 2
    ng = B // nb
    scale = (Dh ** -0.5) * math.log2(math.e)

    akt, avt, bkt, bvt = (jnp.swapaxes(t, 2, 3) for t in
                          (A_k_cache, A_v_cache, B_k_cache, B_v_cache))
    any_spec = pl.BlockSpec(memory_space=pl.ANY)

    return pl.pallas_call(
        functools.partial(_kernel, nb=nb, scale=scale, d=D, sq=Sq,
                          nbatch=B, npairs=npairs, dh=Dh),
        in_specs=[any_spec] * 10,
        out_specs=any_spec,
        out_shape=jax.ShapeDtypeStruct((B, Sq, 2 * D), A_x.dtype),
        scratch_shapes=[
            pltpu.VMEM((ng, 2, nb, Sq, D), bf16),
            pltpu.VMEM((2, 4, nb, 2, Dh, Sk), bf16),
            pltpu.VMEM((2, 2, D, 2 * Dh), bf16),
            pltpu.VMEM((2, 2, 2 * Dh, D), bf16),
            pltpu.VMEM((B, Sq, 2 * D), f32),
            pltpu.VMEM((B, Sq, 2 * D), bf16),
            pltpu.SemaphoreType.DMA((ng,)),
            pltpu.SemaphoreType.DMA((2,)),
            pltpu.SemaphoreType.DMA((2, 4)),
            pltpu.SemaphoreType.DMA(()),
        ],
        compiler_params=pltpu.CompilerParams(
            vmem_limit_bytes=110 * 1024 * 1024,
            disable_bounds_checks=bool(NOBC),
        ),
    )(A_x, akt, avt, A_wq, A_wo, B_x, bkt, bvt, B_wq, B_wo)
```

```python
import functools
import math

import jax
import jax.numpy as jnp
import jax.experimental.pallas as pl
import jax.experimental.pallas.tpu as pltpu

_NN = (((1,), (0,)), ((), ()))
_NT = (((1,), (1,)), ((), ()))
NB = 4
CH = 16
DEP = 2
INLINE_OUT = 1
ORD = 0
QPACK = 1
F32CAT = 3
NPS = 2
bf16 = jnp.bfloat16
f32 = jnp.float32
i32 = jnp.int32


def _dot(a, b, dims=_NN):
    return jax.lax.dot_general(a, b, dims, preferred_element_type=f32)


def _recip(l):
    r = pl.reciprocal(l, approx=True)
    return r * (2.0 - l * r)


def _col(x, i):
    return x[:, 128 * i:128 * (i + 1)]


def _pack(x):
    return pltpu.bitcast(x.astype(bf16), i32)


def _unpack(x):
    return pltpu.bitcast(x, bf16)


def _softmax_terms(s, p_ref):
    sq, sk = s.shape
    rs, toks = [], []
    for ci, c in enumerate(range(0, sq, CH)):
        sc = s[c:c + CH]
        m = jnp.max(sc, axis=-1, keepdims=True)
        m = jnp.broadcast_to(m, (CH, 128))
        if DEP and ci >= DEP:
            never = toks[ci - DEP] < 0
            m = jnp.where(jnp.concatenate([never, never], axis=0), 0.0, m)
        e = [jnp.exp2(_col(sc, k) - m) for k in range(4)]
        t0, t1 = e[0] + e[2], e[1] + e[3]
        l = jnp.broadcast_to(jnp.sum(t0 + t1, axis=-1, keepdims=True), (CH, 128))
        rs.append(_recip(l))
        rows = slice(c // 2, (c + CH) // 2)
        for k, x in enumerate(e + [t0, t1]):
            p_ref[rows, 128 * k:128 * (k + 1)] = _pack(x)
        back = p_ref[rows, :]
        tok = _col(back, 0)
        for k in range(1, 6):
            tok = tok | _col(back, k)
        toks.append(tok)
    return jnp.concatenate(rs, axis=0)


def _lane_lo(rows):
    return jax.lax.broadcasted_iota(i32, (rows, 128), 1) < 64


def _q_operands(qf, q_ref):
    t0, t1, t2 = _col(qf, 0), _col(qf, 1), _col(qf, 2)
    rot = pltpu.roll(t1, 64, 1)
    if QPACK:
        for k, t in enumerate((t0, t1, t2, rot)):
            q_ref[k] = _pack(t)
        t0, t1, t2, rot = (q_ref[k] for k in range(4))
        fin = _unpack
    else:
        fin = lambda t: t.astype(bf16)
    lo = _lane_lo(t0.shape[0])
    h0 = (t0, jnp.where(lo, t0, rot), jnp.where(lo, t1, t0))
    h1 = (t2, jnp.where(lo, t2, t1), jnp.where(lo, rot, t2))
    return tuple(tuple(fin(t) for t in h) for h in (h0, h1))


def _weights(xa, xb, xc):
    h = xa.shape[1] // 2
    xa, xb, xc = xa.astype(f32), xb.astype(f32), xc.astype(f32)
    cat = lambda *xs: jnp.concatenate(xs, axis=0)
    return (cat(xa[:, :h], xb[:, :h] - xb[:, h:]),
            cat(xa[:, h:], xc[:, h:] - xc[:, :h]),
            cat(xc[:, :h], xb[:, h:]))


def _weights_mixed(xa, xb, xc):
    h = xa.shape[1] // 2
    d = lambda u, v: (u.astype(f32) - v.astype(f32)).astype(bf16)
    cat = lambda *xs: jnp.concatenate(xs, axis=0)
    return (cat(xa[:, :h], d(xb[:, :h], xb[:, h:])),
            cat(xa[:, h:], d(xc[:, h:], xc[:, :h])),
            cat(xc[:, :h], xb[:, h:]))


def _head_scores(l, ka, kb, kc):
    w1, w2, w3 = (_weights if F32CAT & 1 else _weights_mixed)(ka, kb, kc)
    out = [None] * 4
    for i in range(2):
        p3 = _dot(l[2], _col(w3, i).astype(bf16))
        p1 = _dot(l[0], _col(w1, i).astype(bf16))
        p2 = _dot(l[1], _col(w2, i).astype(bf16))
        out[i], out[i + 2] = p1 + p3, p2 + p3
    return jnp.concatenate(out, axis=1)


def _scores(q, kt0, kt1):
    s0 = _head_scores(q[0], kt0[:64], kt0[64:128], kt0[128:])
    s1 = _head_scores(q[1], kt1[64:128], kt1[128:], kt1[:64])
    return s0, s1


def _head_pv(p_ref, va, vb, vc):
    w1, w2, w3 = (_weights if F32CAT & 2 else _weights_mixed)(va, vb, vc)
    p1 = _dot(_unpack(p_ref[:, 0:256]), w1.astype(bf16), _NT)
    p2 = _dot(_unpack(p_ref[:, 256:512]), w2.astype(bf16), _NT)
    p3 = _dot(_unpack(p_ref[:, 512:768]), w3.astype(bf16), _NT)
    return p1, p2, p3


def _attend(s0, s1, vt0, vt1, p_ref):
    sq = s0.shape[0]
    r0 = _softmax_terms(s0, p_ref.at[0])
    r1 = _softmax_terms(s1, p_ref.at[1])
    lo = _lane_lo(sq)
    p1, p2, p3 = _head_pv(p_ref.at[0], vt0[:64], vt0[64:128], vt0[128:])
    u1, u2, u3 = _head_pv(p_ref.at[1], vt1[64:128], vt1[128:], vt1[:64])
    o_lo = p1 + jnp.where(lo, p2, p3)
    o_hi = u1 + jnp.where(lo, u2, u3)
    mid = jnp.where(lo, p3, u2) + pltpu.roll(jnp.where(lo, u3, p2), 64, 1)
    return jnp.concatenate([
        o_lo * r0,
        mid * jnp.where(lo, r0, r1),
        o_hi * r1,
    ], axis=1).astype(bf16)


def _kernel(ax, akt, avt, awq, awo, bx, bkt, bvt, bwq, bwo, out,
            xbuf, kvbuf, wqbuf, wobuf, acc, obuf, pbuf, qbuf,
            xsem, kvsem, wsem, osem,
            *, nb, scale, d, sq, nbatch, npairs, dh):
    ng = nbatch // nb
    n = 2 * nb
    xs, wqs, wos = (ax, bx), (awq, bwq), (awo, bwo)
    kvs = (akt, avt, bkt, bvt)

    def kv_start(pp, gg, slot):
        for t in range(4):
            pltpu.make_async_copy(kvs[t].at[pl.ds(gg * nb, nb), pl.ds(2 * pp, 2)],
                                  kvbuf.at[slot, t], kvsem.at[slot]).start()

    def kv_wait(slot):
        pltpu.make_async_copy(kvbuf.at[slot], kvbuf.at[slot], kvsem.at[slot]).wait()

    def w_copies(pp):
        slot = pp % 2
        col = pl.multiple_of(pp * (2 * dh), 128)
        cs = []
        for j in range(2):
            cs.append(pltpu.make_async_copy(wqs[j].at[:, pl.ds(col, 2 * dh)], wqbuf.at[slot, j], wsem.at[slot, j]))
        for j in range(2):
            cs.append(pltpu.make_async_copy(wos[j].at[pl.ds(col, 2 * dh), :], wobuf.at[slot, j], wsem.at[slot, 2 + j]))
        return cs

    def x_start(gg):
        for j in range(2):
            pltpu.make_async_copy(xs[j].at[pl.ds(gg * nb, nb)], xbuf.at[gg, j], xsem.at[gg]).start()

    def x_wait(gg):
        pltpu.make_async_copy(xbuf.at[gg], xbuf.at[gg], xsem.at[gg]).wait()

    def out_copy(b):
        return pltpu.make_async_copy(obuf.at[b], out.at[b], osem)

    x_start(0)
    for c in w_copies(0):
        c.start()
    kv_start(0, 0, 0)

    def step_body(p, g, wslot):
        step = p * ng + g
        slot = step % 2
        first = p == 0
        last = p == npairs - 1

        @pl.when(first)
        def _():
            x_wait(g)

        kv_wait(slot)
        gn = jnp.where(g + 1 < ng, g + 1, 0)
        pn = jnp.where(g + 1 < ng, p, jnp.minimum(p + 1, npairs - 1))
        kv_start(pn, gn, 1 - slot)

        @pl.when(jnp.logical_and(first, g + 1 < ng))
        def _():
            x_start(gn)

        q = {}
        o = {}

        def qproj(u):
            j, i = u % 2, u // 2
            qf = _dot(xbuf[g, j, i], wqbuf[wslot, j]) * scale
            q[u] = _q_operands(qf, qbuf.at[u % 4])

        def oproj(u):
            j, i = u % 2, u // 2
            y = _dot(o.pop(u), wobuf[wslot, j])
            b = g * nb + i
            prev = acc[b, :, j * d:(j + 1) * d]
            y = y + jnp.where(first, 0.0, prev)
            acc[b, :, j * d:(j + 1) * d] = y
            if INLINE_OUT:
                obuf[b, :, j * d:(j + 1) * d] = y.astype(bf16)
                if j == 1:
                    @pl.when(last)
                    def _():
                        out_copy(b).start()

        qproj(0)
        qproj(1)
        for u in range(n):
            j, i = u % 2, u // 2
            s0, s1 = _scores(q.pop(u), kvbuf[slot, 2 * j, i, 0], kvbuf[slot, 2 * j, i, 1])
            if ORD == 0:
                if u >= 2:
                    oproj(u - 2)
                if u + 2 < n:
                    qproj(u + 2)
            else:
                if u + 2 < n:
                    qproj(u + 2)
                if u >= 2:
                    oproj(u - 2)
            o[u] = _attend(s0, s1, kvbuf[slot, 2 * j + 1, i, 0], kvbuf[slot, 2 * j + 1, i, 1],
                           pbuf.at[u % NPS])
        oproj(n - 2)
        oproj(n - 1)

        if not INLINE_OUT:
            @pl.when(last)
            def _():
                for i in range(nb):
                    b = g * nb + i
                    obuf[b] = acc[b].astype(bf16)
                    out_copy(b).start()

    def pair_body(p, carry):
        for c in w_copies(p):
            c.wait()

        @pl.when(p + 1 < npairs)
        def _():
            for c in w_copies(p + 1):
                c.start()

        wslot = p % 2

        def group_body(g, carry):
            step_body(p, g, wslot)
            return carry

        return jax.lax.fori_loop(0, ng, group_body, carry)

    jax.lax.fori_loop(0, npairs, pair_body, 0)

    kv_wait((npairs * ng) % 2)
    pltpu.make_async_copy(obuf, obuf, osem).wait()


@jax.jit
def pallas_concat_heads__gqa_block_cached__mha_block_cached__near_ridge_kernel(
    A_x, A_k_cache, A_v_cache, A_wq, A_wo, B_x, B_k_cache, B_v_cache, B_wq, B_wo,
):
    B, Sq, D = A_x.shape
    _, H, Sk, Dh = A_k_cache.shape
    nb = NB
    npairs = H // 2
    ng = B // nb
    scale = (Dh ** -0.5) * math.log2(math.e)

    akt, avt, bkt, bvt = (jnp.swapaxes(t, 2, 3) for t in
                          (A_k_cache, A_v_cache, B_k_cache, B_v_cache))
    any_spec = pl.BlockSpec(memory_space=pl.ANY)

    return pl.pallas_call(
        functools.partial(_kernel, nb=nb, scale=scale, d=D, sq=Sq,
                          nbatch=B, npairs=npairs, dh=Dh),
        in_specs=[any_spec] * 10,
        out_specs=any_spec,
        out_shape=jax.ShapeDtypeStruct((B, Sq, 2 * D), A_x.dtype),
        scratch_shapes=[
            pltpu.VMEM((ng, 2, nb, Sq, D), bf16),
            pltpu.VMEM((2, 4, nb, 2, Dh, Sk), bf16),
            pltpu.VMEM((2, 2, D, 2 * Dh), bf16),
            pltpu.VMEM((2, 2, 2 * Dh, D), bf16),
            pltpu.VMEM((B, Sq, 2 * D), f32),
            pltpu.VMEM((B, Sq, 2 * D), bf16),
            pltpu.VMEM((NPS, 2, Sq // 2, 768), i32),
            pltpu.VMEM((4, 4, Sq // 2, 128), i32),
            pltpu.SemaphoreType.DMA((ng,)),
            pltpu.SemaphoreType.DMA((2,)),
            pltpu.SemaphoreType.DMA((2, 4)),
            pltpu.SemaphoreType.DMA(()),
        ],
        compiler_params=pltpu.CompilerParams(
            vmem_limit_bytes=110 * 1024 * 1024,
            disable_bounds_checks=True,
        ),
    )(A_x, akt, avt, A_wq, A_wo, B_x, bkt, bvt, B_wq, B_wo)
```

```python
import functools
import math

import jax
import jax.numpy as jnp
import jax.experimental.pallas as pl
import jax.experimental.pallas.tpu as pltpu

_NN = (((1,), (0,)), ((), ()))
_NT = (((1,), (1,)), ((), ()))
CH = 16
DEP = 3
ORD = 0
ONE = 0
SERIAL = 0
NPS = 4
PRENORM = 0
NDEP = 0
SEQS = [
    'q00 w0 q01 s01 w1 q02 w2 q03 p01 s02 w3 q10 p02 s00 o00 q11 p00 s03 o01 q12 p03 s11 o02 q13 p11 s12 o03 s10 p12 o10 s13 p10 o11 p13 o12 o13',
]
bf16 = jnp.bfloat16
f32 = jnp.float32
i32 = jnp.int32


def _dot(a, b, dims=_NN):
    return jax.lax.dot_general(a, b, dims, preferred_element_type=f32)


def _recip(l):
    r = pl.reciprocal(l, approx=True)
    return r * (2.0 - l * r)


def _col(x, i):
    return x[:, 128 * i:128 * (i + 1)]


def _pack(x):
    return pltpu.bitcast(x.astype(bf16), i32)


def _unpack(x):
    return pltpu.bitcast(x, bf16)


def _or_tiles(v):
    t = None
    for r in range(0, v.shape[0], 8):
        for c in range(0, v.shape[1], 128):
            x = v[r:r + 8, c:c + 128]
            t = x if t is None else t | x
    return t


def _after(x, tok, zero):
    t = tok & zero
    return pltpu.bitcast(pltpu.bitcast(x, i32) | jnp.concatenate([t, t], axis=0), f32)


def _softmax_terms(ss, p_refs, zero):
    sq = ss[0].shape[0]
    n = sq // CH
    if SERIAL:
        chains = [[(h, c) for h in range(2) for c in range(n)]]
    else:
        chains = [[(h, c) for c in range(n)] for h in range(2)]
    ls = {}
    for chain in chains:
        toks = []
        for ci, (h, c) in enumerate(chain):
            sc = ss[h][c * CH:(c + 1) * CH]
            m = jnp.broadcast_to(jnp.max(sc, axis=-1, keepdims=True), (CH, 128))
            if ci >= DEP:
                m = _after(m, toks[ci - DEP], zero)
            e = [jnp.exp2(_col(sc, k) - m) for k in range(4)]
            t0, t1 = e[0] + e[2], e[1] + e[3]
            l = jnp.broadcast_to(jnp.sum(t0 + t1, axis=-1, keepdims=True), (CH, 128))
            vals = e + [t0, t1]
            if PRENORM:
                r = _recip(l)
                vals = [v * r for v in vals]
            ls[h, c] = l
            rows = slice(c * CH // 2, (c + 1) * CH // 2)
            for k, x in enumerate(vals):
                p_refs[h][rows, 128 * k:128 * (k + 1)] = _pack(x)
            toks.append(_or_tiles(p_refs[h][rows, :]))
    return ls


def _lane_lo(rows):
    return jax.lax.broadcasted_iota(i32, (rows, 128), 1) < 64


def _q_operands(q_ref, fin):
    t0, t1, t2, rot = (q_ref[k] for k in range(4))
    lo = _lane_lo(t0.shape[0])
    h0 = (t0, jnp.where(lo, t0, rot), jnp.where(lo, t1, t0))
    h1 = (t2, jnp.where(lo, t2, t1), jnp.where(lo, rot, t2))
    return tuple(tuple(functools.partial(fin, t) for t in h) for h in (h0, h1))


def _weights(xa, xb, xc):
    h = xa.shape[1] // 2
    xa, xb, xc = xa.astype(f32), xb.astype(f32), xc.astype(f32)
    cat = lambda *xs: jnp.concatenate(xs, axis=0)
    return (cat(xa[:, :h], xb[:, :h] - xb[:, h:]),
            cat(xa[:, h:], xc[:, h:] - xc[:, :h]),
            cat(xc[:, :h], xb[:, h:]))


def _scores(q, kt0, kt1):
    w = (_weights(kt0[:64], kt0[64:128], kt0[128:]), _weights(kt1[64:128], kt1[128:], kt1[:64]))
    d = lambda h, k, i: _dot(q[h][k](), _col(w[h][k], i).astype(bf16))
    p = {}
    for t, (h, i) in enumerate(((0, 0), (0, 1), (1, 0))):
        for k in (2, 0, 1):
            p[h, k, i] = d(h, k, i)
        k = (2, 0, 1)[t]
        p[1, k, 1] = d(1, k, 1)
    return tuple(jnp.concatenate([p[h, 0, 0] + p[h, 2, 0], p[h, 0, 1] + p[h, 2, 1],
                                  p[h, 1, 0] + p[h, 2, 0], p[h, 1, 1] + p[h, 2, 1]], axis=1)
                 for h in range(2))


def _pv_products(p_ref, vt0, vt1, lhs):
    w = (_weights(vt0[:64], vt0[64:128], vt0[128:]), _weights(vt1[64:128], vt1[128:], vt1[:64]))
    r = {}
    for h, k in ((0, 1), (0, 2), (1, 1), (1, 2), (0, 0), (1, 0)):
        r[h, k] = _dot(lhs(p_ref.at[h][:, 256 * k:256 * (k + 1)]), w[h][k].astype(bf16), _NT)
    return tuple(r[h, k] for h in range(2) for k in range(3))


def _attend(ls, vt0, vt1, p_ref, zero, sink, lhs):
    sq = 2 * p_ref.shape[1]
    lo = _lane_lo(CH)
    pu = _pv_products(p_ref, vt0, vt1, lhs)
    toks = []
    for c in range(sq // CH):
        p1, p2, p3, u1, u2, u3 = (x[c * CH:(c + 1) * CH] for x in pu)
        if PRENORM:
            if NDEP and c >= NDEP:
                p2 = _after(p2, toks[c - NDEP], zero)
                u2 = _after(u2, toks[c - NDEP], zero)
        else:
            l0, l1 = ls[0, c], ls[1, c]
            if NDEP and c >= NDEP:
                l0 = _after(l0, toks[c - NDEP], zero)
                l1 = _after(l1, toks[c - NDEP], zero)
            r0, r1 = _recip(l0), _recip(l1)
        o_lo = p1 + jnp.where(lo, p2, p3)
        o_hi = u1 + jnp.where(lo, u2, u3)
        mid = jnp.where(lo, p3, u2) + pltpu.roll(jnp.where(lo, u3, p2), 64, 1)
        if not PRENORM:
            o_lo, mid, o_hi = o_lo * r0, mid * jnp.where(lo, r0, r1), o_hi * r1
        toks.append(sink(c, jnp.concatenate([o_lo, mid, o_hi], axis=1)))
    return functools.reduce(jnp.bitwise_or, toks[-max(NDEP, 1):]) if NDEP else functools.reduce(jnp.bitwise_or, toks)


def _lhs_combos(a11, a12, a21, a22):
    return (a11 + a22, a21 + a22, a11, a22, a11 + a12, a21 - a11, a12 - a22)


def _rhs_combos(b11, b12, b21, b22):
    return (b11 + b22, b11, b12 - b22, b21 - b11, b22, b11 + b12, b21 + b22)


def _strassen(m, order=(0, 3, 4, 2, 1, 5, 6)):
    p = {k: m(k) for k in order}
    return (p[0] + p[3] - p[4] + p[6], p[2] + p[4], p[1] + p[3], p[0] - p[1] + p[2] + p[5])


def _kernel(ax, akt, avt, awq, awo, bx, bkt, bvt, bwq, bwo, out,
            xbuf, xc, x4, kvbuf, rq, ro, rq0, ro0,
            wqc0, wq40, woc0, wo40, wqc1, wq41, woc1, wo41,
            acc, obuf, pbuf, qbuf, oc, zref,
            xsem, kvsem, rqsem, rosem, isem, osem,
            *, scale, d, sq, nbatch, npass, dh):
    ng = nbatch // 2
    gw = 4 * dh
    hw = 2 * dh
    qr, q4r, orr = 256 // ng, 128 // ng, hw // ng
    xs, wqs, wos = (ax, bx), (awq, bwq), (awo, bwo)
    kvs = (akt, avt, bkt, bvt)
    wsets = ((wqc0, wq40, woc0, wo40), (wqc1, wq41, woc1, wo41))

    def kv_start(pp, gg, slot):
        for t in range(4):
            pltpu.make_async_copy(kvs[t].at[pl.ds(gg * 2, 2), pl.ds(4 * pp, 4)],
                                  kvbuf.at[slot, t], kvsem.at[slot]).start()

    def raw_start(pp, gg, rq_ref, ro_ref, qsem, osem_):
        col = pl.multiple_of(pp * gw, 128)
        for j in range(2):
            for src, dst, n in ((gg * qr, 0, qr), (256 + gg * qr, qr, qr), (512 + gg * q4r, 2 * qr, q4r)):
                pltpu.make_async_copy(wqs[j].at[pl.ds(pl.multiple_of(src, 16), n), pl.ds(col, gw)],
                                      rq_ref.at[j, pl.ds(dst, n)], qsem).start()
            for h in range(2):
                src = pl.multiple_of(pp * gw + h * hw + gg * orr, 16)
                pltpu.make_async_copy(wos[j].at[pl.ds(src, orr)],
                                      ro_ref.at[j, pl.ds(h * orr, orr)], osem_).start()

    def wait_all(ref, sem):
        pltpu.make_async_copy(ref, ref, sem).wait()

    def x_start(gg):
        for j in range(2):
            pltpu.make_async_copy(xs[j].at[pl.ds(gg * 2, 2)], xbuf.at[gg, j], xsem.at[gg]).start()

    def out_copy(b):
        return pltpu.make_async_copy(obuf.at[b], out.at[b], osem)

    def build_x(gg):
        for j in range(2):
            x0 = xbuf[gg, j, 0].astype(f32)
            x1 = xbuf[gg, j, 1].astype(f32)
            cs = _lhs_combos(x0[:, :256], x0[:, 256:512], x1[:, :256], x1[:, 256:512])
            for k, c in enumerate(cs):
                xc.at[gg, j, k][...] = _pack(c)
            x4.at[gg, j, 0][...] = _pack(x0[:, 512:])
            x4.at[gg, j, 1][...] = _pack(x1[:, 512:])

    def build_wq(j, gg, rq_ref, wset):
        wqc, wq4, _, _ = wset
        r = rq_ref[j].astype(f32)
        cs = _rhs_combos(r[:qr, :hw], r[:qr, hw:], r[qr:2 * qr, :hw], r[qr:2 * qr, hw:])
        rows = pl.ds(pl.multiple_of(gg * (qr // 2), 8), qr // 2)
        rows4 = pl.ds(pl.multiple_of(gg * (q4r // 2), 8), q4r // 2)
        dst = [(wqc.at[j, k], rows) for k in range(7)] + [(wq4.at[j], rows4)]
        for (ref, rr), c in zip(dst, cs + (r[2 * qr:],)):
            ref[rr, :] = _pack(c)
        return [ref[rr, :] for ref, rr in dst]

    def build_wo(j, gg, ro_ref, wset):
        _, _, woc, wo4 = wset
        r = ro_ref[j].astype(f32)
        cs = _rhs_combos(r[orr:, :256], r[orr:, 256:512], r[:orr, :256], r[:orr, 256:512])
        rows = pl.ds(pl.multiple_of(gg * (orr // 2), 8), orr // 2)
        dst = [woc.at[j, k] for k in range(7)] + [wo4.at[j, h] for h in range(2)]
        for ref, c in zip(dst, cs + (r[:orr, 512:], r[orr:, 512:])):
            ref[rows, :] = _pack(c)
        return [ref[rows, :] for ref in dst]

    zref[0] = 0
    x_start(0)
    for gg in range(ng):
        raw_start(0, gg, rq0.at[gg], ro0.at[gg], isem.at[0], isem.at[1])
    kv_start(0, 0, 0)
    raw_start(1, 0, rq.at[0], ro.at[0], rqsem.at[0], rosem.at[0])
    wait_all(rq0, isem.at[0])
    wait_all(ro0, isem.at[1])

    def init_body(gg, carry):
        for j in range(2):
            build_wq(j, gg, rq0.at[gg], wsets[0])
            build_wo(j, gg, ro0.at[gg], wsets[0])
        return carry

    jax.lax.fori_loop(0, ng, init_body, 0)

    def step_body(p, g, cur, nxt):
        wqc, wq4, woc, wo4 = cur
        slot = g % 2
        first = p == 0
        last = p == npass - 1

        @pl.when(first)
        def _():
            wait_all(xbuf.at[g], xsem.at[g])
            build_x(g)

        wait_all(kvbuf.at[slot], kvsem.at[slot])
        wait_all(rq.at[slot], rqsem.at[slot])
        wait_all(ro.at[slot], rosem.at[slot])
        gn = jnp.where(g + 1 < ng, g + 1, 0)
        pn = jnp.where(g + 1 < ng, p, jnp.minimum(p + 1, npass - 1))
        kv_start(pn, gn, 1 - slot)
        raw_start(jnp.minimum(pn + 1, npass - 1), gn, rq.at[1 - slot], ro.at[1 - slot],
                  rqsem.at[1 - slot], rosem.at[1 - slot])

        @pl.when(jnp.logical_and(first, g + 1 < ng))
        def _():
            x_start(gn)

        s, qm, om, toks = {}, {}, {}, []
        zero = jnp.full((8, 128), zref[0], i32)

        def lhs(x):
            if toks:
                t = toks.pop(0)
                x = jnp.concatenate([x[:8] | jnp.concatenate([t & zero] * (x.shape[1] // 128), axis=1), x[8:]], axis=0)
            return _unpack(x)

        def token(vals):
            t = None
            for v in vals:
                for r in range(0, v.shape[0], 8):
                    for c in range(0, v.shape[1], 128):
                        x = v[r:r + 8, c:c + 128]
                        t = x if t is None else t | x
            return t

        def qM(j, k, n):
            qm[j, k, n] = _dot(lhs(xc[g, j, k]), _unpack(wqc[j, k, :, 128 * n:128 * (n + 1)]))

        def qK(j, u, n):
            col = (u % 2) * hw + 128 * n
            qm[j, 'k', u, n] = _dot(lhs(x4[g, j, u // 2]), _unpack(wq4[j, :, col:col + 128]))

        def qfin(j, u):
            for n in range(3):
                m = lambda k: qm[j, k, n]
                c = (lambda: (m(0) + qm[j, 'k', 0, n]) + m(6) + (m(3) - m(4)),
                     lambda: m(2) + m(4) + qm[j, 'k', 1, n],
                     lambda: m(1) + m(3) + qm[j, 'k', 2, n],
                     lambda: (m(0) + qm[j, 'k', 3, n]) + m(5) + (m(2) - m(1)))[u]()
                y = c * scale
                qbuf.at[j, u, n][...] = _pack(y)
                if n == 1:
                    qbuf.at[j, u, 3][...] = _pack(pltpu.roll(y, 64, 1))

        def qp(j, part):
            if part == 0:
                for n in range(3):
                    qM(j, 2, n), qM(j, 4, n)
                if j == 0:
                    qK(0, 1, 0), qK(0, 1, 1), qK(0, 1, 2), qK(0, 2, 0)
                else:
                    qK(1, 1, 2), qK(1, 2, 0), qK(1, 2, 1), qK(1, 2, 2)
                qfin(j, 1)
            elif part == 1:
                for n in range(3):
                    qM(j, 1, n), qM(j, 3, n)
                if j == 0:
                    qK(0, 2, 1), qK(0, 2, 2), qK(1, 1, 0), qK(1, 1, 1)
                qfin(j, 2)
            elif part == 2:
                for n in range(3):
                    qM(j, 0, n), qK(j, 0, n), qK(j, 3, n)
            else:
                for n in range(3):
                    qM(j, 6, n), qM(j, 5, n)
                qfin(j, 0)
                qfin(j, 3)

        def sc(j, u):
            i, t = u // 2, u % 2
            s[j, u] = _scores(_q_operands(qbuf.at[j, u], lhs),
                              kvbuf[slot, 2 * j, i, 2 * t], kvbuf[slot, 2 * j, i, 2 * t + 1])

        def pslot(j, u):
            return pbuf.at[(4 * j + (1, 2, 0, 3).index(u)) % NPS]

        def sm(j, u):
            p_ref = pslot(j, u)
            s[j, u] = _softmax_terms(s[j, u], (p_ref.at[0], p_ref.at[1]), zero)

        def pv(j, u):
            i, t = u // 2, u % 2
            if not isinstance(s[j, u], dict):
                sm(j, u)

            def sink(c, o):
                rows = slice(c * CH // 2, (c + 1) * CH // 2)
                prev = lambda k: _unpack(oc.at[j, k][rows, :]).astype(f32)
                new = {1: lambda: {2: o},
                       2: lambda: {3: o, 0: prev(2) + o},
                       0: lambda: {7: o, 4: prev(2) + o, 6: o - prev(3)},
                       3: lambda: {8: o, 1: o + prev(3), 5: o - prev(2)}}[u]()
                for k, v in new.items():
                    oc.at[j, k][rows, :] = _pack(v)
                return functools.reduce(jnp.bitwise_or, [_or_tiles(oc.at[j, k][rows, :]) for k in new])

            pend[j, u] = _attend(s.pop((j, u)), kvbuf[slot, 2 * j + 1, i, 2 * t], kvbuf[slot, 2 * j + 1, i, 2 * t + 1],
                                 pslot(j, u), zero, sink, lhs)

        pend = {}

        def gate_o(j, u):
            toks.append(pend.pop((j, u)))

        def emit(j, i, col, y):
            b = 2 * g + i
            cols = slice(j * d + col, j * d + col + 128)
            y = y + jnp.where(first, 0.0, acc[b, :, cols])
            acc[b, :, cols] = y
            obuf[b, :, cols] = y.astype(bf16)

        def oM(j, k, c):
            om[j, k, c] = _dot(lhs(oc[j, k]), _unpack(woc[j, k, :, 128 * c:128 * (c + 1)]))

        def oN(j, i, tiles):
            for t in tiles:
                h, kt = t // 3, t % 3
                src = ((7, 2), (3, 8))[i][h]
                y = _dot(lhs(oc.at[j, src][:, 128 * kt:128 * (kt + 1)]),
                         _unpack(wo4.at[j, h][64 * kt:64 * (kt + 1), :]))
                om[j, 'n', i] = om[j, 'n', i] + y if (j, 'n', i) in om else y

        def op(j, part):
            m = lambda k, c: om[j, k, c]
            if part == 0:
                oM(j, 2, 0), oM(j, 2, 1)
                oN(j, 0, (3, 4))
            elif part == 1:
                for c in range(2):
                    oM(j, 0, c), oM(j, 3, c)
                if j == 1:
                    oN(0, 1, (0, 1))
                    emit(0, 1, 512, om[0, 'n', 1])
                    oN(1, 1, (0, 1))
            elif part == 2:
                for c in range(2):
                    oM(j, 4, c), oM(j, 6, c)
                    emit(j, 0, 256 + 128 * c, m(2, c) + m(4, c))
                    emit(j, 0, 128 * c, (m(0, c) + m(3, c) - m(4, c)) + m(6, c))
                oN(j, 0, (5, 0, 1, 2))
                emit(j, 0, 512, om[j, 'n', 0])
            else:
                for c in range(2):
                    oM(j, 1, c), oM(j, 5, c)
                    emit(j, 1, 128 * c, m(1, c) + m(3, c))
                    emit(j, 1, 256 + 128 * c, (m(0, c) + m(2, c) - m(1, c)) + m(5, c))
                oN(j, 1, (2, 3, 4, 5))
                if j == 1:
                    emit(1, 1, 512, om[1, 'n', 1])

        def build(k):
            j = k // 2
            back = (build_wq(j, g, rq.at[slot], nxt) if k % 2 == 0
                    else build_wo(j, g, ro.at[slot], nxt))
            toks.append(token(back))

        seq = SEQS[ORD]
        for tok in seq.split():
            kind, a = tok[0], [int(ch) for ch in tok[1:]]
            {'q': qp, 's': sc, 'p': pv, 'o': op, 'w': build, 'g': gate_o, 'x': sm}[kind](*a)

        @pl.when(last)
        def _():
            out_copy(2 * g).start()
            out_copy(2 * g + 1).start()

    def pass_pair(pp, carry):
        for par in range(1 if ONE else 2):
            p = 2 * pp + par

            def group_body(g, carry, p=p, par=par):
                step_body(p, g, wsets[par], wsets[1 - par])
                return carry

            carry = jax.lax.fori_loop(0, ng, group_body, carry)
        return carry

    jax.lax.fori_loop(0, npass // 2, pass_pair, 0)

    if ONE:
        z = zref[0]
        k = pbuf[z, z, 0:8, 0:128] | qbuf[z, z, z, 0:8, :] | oc[z, z, 0:8, 0:128]
        k = k | wqc1[z, z, 0:8, 0:128] | wq41[z, 0:8, 0:128] | woc1[z, z, 0:8, 0:128] | wo41[z, z, 0:8, :]
        obuf[0, 0:8, 0:128] = pltpu.bitcast(k, f32).astype(bf16)
    wait_all(kvbuf.at[0], kvsem.at[0])
    wait_all(rq.at[0], rqsem.at[0])
    wait_all(ro.at[0], rosem.at[0])
    wait_all(obuf, osem)


@jax.jit
def pallas_concat_heads__gqa_block_cached__mha_block_cached__near_ridge_kernel(
    A_x, A_k_cache, A_v_cache, A_wq, A_wo, B_x, B_k_cache, B_v_cache, B_wq, B_wo,
):
    B, Sq, D = A_x.shape
    _, H, Sk, Dh = A_k_cache.shape
    npass = H // 4
    ng = B // 2
    scale = (Dh ** -0.5) * math.log2(math.e)
    gw, hw = 4 * Dh, 2 * Dh
    rqn, ron = 640 // ng, gw // ng

    akt, avt, bkt, bvt = (jnp.swapaxes(t, 2, 3) for t in
                          (A_k_cache, A_v_cache, B_k_cache, B_v_cache))
    any_spec = pl.BlockSpec(memory_space=pl.ANY)
    wset = [
        pltpu.VMEM((2, 7, 128, hw), i32),
        pltpu.VMEM((2, 64, gw), i32),
        pltpu.VMEM((2, 7, hw // 2, 256), i32),
        pltpu.VMEM((2, 2, hw // 2, 128), i32),
    ]

    return pl.pallas_call(
        functools.partial(_kernel, scale=scale, d=D, sq=Sq,
                          nbatch=B, npass=npass, dh=Dh),
        in_specs=[any_spec] * 10,
        out_specs=any_spec,
        out_shape=jax.ShapeDtypeStruct((B, Sq, 2 * D), A_x.dtype),
        scratch_shapes=[
            pltpu.VMEM((ng, 2, 2, Sq, D), bf16),
            pltpu.VMEM((ng, 2, 7, Sq // 2, 256), i32),
            pltpu.VMEM((ng, 2, 2, Sq // 2, 128), i32),
            pltpu.VMEM((2, 4, 2, 4, Dh, Sk), bf16),
            pltpu.VMEM((2, 2, rqn, gw), bf16),
            pltpu.VMEM((2, 2, ron, D), bf16),
            pltpu.VMEM((ng, 2, rqn, gw), bf16),
            pltpu.VMEM((ng, 2, ron, D), bf16),
            *wset, *wset,
            pltpu.VMEM((B, Sq, 2 * D), f32),
            pltpu.VMEM((B, Sq, 2 * D), bf16),
            pltpu.VMEM((NPS, 2, Sq // 2, 768), i32),
            pltpu.VMEM((2, 4, 4, Sq // 2, 128), i32),
            pltpu.VMEM((2, 9, Sq // 2, hw), i32),
            pltpu.SMEM((1,), i32),
            pltpu.SemaphoreType.DMA((ng,)),
            pltpu.SemaphoreType.DMA((2,)),
            pltpu.SemaphoreType.DMA((2,)),
            pltpu.SemaphoreType.DMA((2,)),
            pltpu.SemaphoreType.DMA((2,)),
            pltpu.SemaphoreType.DMA(()),
        ],
        compiler_params=pltpu.CompilerParams(
            vmem_limit_bytes=110 * 1024 * 1024,
            disable_bounds_checks=True,
        ),
    )(A_x, akt, avt, A_wq, A_wo, B_x, bkt, bvt, B_wq, B_wo)
```

```python
import functools
import math

import jax
import jax.numpy as jnp
import jax.experimental.pallas as pl
import jax.experimental.pallas.tpu as pltpu

_NN = (((1,), (0,)), ((), ()))
_NT = (((1,), (1,)), ((), ()))
CH = 16
DEP = 3
ORD = 0
NODMA = 0
NPP = 4
NOBX = 0
RMIX = 0
RGATE = 0
Q2 = 0
ONE = 0
SERIAL = 0
NPS = 4
PRENORM = 0
NDEP = 0
SEQS = [
    'q00 w0 q01 s01 q02 w1 p01 w2 s02 w3 q03 q10 p02 s00 q11 p00 s03 o01 o00 p03 s11 q12 q13 o02 p11 s12 o03 s10 p12 o10 s13 p10 o11 p13 o12 o13',
]
bf16 = jnp.bfloat16
f32 = jnp.float32
i32 = jnp.int32


def _dot(a, b, dims=_NN):
    return jax.lax.dot_general(a, b, dims, preferred_element_type=f32)


def _recip(l):
    r = pl.reciprocal(l, approx=True)
    return r * (2.0 - l * r)


def _col(x, i):
    return x[:, 128 * i:128 * (i + 1)]


def _pack(x):
    return pltpu.bitcast(x.astype(bf16), i32)


def _unpack(x):
    return pltpu.bitcast(x, bf16)


def _or_tiles(v):
    t = None
    for r in range(0, v.shape[0], 8):
        for c in range(0, v.shape[1], 128):
            x = v[r:r + 8, c:c + 128]
            t = x if t is None else t | x
    return t


def _after(x, tok, zero):
    t = tok & zero
    return pltpu.bitcast(pltpu.bitcast(x, i32) | jnp.concatenate([t, t], axis=0), f32)


def _softmax_terms(ss, p_refs, zero):
    sq = ss[0].shape[0]
    n = sq // CH
    if SERIAL:
        chains = [[(h, c) for h in range(2) for c in range(n)]]
    else:
        chains = [[(h, c) for c in range(n)] for h in range(2)]
    ls = {}
    for chain in chains:
        toks = []
        for ci, (h, c) in enumerate(chain):
            sc = ss[h][c * CH:(c + 1) * CH]
            m = jnp.broadcast_to(jnp.max(sc, axis=-1, keepdims=True), (CH, 128))
            if ci >= DEP:
                m = _after(m, toks[ci - DEP], zero)
            e = [jnp.exp2(_col(sc, k) - m) for k in range(4)]
            t0, t1 = e[0] + e[2], e[1] + e[3]
            l = jnp.broadcast_to(jnp.sum(t0 + t1, axis=-1, keepdims=True), (CH, 128))
            vals = e + [t0, t1]
            if PRENORM:
                r = _recip(l)
                vals = [v * r for v in vals]
            ls[h, c] = l
            rows = slice(c * CH // 2, (c + 1) * CH // 2)
            for k, x in enumerate(vals):
                p_refs[h][rows, 128 * k:128 * (k + 1)] = _pack(x)
            toks.append(_or_tiles(p_refs[h][rows, :]))
    return ls


def _lane_lo(rows):
    return jax.lax.broadcasted_iota(i32, (rows, 128), 1) < 64


def _q_operands(q_ref, fin):
    t0, t1, t2, rot = (q_ref[:, 128 * k:128 * (k + 1)] for k in range(4))
    lo = _lane_lo(t0.shape[0])
    h0 = (t0, jnp.where(lo, t0, rot), jnp.where(lo, t1, t0))
    h1 = (t2, jnp.where(lo, t2, t1), jnp.where(lo, rot, t2))
    return tuple(tuple(functools.partial(fin, t) for t in h) for h in (h0, h1))


def _weights(xa, xb, xc):
    h = xa.shape[1] // 2
    xa, xb, xc = xa.astype(f32), xb.astype(f32), xc.astype(f32)
    cat = lambda *xs: jnp.concatenate(xs, axis=0)
    return (cat(xa[:, :h], xb[:, :h] - xb[:, h:]),
            cat(xa[:, h:], xc[:, h:] - xc[:, :h]),
            cat(xc[:, :h], xb[:, h:]))


def _scores(q, kt0, kt1):
    w = (_weights(kt0[:64], kt0[64:128], kt0[128:]), _weights(kt1[64:128], kt1[128:], kt1[:64]))
    d = lambda h, k, i: _dot(q[h][k](), _col(w[h][k], i).astype(bf16))
    p = {}
    for t, (h, i) in enumerate(((0, 0), (0, 1), (1, 0))):
        for k in (2, 0, 1):
            p[h, k, i] = d(h, k, i)
        k = (2, 0, 1)[t]
        p[1, k, 1] = d(1, k, 1)
    return tuple(jnp.concatenate([p[h, 0, 0] + p[h, 2, 0], p[h, 0, 1] + p[h, 2, 1],
                                  p[h, 1, 0] + p[h, 2, 0], p[h, 1, 1] + p[h, 2, 1]], axis=1)
                 for h in range(2))


def _pv_products(p_ref, vt0, vt1, lhs):
    w = (_weights(vt0[:64], vt0[64:128], vt0[128:]), _weights(vt1[64:128], vt1[128:], vt1[:64]))
    r = {}
    for h, k in ((0, 1), (0, 2), (1, 1), (1, 2), (0, 0), (1, 0)):
        r[h, k] = _dot(lhs(p_ref.at[h][:, 256 * k:256 * (k + 1)]), w[h][k].astype(bf16), _NT)
    return tuple(r[h, k] for h in range(2) for k in range(3))


def _attend(ls, vt0, vt1, p_ref, sink, lhs):
    n = 2 * p_ref.shape[1] // CH
    lo = _lane_lo(CH)
    pu = _pv_products(p_ref, vt0, vt1, lhs)

    def rows(c):
        p1, p2, p3, u1, u2, u3 = (x[c * CH:(c + 1) * CH] for x in pu)
        if RMIX:
            rm = ls[c]
            rr = pltpu.roll(rm, 64, 1)
            r0, r1 = jnp.where(lo, rm, rr), jnp.where(lo, rr, rm)
        else:
            r0, r1 = _recip(ls[0, c]), _recip(ls[1, c])
            rm = jnp.where(lo, r0, r1)
        o_lo = p1 + jnp.where(lo, p2, p3)
        o_hi = u1 + jnp.where(lo, u2, u3)
        mid = jnp.where(lo, p3, u2) + pltpu.roll(jnp.where(lo, u3, p2), 64, 1)
        return jnp.concatenate([o_lo * r0, mid * rm, o_hi * r1], axis=1)

    for c in range(n // 2):
        sink(c, rows(c), rows(c + n // 2))


def _lhs_combos(a11, a12, a21, a22):
    return (a11 + a22, a21 + a22, a11, a22, a11 + a12, a21 - a11, a12 - a22)


def _rhs_combos(b11, b12, b21, b22):
    return (b11 + b22, b11, b12 - b22, b21 - b11, b22, b11 + b12, b21 + b22)


def _strassen(m, order=(0, 3, 4, 2, 1, 5, 6)):
    p = {k: m(k) for k in order}
    return (p[0] + p[3] - p[4] + p[6], p[2] + p[4], p[1] + p[3], p[0] - p[1] + p[2] + p[5])


def _kernel(ax, akt, avt, awq, awo, bx, bkt, bvt, bwq, bwo, out,
            xbuf, xc, x4, kvbuf, rq, ro, rq0, ro0,
            wqc0, wq40, woc0, wo40, wqc1, wq41, woc1, wo41,
            acc, obuf, pbuf, qbuf, oc, oraw, zref,
            xsem, kvsem, rqsem, rosem, isem, osem,
            *, scale, d, sq, nbatch, npass, dh):
    ng = nbatch // 2
    gw = 4 * dh
    hw = 2 * dh
    qr, q4r, orr = 256 // ng, 128 // ng, hw // ng
    xs, wqs, wos = (ax, bx), (awq, bwq), (awo, bwo)
    kvs = (akt, avt, bkt, bvt)
    wsets = ((wqc0, wq40, woc0, wo40), (wqc1, wq41, woc1, wo41))

    def kv_start(pp, gg, slot):
        for t in range(4):
            pltpu.make_async_copy(kvs[t].at[pl.ds(gg * 2, 2), pl.ds(4 * pp, 4)],
                                  kvbuf.at[slot, t], kvsem.at[slot]).start()

    def raw_start(pp, gg, slot):
        col = pl.multiple_of(pp * gw, 128)
        for j in range(2):
            for t in range(5):
                pltpu.make_async_copy(wqs[j].at[t, pl.ds(pl.multiple_of(gg * q4r, 16), q4r), pl.ds(col, gw)],
                                      rq.at[slot, j, t], rqsem.at[slot]).start()
            pltpu.make_async_copy(wos[j].at[pp, :, pl.ds(pl.multiple_of(gg * q4r, 16), q4r)],
                                  ro.at[slot, j], rosem.at[slot]).start()

    def wait_all(ref, sem):
        pltpu.make_async_copy(ref, ref, sem).wait()

    def x_start(gg):
        for j in range(2):
            pltpu.make_async_copy(xs[j].at[pl.ds(gg * 2, 2)], xbuf.at[gg, j], xsem.at[gg]).start()

    def out_copy(b):
        return pltpu.make_async_copy(obuf.at[b], out.at[b], osem)

    def build_x1(gg):
        for j in range(2):
            for r in range(0, sq, 32):
                x0 = xbuf.at[gg, j, 0][r:r + 32, :].astype(f32)
                x1 = xbuf.at[gg, j, 1][r:r + 32, :].astype(f32)
                rows = slice(r // 2, r // 2 + 16)
                cs = _lhs_combos(x0[:, :256], x0[:, 256:512], x1[:, :256], x1[:, 256:512])
                for k, c in enumerate(cs):
                    xc.at[gg, j, k][rows, :] = _pack(c)
                x4.at[gg, j][rows, :128] = _pack(x0[:, 512:])
                x4.at[gg, j][rows, 128:] = _pack(x1[:, 512:])

    def build_x2(gg):
        hs = sq // 2
        for j in range(2):
            for r in range(0, hs, 16):
                l1 = []
                for h in range(2):
                    x0 = xbuf.at[gg, j, 0][h * hs + r:h * hs + r + 16, :].astype(f32)
                    x1 = xbuf.at[gg, j, 1][h * hs + r:h * hs + r + 16, :].astype(f32)
                    l1.append(_lhs_combos(x0[:, :256], x0[:, 256:512], x1[:, :256], x1[:, 256:512]))
                    rows4 = slice((h * hs + r) // 2, (h * hs + r) // 2 + 8)
                    x4.at[gg, j][rows4, :] = _pack(jnp.concatenate([x0[:, 512:], x1[:, 512:]], axis=1))
                for k in range(7):
                    a11, a12, a21, a22 = (_col(l1[h][k], t) for h in range(2) for t in range(2))
                    blocks = _lhs_combos(a11, a12, a21, a22) + (a12, a21)
                    xc.at[gg, j, k][r // 2:r // 2 + 8, :] = _pack(jnp.concatenate(blocks, axis=1))

    build_x = build_x2 if Q2 else build_x1

    def build_wq(j, gg, raw, wset):
        wqc, wq4, _, _ = wset
        kt = [raw(t).astype(f32) for t in range(5)]
        l1 = [_rhs_combos(kt[t][:, :hw], kt[t][:, hw:], kt[2 + t][:, :hw], kt[2 + t][:, hw:]) for t in range(2)]
        rows = pl.ds(pl.multiple_of(gg * (q4r // 2), 8), q4r // 2)
        back = []
        for k in range(7):
            b = [[_col(l1[t][k], n) for n in range(3)] for t in range(2)]
            if k == 5 or not Q2:
                tiles = b[0] + b[1]
            else:
                tiles = list(_rhs_combos(b[0][0], b[0][1], b[1][0], b[1][1])) + [b[0][2], b[1][2]]
            cols = slice(0, 128 * len(tiles))
            wqc.at[j, k][rows, cols] = _pack(jnp.concatenate(tiles, axis=1))
            back.append(wqc.at[j, k][rows, cols])
        wq4.at[j][rows, :] = _pack(kt[4])
        return back + [wq4.at[j][rows, :]]

    def build_wo(j, gg, raw, wset):
        _, _, woc, wo4 = wset
        kt = [raw(t).astype(f32) for t in range(6)]
        l1 = [_rhs_combos(kt[3 + t][:, :256], kt[3 + t][:, 256:512], kt[t][:, :256], kt[t][:, 256:512])
              for t in range(3)]
        rows = pl.ds(pl.multiple_of(gg * (q4r // 2), 8), q4r // 2)
        back = []
        for k in range(7):
            b = [[_col(l1[t][k], n) for n in range(2)] for t in range(3)]
            if k == 2:
                tiles = [b[t][n] for n in range(2) for t in range(3)]
            else:
                tiles = list(_rhs_combos(b[0][0], b[0][1], b[1][0], b[1][1])) + b[2]
            cols = slice(0, 128 * len(tiles))
            woc.at[j, k][rows, cols] = _pack(jnp.concatenate(tiles, axis=1))
            back.append(woc.at[j, k][rows, cols])
        wo4.at[j][rows, :] = _pack(jnp.concatenate([x[:, 512:] for x in kt], axis=1))
        return back + [wo4.at[j][rows, :]]

    zref[0] = 0
    x_start(0)
    for j in range(2):
        pltpu.make_async_copy(wqs[j].at[:, :, pl.ds(0, gw)], rq0.at[j], isem.at[0]).start()
        pltpu.make_async_copy(wos[j].at[0], ro0.at[j], isem.at[1]).start()
    wait_all(xbuf.at[0], xsem.at[0])
    kv_start(0, 0, 0)
    raw_start(1, 0, 0)
    build_x(0)
    wait_all(rq0, isem.at[0])
    wait_all(ro0, isem.at[1])

    def init_body(gg, carry):
        for j in range(2):
            qrows = pl.ds(pl.multiple_of(gg * q4r, 16), q4r)
            build_wq(j, gg, lambda t: rq0.at[j, t][qrows, :], wsets[0])
            build_wo(j, gg, lambda t: ro0.at[j, t][qrows, :], wsets[0])
        return carry

    jax.lax.fori_loop(0, ng, init_body, 0)

    def step_body(p, g, par):
        cur, nxt = wsets[par], wsets[1 - par]
        wqc, wq4, woc, wo4 = cur
        slot = g % 2
        first = p == 0
        last = p == 2 * NPP - (2 if ONE else 1)

        if par == 0:
            @pl.when(jnp.logical_and(first, g > 0))
            def _():
                wait_all(xbuf.at[g], xsem.at[g])
                if not NOBX:
                    build_x(g)

        if NODMA:
            @pl.when(jnp.logical_and(first, g < 2))
            def _():
                wait_all(kvbuf.at[slot], kvsem.at[slot])
        else:
            wait_all(kvbuf.at[slot], kvsem.at[slot])
        wait_all(rq.at[slot], rqsem.at[slot])
        wait_all(ro.at[slot], rosem.at[slot])
        gn = jnp.where(g + 1 < ng, g + 1, 0)
        pn = jnp.where(g + 1 < ng, p, jnp.minimum(p + 1, npass - 1))
        if NODMA:
            @pl.when(jnp.logical_and(first, g < 1))
            def _():
                kv_start(pn, gn, 1 - slot)
        else:
            kv_start(pn, gn, 1 - slot)
        raw_start(jnp.minimum(pn + 1, npass - 1), gn, 1 - slot)

        if par == 0:
            @pl.when(jnp.logical_and(first, g + 1 < ng))
            def _():
                x_start(gn)

        s, qm, om, toks = {}, {}, {}, []
        zero = jnp.full((8, 128), zref[0], i32)

        def lhs(x):
            if toks:
                t = toks.pop(0)
                x = jnp.concatenate([x[:8] | jnp.concatenate([t & zero] * (x.shape[1] // 128), axis=1), x[8:]], axis=0)
            return _unpack(x)

        def token(vals):
            t = None
            for v in vals:
                for r in range(0, v.shape[0], 8):
                    for c in range(0, v.shape[1], 128):
                        x = v[r:r + 8, c:c + 128]
                        t = x if t is None else t | x
            return t

        def xblk(j, k, t):
            return xc.at[g, j, k][:, 128 * t:128 * (t + 1)]

        def wblk(j, k, t):
            return _unpack(wqc.at[j, k][:, 128 * t:128 * (t + 1)])

        def xfull(j, k, kt):
            return jnp.concatenate([xblk(j, k, (2, 7)[kt]), xblk(j, k, (8, 3)[kt])], axis=0)

        def qh(j, k, ms):
            for t in ms:
                qm[j, k, 'h', t] = _dot(lhs(xblk(j, k, t)), wblk(j, k, t))
            if all((j, k, 'h', t) in qm for t in range(7)):
                m = lambda t: qm[j, k, 'h', t]
                qm[j, k, 0] = jnp.concatenate([m(0) + m(3) - m(4) + m(6), m(1) + m(3)], axis=0)
                qm[j, k, 1] = jnp.concatenate([m(2) + m(4), (m(0) - m(1)) + (m(2) + m(5))], axis=0)

        def qM(j, k, n):
            w = (n, 3 + n) if k == 5 or not Q2 else (7, 8)
            xf = xfull if Q2 else xblk
            qm[j, k, n] = (_dot(lhs(xf(j, k, 0)), wblk(j, k, w[0]))
                           + _dot(lhs(xf(j, k, 1)), wblk(j, k, w[1])))

        def qK(j, u, n, half=None):
            col = (u % 2) * hw + 128 * n
            x = x4.at[g, j][:, 128 * (u // 2):128 * (u // 2 + 1)]
            w = _unpack(wq4[j, :, col:col + 128])
            if half is None:
                qm[j, 'k', u, n] = _dot(lhs(x), w)
            else:
                hq = sq // 4
                qm[j, 'k', u, n, half] = _dot(lhs(x[half * hq:(half + 1) * hq]), w)
                if half == 1:
                    qm[j, 'k', u, n] = jnp.concatenate([qm[j, 'k', u, n, h] for h in range(2)], axis=0)

        def qfin(j, u):
            for n in range(3):
                m = lambda k: qm[j, k, n]
                c = (lambda: (m(0) + qm[j, 'k', 0, n]) + m(6) + (m(3) - m(4)),
                     lambda: m(2) + m(4) + qm[j, 'k', 1, n],
                     lambda: m(1) + m(3) + qm[j, 'k', 2, n],
                     lambda: (m(0) + qm[j, 'k', 3, n]) + m(5) + (m(2) - m(1)))[u]()
                y = c * scale
                qbuf.at[j, u][:, 128 * n:128 * (n + 1)] = _pack(y)
                if n == 1:
                    qbuf.at[j, u][:, 384:] = _pack(pltpu.roll(y, 64, 1))

        def qp1(j, part):
            if part == 0:
                for n in range(3):
                    qM(j, 2, n), qM(j, 4, n)
                if j == 0:
                    qK(0, 1, 0), qK(0, 1, 1), qK(0, 1, 2), qK(0, 2, 0)
                else:
                    qK(1, 1, 2), qK(1, 2, 0), qK(1, 2, 1), qK(1, 2, 2)
                qfin(j, 1)
            elif part == 1:
                for n in range(3):
                    qM(j, 1, n), qM(j, 3, n)
                if j == 0:
                    qK(0, 2, 1), qK(0, 2, 2), qK(1, 1, 0), qK(1, 1, 1)
                qfin(j, 2)
            elif part == 2:
                for n in range(3):
                    qM(j, 0, n), qK(j, 0, n), qK(j, 3, n)
            else:
                for n in range(3):
                    qM(j, 6, n), qM(j, 5, n)
                qfin(j, 0)
                qfin(j, 3)

        def qp2(j, part):
            r1, r2 = (0, 3, 4, 6), (1, 2, 5)
            if part < 2:
                ka, kb = ((2, 4), (1, 3))[part]
                ks = (((0, 1, 0), (0, 1, 1), (0, 1, 2)), ((0, 2, 0), (0, 2, 1), (0, 2, 2)),
                      ((1, 1, 1), (1, 1, 2), (1, 2, 0)), ((1, 2, 1), (1, 2, 2), (1, 0, 0)))[2 * j + part]
                qh(j, ka, r1), qh(j, ka, r2), qK(*ks[0], 0)
                qh(j, kb, r1), qh(j, kb, r2), qK(*ks[0], 1)
                qK(*ks[1], 0), qK(*ks[1], 1), qK(*ks[2], 0), qK(*ks[2], 1)
                qM(j, ka, 2), qM(j, kb, 2)
                qfin(j, 1 + part)
            elif part == 2:
                x = (1, 1, 0) if j == 0 else (1, 0, 1)
                qh(j, 0, r1), qh(j, 0, r2), qK(*x, 0)
                qh(j, 6, r1), qh(j, 6, r2), qK(*x, 1)
                qM(j, 0, 2), qM(j, 6, 2)
            else:
                if j == 0:
                    qM(j, 5, 0), qK(j, 0, 0), qK(j, 3, 0)
                    qM(j, 5, 1), qK(j, 0, 1), qK(j, 3, 1)
                    qM(j, 5, 2), qK(j, 0, 2), qK(j, 3, 2)
                else:
                    qM(j, 5, 0), qK(j, 3, 0), qK(j, 0, 2)
                    qM(j, 5, 1), qM(j, 5, 2)
                    qK(j, 3, 1, 0), qK(j, 3, 1, 1), qK(j, 3, 2, 0), qK(j, 3, 2, 1)
                qfin(j, 0)
                qfin(j, 3)

        qp = qp2 if Q2 else qp1

        def sc(j, u):
            i, t = u // 2, u % 2
            s[j, u] = _scores(_q_operands(qbuf.at[j, u], lhs),
                              kvbuf[slot, 2 * j, i, 2 * t], kvbuf[slot, 2 * j, i, 2 * t + 1])

        def pslot(j, u):
            return pbuf.at[(4 * j + (1, 2, 0, 3).index(u)) % NPS]

        def sm(j, u):
            p_ref = pslot(j, u)
            ls = _softmax_terms(s[j, u], (p_ref.at[0], p_ref.at[1]), zero)
            if RMIX:
                lo = _lane_lo(CH)
                ls = {c: _recip(jnp.where(lo, ls[0, c], ls[1, c])) for c in range(sq // CH)}
            if RGATE:
                toks.append(token([pltpu.bitcast(v, i32) for v in ls.values()]))
            s[j, u] = ls

        def pv(j, u):
            i, t = u // 2, u % 2
            if not isinstance(s[j, u], dict):
                sm(j, u)

            def sink(c, *o):
                hq = sq // 4
                rows = [slice(h * hq + c * CH // 2, h * hq + (c + 1) * CH // 2) for h in range(2)]
                prev = lambda v: [_unpack(oraw.at[j, v][rows[h], :]).astype(f32) for h in range(2)]
                add = lambda x, y: [x[h] + y[h] for h in range(2)]
                sub = lambda x, y: [x[h] - y[h] for h in range(2)]
                for h in range(2):
                    oraw.at[j, u][rows[h], :] = _pack(o[h])
                new = {1: lambda: {},
                       2: lambda: {3: o, 0: add(prev(1), o)},
                       0: lambda: {4: add(prev(1), o), 6: sub(o, prev(2))},
                       3: lambda: {1: add(o, prev(2)), 5: sub(o, prev(1))}}[u]()
                for k, v in new.items():
                    cs = _lhs_combos(_col(v[0], 0), _col(v[0], 1), _col(v[1], 0), _col(v[1], 1))
                    blocks = [cs[t] for t in (0, 1, 4, 5, 6)]
                    if k != 3:
                        blocks += [cs[2], cs[3], _col(v[0], 2), _col(v[1], 2)]
                    oc.at[j, k][rows[0], :128 * len(blocks)] = _pack(jnp.concatenate(blocks, axis=1))

            _attend(s.pop((j, u)), kvbuf[slot, 2 * j + 1, i, 2 * t], kvbuf[slot, 2 * j + 1, i, 2 * t + 1],
                    pslot(j, u), sink, lhs)

        def emit(j, i, col, y):
            b = 2 * g + i
            cols = slice(j * d + col, j * d + col + 128)
            prev = acc[b, :, cols]
            y = y + (jnp.where(first, 0.0, prev) if par == 0 else prev)
            acc[b, :, cols] = y
            if par == 1 or ONE:
                obuf[b, :, cols] = y.astype(bf16)

        def oblk(j, k, t):
            hq = sq // 4
            if k == 3 and t in (2, 3, 7, 8):
                h, kt = {2: (0, 0), 3: (1, 1), 7: (0, 2), 8: (1, 2)}[t]
                return oraw.at[j, 2][h * hq:(h + 1) * hq, 128 * kt:128 * (kt + 1)]
            pos = (0, 1, 4, 5, 6, 2, 3, 7, 8).index(t)
            return oc.at[j, k][:, 128 * pos:128 * (pos + 1)]

        def owt(j, k, t):
            return _unpack(woc.at[j, k][:, 128 * t:128 * (t + 1)])

        def oM(j, k):
            mm = lambda t: _dot(lhs(oblk(j, k, t)), owt(j, k, t))
            kk = lambda h, n: _dot(lhs(oblk(j, k, 7 + h)), owt(j, k, 7 + n))
            m2, m4, k01, m0 = mm(2), mm(4), kk(0, 1), mm(0)
            m1, m3, k10, m6 = mm(1), mm(3), kk(1, 0), mm(6)
            k00, m5, k11 = kk(0, 0), mm(5), kk(1, 1)
            om[j, k, 0] = jnp.concatenate([((m0 - m4) + (m3 + m6)) + k00, m1 + m3 + k10], axis=0)
            om[j, k, 1] = jnp.concatenate([m2 + m4 + k01, ((m0 + m2) - m1) + (m5 + k11)], axis=0)

        def oN(j, i, tiles, half=None):
            hq = sq // 4
            for t in tiles:
                x = oraw.at[j, 2 * i + t // 3][:, 128 * (t % 3):128 * (t % 3 + 1)]
                w = _unpack(wo4.at[j][:, 128 * t:128 * (t + 1)])
                for h in (range(2) if half is None else (half,)):
                    key = (j, 'n', i, h)
                    if half is None:
                        if h == 0:
                            y = _dot(lhs(x), w)
                        yh = y[h * 2 * hq:(h + 1) * 2 * hq]
                    else:
                        yh = _dot(lhs(x[h * hq:(h + 1) * hq]), w)
                    om[key] = om[key] + yh if key in om else yh

        def emit_n(j, i):
            emit(j, i, 512, jnp.concatenate([om[j, 'n', i, h] for h in range(2)], axis=0))

        def op(j, part):
            m = lambda k, c: om[j, k, c]
            if part == 0:
                for c in range(2):
                    om[j, 2, c] = _dot(lhs(oraw[j, 1]),
                                       jnp.concatenate([owt(j, 2, 3 * c + t) for t in range(3)], axis=0))
                oN(j, 0, (3, 4))
                return
            ka, kb = ((0, 3), (4, 6), (1, 5))[part - 1]
            oM(j, ka), oN(j, 1, (part - 1,), 0)
            oM(j, kb), oN(j, 1, (part - 1,), 1)
            if part == 2:
                for c in range(2):
                    emit(j, 0, 256 + 128 * c, m(2, c) + m(4, c))
                    emit(j, 0, 128 * c, (m(0, c) + m(3, c) - m(4, c)) + m(6, c))
                oN(j, 0, (5, 0, 1, 2))
                emit_n(j, 0)
            elif part == 3:
                for c in range(2):
                    emit(j, 1, 128 * c, m(1, c) + m(3, c))
                    emit(j, 1, 256 + 128 * c, (m(0, c) + m(2, c) - m(1, c)) + m(5, c))
                if j == 0:
                    for t in (3, 4):
                        oN(0, 1, (t,), 0), oN(0, 1, (t,), 1)
                else:
                    oN(0, 1, (5,))
                    emit_n(0, 1)
                    oN(1, 1, (3, 4, 5))
                    emit_n(1, 1)

        def build(k):
            j = k // 2
            back = (build_wq(j, g, lambda t: rq[slot, j, t], nxt) if k % 2 == 0
                    else build_wo(j, g, lambda h: ro[slot, j, h], nxt))
            toks.append(token(back))

        seq = SEQS[ORD]
        for tok in seq.split():
            kind, a = tok[0], [int(ch) for ch in tok[1:]]
            {'q': qp, 's': sc, 'p': pv, 'o': op, 'w': build, 'x': sm}[kind](*a)

        if par == 1 or ONE:
            @pl.when(last)
            def _():
                out_copy(2 * g).start()
                out_copy(2 * g + 1).start()

    def pass_pair(pp, carry):
        for par in range(1 if ONE else 2):
            p = 2 * pp + par

            def group_body(g, carry, p=p, par=par):
                step_body(p, g, par)
                return carry

            carry = jax.lax.fori_loop(0, ng, group_body, carry)
        return carry

    jax.lax.fori_loop(0, NPP, pass_pair, 0)

    if ONE:
        z = zref[0]
        k = pbuf[z, z, 0:8, 0:128] | qbuf[z, z, 0:8, 0:128] | oc[z, z, 0:8, 0:128] | oraw[z, z, 0:8, 0:128]
        k = k | wqc1[z, z, 0:8, 0:128] | wq41[z, 0:8, 0:128] | woc1[z, z, 0:8, 0:128] | wo41[z, 0:8, 0:128]
        obuf[0, 0:8, 0:128] = pltpu.bitcast(k, f32).astype(bf16)
    if not NODMA:
        wait_all(kvbuf.at[0], kvsem.at[0])
    wait_all(rq.at[0], rqsem.at[0])
    wait_all(ro.at[0], rosem.at[0])
    if NPP:
        wait_all(obuf, osem)


@jax.jit
def pallas_concat_heads__gqa_block_cached__mha_block_cached__near_ridge_kernel(
    A_x, A_k_cache, A_v_cache, A_wq, A_wo, B_x, B_k_cache, B_v_cache, B_wq, B_wo,
):
    B, Sq, D = A_x.shape
    _, H, Sk, Dh = A_k_cache.shape
    npass = H // 4
    ng = B // 2
    scale = (Dh ** -0.5) * math.log2(math.e)
    gw, hw = 4 * Dh, 2 * Dh

    akt, avt, bkt, bvt = (jnp.swapaxes(t, 2, 3) for t in
                          (A_k_cache, A_v_cache, B_k_cache, B_v_cache))
    awq, bwq = (w.reshape(5, 128, H * Dh) for w in (A_wq, B_wq))
    awo, bwo = (w.reshape(npass, 6, 128, D) for w in (A_wo, B_wo))
    any_spec = pl.BlockSpec(memory_space=pl.ANY)
    wset = [
        pltpu.VMEM((2, 7, 64, 9 * 128), i32),
        pltpu.VMEM((2, 64, gw), i32),
        pltpu.VMEM((2, 7, 64, 9 * 128), i32),
        pltpu.VMEM((2, 64, 6 * 128), i32),
    ]

    return pl.pallas_call(
        functools.partial(_kernel, scale=scale, d=D, sq=Sq,
                          nbatch=B, npass=npass, dh=Dh),
        in_specs=[any_spec] * 10,
        out_specs=any_spec,
        out_shape=jax.ShapeDtypeStruct((B, Sq, 2 * D), A_x.dtype),
        scratch_shapes=[
            pltpu.VMEM((ng, 2, 2, Sq, D), bf16),
            pltpu.VMEM((ng, 2, 7, Sq // 4, 9 * 128) if Q2 else (ng, 2, 7, Sq // 2, 256), i32),
            pltpu.VMEM((ng, 2, Sq // 2, 256), i32),
            pltpu.VMEM((2, 4, 2, 4, Dh, Sk), bf16),
            pltpu.VMEM((2, 2, 5, 128 // ng, gw), bf16),
            pltpu.VMEM((2, 2, 6, 128 // ng, D), bf16),
            pltpu.VMEM((2, 5, 128, gw), bf16),
            pltpu.VMEM((2, 6, 128, D), bf16),
            *wset, *wset,
            pltpu.VMEM((B, Sq, 2 * D), f32),
            pltpu.VMEM((B, Sq, 2 * D), bf16),
            pltpu.VMEM((NPS, 2, Sq // 2, 768), i32),
            pltpu.VMEM((2, 4, Sq // 2, 512), i32),
            pltpu.VMEM((2, 7, Sq // 4, 9 * 128), i32),
            pltpu.VMEM((2, 4, Sq // 2, hw), i32),
            pltpu.SMEM((1,), i32),
            pltpu.SemaphoreType.DMA((ng,)),
            pltpu.SemaphoreType.DMA((2,)),
            pltpu.SemaphoreType.DMA((2,)),
            pltpu.SemaphoreType.DMA((2,)),
            pltpu.SemaphoreType.DMA((2,)),
            pltpu.SemaphoreType.DMA(()),
        ],
        compiler_params=pltpu.CompilerParams(
            vmem_limit_bytes=110 * 1024 * 1024,
            disable_bounds_checks=True,
        ),
    )(A_x, akt, avt, awq, awo, B_x, bkt, bvt, bwq, bwo)
```

```python
import functools
import math

import jax
import jax.numpy as jnp
import jax.experimental.pallas as pl
import jax.experimental.pallas.tpu as pltpu

_NN = (((1,), (0,)), ((), ()))
_NT = (((1,), (1,)), ((), ()))
bf16 = jnp.bfloat16
f32 = jnp.float32
i32 = jnp.int32

CH = 16
DEP = 3
NKV = 3
NPS = 4

_SEQ_FULL = ('q00 w0 q01 s01 q02 w2 q10 w1 p01 s02 q03 w3 p02 s00 p00 q11 s03 o01 '
             'q12 p03 s11 o00 p11 q13 o02 s12 o03 s10 p12 o10 s13 p10 o11 p13 o12 o13')
_SEQ_NOQ = ('s01 s02 w0 p01 s00 w1 p02 o00 s03 p00 o01 s11 w2 p03 o02 s12 p11 o03 '
            's10 w3 p12 o10 s13 p10 o11 p13 o12 o13')
_SEQ_Q = 'q00 q01 q02 q03 q10 q11 q12 q13'


def _dot(a, b, dims=_NN):
    return jax.lax.dot_general(a, b, dims, preferred_element_type=f32)


def _recip(l):
    r = pl.reciprocal(l, approx=True)
    return r * (2.0 - l * r)


def _col(x, i):
    return x[:, 128 * i:128 * (i + 1)]


def _pack(x):
    return pltpu.bitcast(x.astype(bf16), i32)


def _unpack(x):
    return pltpu.bitcast(x, bf16)


def _cat(xs, axis):
    return jnp.concatenate(list(xs), axis=axis)


def _or_tiles(vals):
    t = None
    for v in vals:
        for r in range(0, v.shape[0], 8):
            for c in range(0, v.shape[1], 128):
                x = v[r:r + 8, c:c + 128]
                t = x if t is None else t | x
    return t


def _lane_lo(rows):
    return jax.lax.broadcasted_iota(i32, (rows, 128), 1) < 64


def _lhs_combos(a11, a12, a21, a22):
    return (a11 + a22, a21 + a22, a11, a22, a11 + a12, a21 - a11, a12 - a22)


def _rhs_combos(b11, b12, b21, b22):
    return (b11 + b22, b11, b12 - b22, b21 - b11, b22, b11 + b12, b21 + b22)


def _weights(xa, xb, xc):
    h = xa.shape[1] // 2
    xa, xb, xc = xa.astype(f32), xb.astype(f32), xc.astype(f32)
    return (_cat([xa[:, :h], xb[:, :h] - xb[:, h:]], 0),
            _cat([xa[:, h:], xc[:, h:] - xc[:, :h]], 0),
            _cat([xc[:, :h], xb[:, h:]], 0))


def _pair_weights(t0, t1):
    return (_weights(t0[:64], t0[64:128], t0[128:]), _weights(t1[64:128], t1[128:], t1[:64]))


def _scores(q_ref, kt0, kt1, lhs):
    t0, t1, t2, rot = (q_ref[:, 128 * k:128 * (k + 1)] for k in range(4))
    lo = _lane_lo(t0.shape[0])
    q = ((t0, jnp.where(lo, t0, rot), jnp.where(lo, t1, t0)),
         (t2, jnp.where(lo, t2, t1), jnp.where(lo, rot, t2)))
    w = _pair_weights(kt0, kt1)
    p = {}

    def run(h, k, i):
        p[h, k, i] = _dot(lhs(q[h][k]), _col(w[h][k], i).astype(bf16))

    for t, (h, i) in enumerate(((0, 0), (0, 1), (1, 0))):
        run(h, 2, i), run(h, 0, i), run(h, 1, i), run(1, (2, 0, 1)[t], 1)
    return tuple(_cat([p[h, 0, 0] + p[h, 2, 0], p[h, 0, 1] + p[h, 2, 1],
                       p[h, 1, 0] + p[h, 2, 0], p[h, 1, 1] + p[h, 2, 1]], 1) for h in range(2))


def _softmax_terms(s, p_ref, zero):
    ls, toks = [], []
    for c in range(s.shape[0] // CH):
        sc = s[c * CH:(c + 1) * CH]
        m = jnp.broadcast_to(jnp.max(sc, axis=-1, keepdims=True), (CH, 128))
        if c >= DEP:
            t = toks[c - DEP] & zero
            m = pltpu.bitcast(pltpu.bitcast(m, i32) | _cat([t, t], 0), f32)
        e = [jnp.exp2(_col(sc, k) - m) for k in range(4)]
        t0, t1 = e[0] + e[2], e[1] + e[3]
        ls.append(jnp.broadcast_to(jnp.sum(t0 + t1, axis=-1, keepdims=True), (CH, 128)))
        rows = slice(c * CH // 2, (c + 1) * CH // 2)
        for k, x in enumerate(e + [t0, t1]):
            p_ref[rows, 128 * k:128 * (k + 1)] = _pack(x)
        toks.append(_or_tiles([p_ref[rows, :]]))
    return ls


def _attend(s, vt0, vt1, p_ref, zero, lhs, sink):
    ls = [_softmax_terms(s[h], p_ref.at[h], zero) for h in range(2)]
    w = _pair_weights(vt0, vt1)
    r = {}
    for h, k in ((0, 1), (0, 2), (1, 1), (1, 2), (0, 0), (1, 0)):
        r[h, k] = _dot(lhs(p_ref.at[h][:, 256 * k:256 * (k + 1)]), w[h][k].astype(bf16), _NT)
    lo = _lane_lo(CH)

    def rows(c):
        p1, p2, p3, u1, u2, u3 = (r[h, k][c * CH:(c + 1) * CH] for h in range(2) for k in range(3))
        r0, r1 = _recip(ls[0][c]), _recip(ls[1][c])
        o_lo = p1 + jnp.where(lo, p2, p3)
        o_hi = u1 + jnp.where(lo, u2, u3)
        mid = jnp.where(lo, p3, u2) + pltpu.roll(jnp.where(lo, u3, p2), 64, 1)
        return _cat([o_lo * r0, mid * jnp.where(lo, r0, r1), o_hi * r1], 1)

    n = len(ls[0]) // 2
    for c in range(n):
        sink(c, rows(c), rows(c + n))


def _kernel(ax, akt, avt, awq, awo, bx, bkt, bvt, bwq, bwo, out,
            xbuf, xc, x4, kvbuf, rq, ro, rq0, ro0,
            wqc0, wq40, woc0, wo40, wqc1, wq41, woc1, wo41,
            acc, obuf, pbuf, qbuf, qall, oc, oraw, zref,
            xsem, kvsem, rqsem, rosem, isem, osem,
            *, scale, d, sq, nbatch, npass, dh):
    ng = nbatch // 2
    nsteps = npass * ng
    gw, hw = 4 * dh, 2 * dh
    wr = 128 // ng
    hq = sq // 4
    xs, wqs, wos = (ax, bx), (awq, bwq), (awo, bwo)
    kvs = (akt, avt, bkt, bvt)
    wsets = ((wqc0, wq40, woc0, wo40), (wqc1, wq41, woc1, wo41))

    def wait_all(ref, sem):
        pltpu.make_async_copy(ref, ref, sem).wait()

    def fetch(pp, gg, slot):
        for t in range(4):
            pltpu.make_async_copy(kvs[t].at[pl.ds(gg * 2, 2), pl.ds(4 * pp, 4)],
                                  kvbuf.at[slot, t], kvsem.at[slot]).start()
        pw = jnp.minimum(pp + 1, npass - 1)
        rows = pl.ds(pl.multiple_of(gg * wr, 16), wr)
        for j in range(2):
            for t in range(5):
                pltpu.make_async_copy(wqs[j].at[t, rows, pl.ds(pl.multiple_of(pw * gw, 128), gw)],
                                      rq.at[slot, j, t], rqsem.at[slot]).start()
            pltpu.make_async_copy(wos[j].at[pw, :, rows], ro.at[slot, j], rosem.at[slot]).start()

    def fetch_wait(slot):
        wait_all(kvbuf.at[slot], kvsem.at[slot])
        wait_all(rq.at[slot], rqsem.at[slot])
        wait_all(ro.at[slot], rosem.at[slot])

    def x_start(gg):
        for j in range(2):
            pltpu.make_async_copy(xs[j].at[pl.ds(gg * 2, 2)], xbuf.at[gg, j], xsem.at[gg]).start()

    def build_x(gg):
        for j in range(2):
            for r in range(0, sq, 32):
                x0 = xbuf.at[gg, j, 0][r:r + 32, :].astype(f32)
                x1 = xbuf.at[gg, j, 1][r:r + 32, :].astype(f32)
                rows = slice(r // 2, r // 2 + 16)
                cs = _lhs_combos(x0[:, :256], x0[:, 256:512], x1[:, :256], x1[:, 256:512])
                for k, c in enumerate(cs):
                    xc.at[gg, j, k][rows, :] = _pack(c)
                x4.at[gg, j][rows, :] = _pack(_cat([x0[:, 512:], x1[:, 512:]], 1))

    def build_wq(j, gg, raw, wset):
        wqc, wq4, _, _ = wset
        kt = [raw(t).astype(f32) for t in range(5)]
        l1 = [_rhs_combos(kt[t][:, :hw], kt[t][:, hw:], kt[2 + t][:, :hw], kt[2 + t][:, hw:])
              for t in range(2)]
        rows = pl.ds(pl.multiple_of(gg * (wr // 2), 8), wr // 2)
        for k in range(7):
            wqc.at[j, k][rows, :] = _pack(_cat([l1[0][k], l1[1][k]], 1))
        wq4.at[j][rows, :] = _pack(kt[4])
        return [wqc.at[j, k][rows, :] for k in range(7)] + [wq4.at[j][rows, :]]

    def build_wo(j, gg, raw, wset):
        _, _, woc, wo4 = wset
        kt = [raw(t).astype(f32) for t in range(6)]
        l1 = [_rhs_combos(kt[3 + t][:, :256], kt[3 + t][:, 256:512], kt[t][:, :256], kt[t][:, 256:512])
              for t in range(3)]
        rows = pl.ds(pl.multiple_of(gg * (wr // 2), 8), wr // 2)
        back = []
        for k in range(7):
            b = [[_col(l1[t][k], n) for n in range(2)] for t in range(3)]
            if k == 2:
                tiles = [b[t][n] for n in range(2) for t in range(3)]
            else:
                tiles = list(_rhs_combos(b[0][0], b[0][1], b[1][0], b[1][1])) + b[2]
            cols = slice(0, 128 * len(tiles))
            woc.at[j, k][rows, cols] = _pack(_cat(tiles, 1))
            back.append(woc.at[j, k][rows, cols])
        wo4.at[j][rows, :] = _pack(_cat([x[:, 512:] for x in kt], 1))
        return back + [wo4.at[j][rows, :]]

    def compute(seq, g, slot, par, q_ref, first, write_out):
        wqc, wq4, woc, wo4 = wsets[par]
        s, qm, om, toks = {}, {}, {}, []
        zero = jnp.full((8, 128), zref[0], i32)

        def lhs(x):
            if toks:
                t = toks.pop(0) & zero
                x = _cat([x[:8] | _cat([t] * (x.shape[1] // 128), 1), x[8:]], 0)
            return _unpack(x)

        def q_m(j, k, n):
            x, w = xc.at[g, j, k], wqc.at[j, k]
            qm[j, k, n] = (_dot(lhs(x[:, :128]), _unpack(w[:, 128 * n:128 * (n + 1)]))
                           + _dot(lhs(x[:, 128:]), _unpack(w[:, hw + 128 * n:hw + 128 * (n + 1)])))

        def q_k(j, u, n):
            col = (u % 2) * hw + 128 * n
            qm[j, 'k', u, n] = _dot(lhs(x4.at[g, j][:, 128 * (u // 2):128 * (u // 2 + 1)]),
                                    _unpack(wq4.at[j][:, col:col + 128]))

        def q_fin(j, u):
            for n in range(3):
                m = lambda k: qm[j, k, n]
                kk = qm[j, 'k', u, n]
                y = (lambda: (m(0) + kk) + m(6) + (m(3) - m(4)), lambda: m(2) + m(4) + kk,
                     lambda: m(1) + m(3) + kk, lambda: (m(0) + kk) + m(5) + (m(2) - m(1)))[u]()
                y = y * scale
                q_ref.at[j, u][:, 128 * n:128 * (n + 1)] = _pack(y)
                if n == 1:
                    q_ref.at[j, u][:, 384:] = _pack(pltpu.roll(y, 64, 1))

        def q_piece(j, part):
            if part < 2:
                for n in range(3):
                    q_m(j, (2, 1)[part], n), q_m(j, (4, 3)[part], n)
                for a in (((0, 1, 0), (0, 1, 1), (0, 1, 2), (0, 2, 0)),
                          ((0, 2, 1), (0, 2, 2), (1, 1, 0), (1, 1, 1)),
                          ((1, 1, 2), (1, 2, 0), (1, 2, 1), (1, 2, 2)), ())[2 * j + part]:
                    q_k(*a)
                q_fin(j, 1 + part)
            elif part == 2:
                for n in range(3):
                    q_m(j, 0, n), q_k(j, 0, n), q_k(j, 3, n)
            else:
                for n in range(3):
                    q_m(j, 6, n), q_m(j, 5, n)
                q_fin(j, 0)
                q_fin(j, 3)

        def kv(j, which, u):
            return tuple(kvbuf[slot, 2 * j + which, u // 2, 2 * (u % 2) + h] for h in range(2))

        def s_piece(j, u):
            s[j, u] = _scores(q_ref.at[j, u], *kv(j, 0, u), lhs)

        def p_piece(j, u):
            def sink(c, *o):
                rows = [slice(h * hq + c * CH // 2, h * hq + (c + 1) * CH // 2) for h in range(2)]
                prev = lambda v: [_unpack(oraw.at[j, v][rows[h], :]).astype(f32) for h in range(2)]
                add = lambda x, y: [x[h] + y[h] for h in range(2)]
                sub = lambda x, y: [x[h] - y[h] for h in range(2)]
                for h in range(2):
                    oraw.at[j, u][rows[h], :] = _pack(o[h])
                new = {1: lambda: {},
                       2: lambda: {3: o, 0: add(prev(1), o)},
                       0: lambda: {4: add(prev(1), o), 6: sub(o, prev(2))},
                       3: lambda: {1: add(o, prev(2)), 5: sub(o, prev(1))}}[u]()
                for k, v in new.items():
                    cs = _lhs_combos(_col(v[0], 0), _col(v[0], 1), _col(v[1], 0), _col(v[1], 1))
                    blocks = [cs[t] for t in (0, 1, 4, 5, 6)]
                    if k != 3:
                        blocks += [cs[2], cs[3], _col(v[0], 2), _col(v[1], 2)]
                    oc.at[j, k][rows[0], :128 * len(blocks)] = _pack(_cat(blocks, 1))

            _attend(s.pop((j, u)), *kv(j, 1, u), pbuf.at[(1, 2, 0, 3).index(u)], zero, lhs, sink)

        def emit(j, i, col, y):
            b = 2 * g + i
            cols = slice(j * d + col, j * d + col + 128)
            if not first:
                y = y + acc[b, :, cols]
            acc[b, :, cols] = y
            if write_out:
                obuf[b, :, cols] = y.astype(bf16)

        def o_w(j, k, t):
            return _unpack(woc.at[j, k][:, 128 * t:128 * (t + 1)])

        def o_m(j, k):
            def blk(t):
                if k == 3 and t in (2, 3, 7, 8):
                    h, kt = {2: (0, 0), 3: (1, 1), 7: (0, 2), 8: (1, 2)}[t]
                    return oraw.at[j, 2][h * hq:(h + 1) * hq, 128 * kt:128 * (kt + 1)]
                pos = (0, 1, 4, 5, 6, 2, 3, 7, 8).index(t)
                return oc.at[j, k][:, 128 * pos:128 * (pos + 1)]

            mm = lambda t: _dot(lhs(blk(t)), o_w(j, k, t))
            kk = lambda h, n: _dot(lhs(blk(7 + h)), o_w(j, k, 7 + n))
            m2, m4, k01, m0 = mm(2), mm(4), kk(0, 1), mm(0)
            m1, m3, k10, m6 = mm(1), mm(3), kk(1, 0), mm(6)
            k00, m5, k11 = kk(0, 0), mm(5), kk(1, 1)
            om[j, k, 0] = _cat([((m0 - m4) + (m3 + m6)) + k00, m1 + m3 + k10], 0)
            om[j, k, 1] = _cat([m2 + m4 + k01, ((m0 + m2) - m1) + (m5 + k11)], 0)

        def o_n(j, i, t, half=None):
            x = oraw.at[j, 2 * i + t // 3][:, 128 * (t % 3):128 * (t % 3 + 1)]
            w = _unpack(wo4.at[j][:, 128 * t:128 * (t + 1)])
            if half is None:
                y = _dot(lhs(x), w)
                parts = {h: y[h * 2 * hq:(h + 1) * 2 * hq] for h in range(2)}
            else:
                parts = {half: _dot(lhs(x[half * hq:(half + 1) * hq]), w)}
            for h, y in parts.items():
                om[j, 'n', i, h] = om[j, 'n', i, h] + y if (j, 'n', i, h) in om else y

        def emit_n(j, i):
            emit(j, i, 512, _cat([om[j, 'n', i, h] for h in range(2)], 0))

        def o_piece(j, part):
            m = lambda k, c: om[j, k, c]
            if part == 0:
                for c in range(2):
                    om[j, 2, c] = _dot(lhs(oraw[j, 1]), _cat([o_w(j, 2, 3 * c + t) for t in range(3)], 0))
                o_n(j, 0, 3), o_n(j, 0, 4)
                return
            ka, kb = ((0, 3), (4, 6), (1, 5))[part - 1]
            o_m(j, ka), o_n(j, 1, part - 1, 0)
            o_m(j, kb), o_n(j, 1, part - 1, 1)
            if part == 2:
                for c in range(2):
                    emit(j, 0, 256 + 128 * c, m(2, c) + m(4, c))
                    emit(j, 0, 128 * c, (m(0, c) + m(3, c) - m(4, c)) + m(6, c))
                for t in (5, 0, 1, 2):
                    o_n(j, 0, t)
                emit_n(j, 0)
            elif part == 3:
                for c in range(2):
                    emit(j, 1, 128 * c, m(1, c) + m(3, c))
                    emit(j, 1, 256 + 128 * c, (m(0, c) + m(2, c) - m(1, c)) + m(5, c))
                if j == 0:
                    for t in (3, 4):
                        o_n(0, 1, t, 0), o_n(0, 1, t, 1)
                else:
                    o_n(0, 1, 5)
                    emit_n(0, 1)
                    for t in (3, 4, 5):
                        o_n(1, 1, t)
                    emit_n(1, 1)

        def w_piece(k):
            j = k // 2
            back = (build_wq(j, g, lambda t: rq[slot, j, t], wsets[1 - par]) if k % 2 == 0
                    else build_wo(j, g, lambda t: ro[slot, j, t], wsets[1 - par]))
            toks.append(_or_tiles(back))

        run = {'q': q_piece, 's': s_piece, 'p': p_piece, 'o': o_piece, 'w': w_piece}
        for tok in seq.split():
            run[tok[0]](*(int(ch) for ch in tok[1:]))

    def run_pass(p, par, first, slot0):
        def step(g, slot):
            fetch_wait(slot)

            wrap = g + 2 >= ng
            fetch(jnp.minimum(jnp.where(wrap, p + 1, p), npass - 1),
                  jnp.where(wrap, g + 2 - ng, g + 2), jnp.where(slot == 0, NKV - 1, slot - 1))

            if first:
                compute(_SEQ_NOQ, g, slot, par, qall.at[g], True, False)
            else:
                compute(_SEQ_FULL, g, slot, par, qbuf, False, par == 1)
            if par == 1:
                @pl.when(p == npass - 1)
                def _():
                    for i in range(2):
                        pltpu.make_async_copy(obuf.at[2 * g + i], out.at[2 * g + i], osem).start()
            return jnp.where(slot == NKV - 1, 0, slot + 1)

        jax.lax.fori_loop(0, ng, step, slot0)

    def init_weights(build, raw):
        def body(gg, carry):
            rows = pl.ds(pl.multiple_of(gg * wr, 16), wr)
            for j in range(2):
                build(j, gg, lambda t: raw.at[j, t][rows, :], wsets[0])
            return carry

        jax.lax.fori_loop(0, ng, body, 0)

    zref[0] = 0
    x_start(0)
    for j in range(2):
        pltpu.make_async_copy(wqs[j].at[:, :, pl.ds(0, gw)], rq0.at[j], isem.at[0]).start()
    wait_all(xbuf.at[0], xsem.at[0])
    build_x(0)
    wait_all(rq0, isem.at[0])
    for gg in range(1, ng):
        x_start(gg)
    init_weights(build_wq, rq0)

    def q_step(g, carry):
        @pl.when(g == 1)
        def _():
            for j in range(2):
                pltpu.make_async_copy(wos[j].at[0], ro0.at[j], isem.at[1]).start()
            fetch(0, 0, 0)

        @pl.when(g == 4)
        def _():
            fetch(0, 1, 1)

        @pl.when(g > 0)
        def _():
            wait_all(xbuf.at[g], xsem.at[g])
            build_x(g)

        compute(_SEQ_Q, g, 0, 0, qall.at[g], True, False)
        return carry

    jax.lax.fori_loop(0, ng, q_step, 0)
    wait_all(ro0, isem.at[1])
    init_weights(build_wo, ro0)

    run_pass(0, 0, True, 0)

    def pass_pair(pp, carry):
        run_pass(2 * pp + 1, 1, False, ((2 * pp + 1) * ng) % NKV)

        @pl.when(2 * pp + 2 < npass)
        def _():
            run_pass(2 * pp + 2, 0, False, ((2 * pp + 2) * ng) % NKV)

        return carry

    jax.lax.fori_loop(0, npass // 2, pass_pair, 0)
    fetch_wait(nsteps % NKV)
    fetch_wait((nsteps + 1) % NKV)
    wait_all(out, osem)


@jax.jit
def pallas_concat_heads__gqa_block_cached__mha_block_cached__near_ridge_kernel(
    A_x: jax.Array,
    A_k_cache: jax.Array,
    A_v_cache: jax.Array,
    A_wq: jax.Array,
    A_wo: jax.Array,
    B_x: jax.Array,
    B_k_cache: jax.Array,
    B_v_cache: jax.Array,
    B_wq: jax.Array,
    B_wo: jax.Array,
):
    B, Sq, D = A_x.shape
    _, H, Sk, Dh = A_k_cache.shape
    assert (B, Sq, D, H, Sk, Dh) == (16, 160, 640, 32, 512, 192)
    npass, ng = H // 4, B // 2
    gw, hw = 4 * Dh, 2 * Dh
    scale = (Dh ** -0.5) * math.log2(math.e)

    akt, avt, bkt, bvt = (jnp.swapaxes(t, 2, 3) for t in
                          (A_k_cache, A_v_cache, B_k_cache, B_v_cache))
    awq, bwq = (w.reshape(5, 128, H * Dh) for w in (A_wq, B_wq))
    awo, bwo = (w.reshape(npass, 6, 128, D) for w in (A_wo, B_wo))
    any_spec = pl.BlockSpec(memory_space=pl.ANY)
    wset = [
        pltpu.VMEM((2, 7, 64, 2 * hw), i32),
        pltpu.VMEM((2, 64, gw), i32),
        pltpu.VMEM((2, 7, 64, 9 * 128), i32),
        pltpu.VMEM((2, 64, 6 * 128), i32),
    ]

    return pl.pallas_call(
        functools.partial(_kernel, scale=scale, d=D, sq=Sq, nbatch=B, npass=npass, dh=Dh),
        in_specs=[any_spec] * 10,
        out_specs=any_spec,
        out_shape=jax.ShapeDtypeStruct((B, Sq, 2 * D), A_x.dtype),
        scratch_shapes=[
            pltpu.VMEM((ng, 2, 2, Sq, D), bf16),
            pltpu.VMEM((ng, 2, 7, Sq // 2, 256), i32),
            pltpu.VMEM((ng, 2, Sq // 2, 256), i32),
            pltpu.VMEM((NKV, 4, 2, 4, Dh, Sk), bf16),
            pltpu.VMEM((NKV, 2, 5, 128 // ng, gw), bf16),
            pltpu.VMEM((NKV, 2, 6, 128 // ng, D), bf16),
            pltpu.VMEM((2, 5, 128, gw), bf16),
            pltpu.VMEM((2, 6, 128, D), bf16),
            *wset, *wset,
            pltpu.VMEM((B, Sq, 2 * D), f32),
            pltpu.VMEM((B, Sq, 2 * D), bf16),
            pltpu.VMEM((NPS, 2, Sq // 2, 768), i32),
            pltpu.VMEM((2, 4, Sq // 2, 512), i32),
            pltpu.VMEM((ng, 2, 4, Sq // 2, 512), i32),
            pltpu.VMEM((2, 7, Sq // 4, 9 * 128), i32),
            pltpu.VMEM((2, 4, Sq // 2, hw), i32),
            pltpu.SMEM((1,), i32),
            pltpu.SemaphoreType.DMA((ng,)),
            pltpu.SemaphoreType.DMA((NKV,)),
            pltpu.SemaphoreType.DMA((NKV,)),
            pltpu.SemaphoreType.DMA((NKV,)),
            pltpu.SemaphoreType.DMA((2,)),
            pltpu.SemaphoreType.DMA(()),
        ],
        compiler_params=pltpu.CompilerParams(
            vmem_limit_bytes=116 * 1024 * 1024,
            disable_bounds_checks=True,
        ),
    )(A_x, akt, avt, awq, awo, B_x, bkt, bvt, bwq, bwo)
```

```python
import functools
import math

import jax
import jax.numpy as jnp
import jax.experimental.pallas as pl
import jax.experimental.pallas.tpu as pltpu

_NN = (((1,), (0,)), ((), ()))
_NT = (((1,), (1,)), ((), ()))
bf16 = jnp.bfloat16
f32 = jnp.float32
i32 = jnp.int32

CH = 16
DEP = 3
NKV = 3
NPS = 4

_SEQ_FULL = ('q00 w0 q01 s01 q02 w2 q10 w1 p01 s02 q03 w3 p02 s00 p00 q11 s03 o01 '
             'q12 p03 s11 o00 p11 q13 o02 s12 o03 s10 p12 o10 s13 p10 o11 p13 o12 o13')
_SEQ_NOQ = ('s01 s02 p01 w1 w0 s00 p02 p00 s03 o01 w2 p03 s11 p11 o00 s12 o02 p12 '
            's10 o03 p10 o10 w3 s13 o11 p13 o12 o13')
_SEQ_Q = 'x1 r00 r01 q02 q03 r10 r11 x0 q12 q13'


def _dot(a, b, dims=_NN):
    return jax.lax.dot_general(a, b, dims, preferred_element_type=f32)


def _recip(l):
    r = pl.reciprocal(l, approx=True)
    return r * (2.0 - l * r)


def _col(x, i):
    return x[:, 128 * i:128 * (i + 1)]


def _pack(x):
    return pltpu.bitcast(x.astype(bf16), i32)


def _unpack(x):
    return pltpu.bitcast(x, bf16)


def _cat(xs, axis):
    return jnp.concatenate(list(xs), axis=axis)


def _or_tiles(vals):
    t = None
    for v in vals:
        for r in range(0, v.shape[0], 8):
            for c in range(0, v.shape[1], 128):
                x = v[r:r + 8, c:c + 128]
                t = x if t is None else t | x
    return t


def _lane_lo(rows):
    return jax.lax.broadcasted_iota(i32, (rows, 128), 1) < 64


def _lhs_combos(a11, a12, a21, a22):
    return (a11 + a22, a21 + a22, a11, a22, a11 + a12, a21 - a11, a12 - a22)


def _rhs_combos(b11, b12, b21, b22):
    return (b11 + b22, b11, b12 - b22, b21 - b11, b22, b11 + b12, b21 + b22)


def _weights(xa, xb, xc):
    h = xa.shape[1] // 2
    xa, xb, xc = xa.astype(f32), xb.astype(f32), xc.astype(f32)
    return (_cat([xa[:, :h], xb[:, :h] - xb[:, h:]], 0),
            _cat([xa[:, h:], xc[:, h:] - xc[:, :h]], 0),
            _cat([xc[:, :h], xb[:, h:]], 0))


def _pair_weights(t0, t1):
    return (_weights(t0[:64], t0[64:128], t0[128:]), _weights(t1[64:128], t1[128:], t1[:64]))


def _scores(q_ref, kt0, kt1, lhs):
    t0, t1, t2, rot = (q_ref[:, 128 * k:128 * (k + 1)] for k in range(4))
    lo = _lane_lo(t0.shape[0])
    q = ((t0, jnp.where(lo, t0, rot), jnp.where(lo, t1, t0)),
         (t2, jnp.where(lo, t2, t1), jnp.where(lo, rot, t2)))
    w = _pair_weights(kt0, kt1)
    p = {}

    def run(h, k, i):
        p[h, k, i] = _dot(lhs(q[h][k]), _col(w[h][k], i).astype(bf16))

    for t, (h, i) in enumerate(((0, 0), (0, 1), (1, 0))):
        run(h, 2, i), run(h, 0, i), run(h, 1, i), run(1, (2, 0, 1)[t], 1)
    return tuple(_cat([p[h, 0, 0] + p[h, 2, 0], p[h, 0, 1] + p[h, 2, 1],
                       p[h, 1, 0] + p[h, 2, 0], p[h, 1, 1] + p[h, 2, 1]], 1) for h in range(2))


def _softmax_terms(s, p_ref, zero):
    ls, toks = [], []
    for c in range(s.shape[0] // CH):
        sc = s[c * CH:(c + 1) * CH]
        m = jnp.broadcast_to(jnp.max(sc, axis=-1, keepdims=True), (CH, 128))
        if c >= DEP:
            t = toks[c - DEP] & zero
            m = pltpu.bitcast(pltpu.bitcast(m, i32) | _cat([t, t], 0), f32)
        e = [jnp.exp2(_col(sc, k) - m) for k in range(4)]
        t0, t1 = e[0] + e[2], e[1] + e[3]
        ls.append(jnp.broadcast_to(jnp.sum(t0 + t1, axis=-1, keepdims=True), (CH, 128)))
        rows = slice(c * CH // 2, (c + 1) * CH // 2)
        for k, x in enumerate(e + [t0, t1]):
            p_ref[rows, 128 * k:128 * (k + 1)] = _pack(x)
        toks.append(_or_tiles([p_ref[rows, :]]))
    return ls


def _attend(s, vt0, vt1, p_ref, zero, lhs, sink):
    ls = [_softmax_terms(s[h], p_ref.at[h], zero) for h in range(2)]
    w = _pair_weights(vt0, vt1)
    r = {}
    for h, k in ((0, 1), (0, 2), (1, 1), (1, 2), (0, 0), (1, 0)):
        r[h, k] = _dot(lhs(p_ref.at[h][:, 256 * k:256 * (k + 1)]), w[h][k].astype(bf16), _NT)
    lo = _lane_lo(CH)

    def rows(c):
        p1, p2, p3, u1, u2, u3 = (r[h, k][c * CH:(c + 1) * CH] for h in range(2) for k in range(3))
        r0, r1 = _recip(ls[0][c]), _recip(ls[1][c])
        o_lo = p1 + jnp.where(lo, p2, p3)
        o_hi = u1 + jnp.where(lo, u2, u3)
        mid = jnp.where(lo, p3, u2) + pltpu.roll(jnp.where(lo, u3, p2), 64, 1)
        return _cat([o_lo * r0, mid * jnp.where(lo, r0, r1), o_hi * r1], 1)

    n = len(ls[0]) // 2
    for c in range(n):
        sink(c, rows(c), rows(c + n))


def _kernel(ax, akt, avt, awq, awo, bx, bkt, bvt, bwq, bwo, out,
            xbuf, xca, xcb, x4a, x4b, kvbuf, rq, ro, rq0, ro0,
            wqc0, wq40, woc0, wo40, wqc1, wq41, woc1, wo41,
            acc, obuf, pbuf, qbuf, qall, oc, oraw, zref,
            xsem, kvsem, rqsem, rosem, isem, osem,
            *, scale, d, sq, nbatch, npass, dh):
    ng = nbatch // 2
    nsteps = npass * ng
    gw, hw = 4 * dh, 2 * dh
    wr = 128 // ng
    hq = sq // 4
    xs, wqs, wos = (ax, bx), (awq, bwq), (awo, bwo)
    kvs = (akt, avt, bkt, bvt)
    xc, x4 = (xca, xcb), (x4a, x4b)
    wsets = ((wqc0, wq40, woc0, wo40), (wqc1, wq41, woc1, wo41))

    def wait_all(ref, sem):
        pltpu.make_async_copy(ref, ref, sem).wait()

    def fetch(pp, gg, slot):
        for t in range(4):
            pltpu.make_async_copy(kvs[t].at[pl.ds(gg * 2, 2), pl.ds(4 * pp, 4)],
                                  kvbuf.at[slot, t], kvsem.at[slot]).start()
        pw = jnp.minimum(pp + 1, npass - 1)
        rows = pl.ds(pl.multiple_of(gg * wr, 16), wr)
        for j in range(2):
            for t in range(5):
                pltpu.make_async_copy(wqs[j].at[t, rows, pl.ds(pl.multiple_of(pw * gw, 128), gw)],
                                      rq.at[slot, j, t], rqsem.at[slot]).start()
            pltpu.make_async_copy(wos[j].at[pw, :, rows], ro.at[slot, j], rosem.at[slot]).start()

    def fetch_wait(slot):
        wait_all(kvbuf.at[slot], kvsem.at[slot])
        wait_all(rq.at[slot], rqsem.at[slot])
        wait_all(ro.at[slot], rosem.at[slot])

    def x_copy(j, gg):
        return pltpu.make_async_copy(xs[j].at[pl.ds(gg * 2, 2)], xbuf.at[j, gg], xsem.at[j, gg])

    def build_x(j, gg):
        back = []
        for r in range(0, sq, 32):
            x0 = xbuf.at[j, gg, 0][r:r + 32, :].astype(f32)
            x1 = xbuf.at[j, gg, 1][r:r + 32, :].astype(f32)
            rows = slice(r // 2, r // 2 + 16)
            cs = _lhs_combos(x0[:, :256], x0[:, 256:512], x1[:, :256], x1[:, 256:512])
            for k, c in enumerate(cs):
                xc[j].at[gg, k][rows, :] = _pack(c)
            x4[j].at[gg][rows, :] = _pack(_cat([x0[:, 512:], x1[:, 512:]], 1))
            back += [xc[j].at[gg, k][rows, :] for k in range(7)] + [x4[j].at[gg][rows, :]]
        return back

    def build_wq(j, gg, raw, wset):
        wqc, wq4, _, _ = wset
        kt = [raw(t).astype(f32) for t in range(5)]
        l1 = [_rhs_combos(kt[t][:, :hw], kt[t][:, hw:], kt[2 + t][:, :hw], kt[2 + t][:, hw:])
              for t in range(2)]
        rows = pl.ds(pl.multiple_of(gg * (wr // 2), 8), wr // 2)
        for k in range(7):
            wqc.at[j, k][rows, :] = _pack(_cat([l1[0][k], l1[1][k]], 1))
        wq4.at[j][rows, :] = _pack(kt[4])
        return [wqc.at[j, k][rows, :] for k in range(7)] + [wq4.at[j][rows, :]]

    def build_wo(j, gg, raw, wset):
        _, _, woc, wo4 = wset
        kt = [raw(t).astype(f32) for t in range(6)]
        l1 = [_rhs_combos(kt[3 + t][:, :256], kt[3 + t][:, 256:512], kt[t][:, :256], kt[t][:, 256:512])
              for t in range(3)]
        rows = pl.ds(pl.multiple_of(gg * (wr // 2), 8), wr // 2)
        back = []
        for k in range(7):
            b = [[_col(l1[t][k], n) for n in range(2)] for t in range(3)]
            if k == 2:
                tiles = [b[t][n] for n in range(2) for t in range(3)]
            else:
                tiles = list(_rhs_combos(b[0][0], b[0][1], b[1][0], b[1][1])) + b[2]
            cols = slice(0, 128 * len(tiles))
            woc.at[j, k][rows, cols] = _pack(_cat(tiles, 1))
            back.append(woc.at[j, k][rows, cols])
        wo4.at[j][rows, :] = _pack(_cat([x[:, 512:] for x in kt], 1))
        return back + [wo4.at[j][rows, :]]

    def compute(seq, g, slot, par, q_ref, first, write_out, last=None):
        wqc, wq4, woc, wo4 = wsets[par]
        s, qm, om, toks = {}, {}, {}, []
        zero = jnp.full((8, 128), zref[0], i32)

        def lhs(x):
            if toks:
                t = toks.pop(0) & zero
                x = _cat([x[:8] | _cat([t] * (x.shape[1] // 128), 1), x[8:]], 0)
            return _unpack(x)

        def q_m(j, k, n):
            x, w = xc[j].at[g, k], wqc.at[j, k]
            qm[j, k, n] = (_dot(lhs(x[:, :128]), _unpack(w[:, 128 * n:128 * (n + 1)]))
                           + _dot(lhs(x[:, 128:]), _unpack(w[:, hw + 128 * n:hw + 128 * (n + 1)])))

        def q_k(j, u, n):
            col = (u % 2) * hw + 128 * n
            qm[j, 'k', u, n] = _dot(lhs(x4[j].at[g][:, 128 * (u // 2):128 * (u // 2 + 1)]),
                                    _unpack(wq4.at[j][:, col:col + 128]))

        def q_fin(j, u):
            for n in range(3):
                m = lambda k: qm[j, k, n]
                kk = qm[j, 'k', u, n]
                y = (lambda: (m(0) + kk) + m(6) + (m(3) - m(4)), lambda: m(2) + m(4) + kk,
                     lambda: m(1) + m(3) + kk, lambda: (m(0) + kk) + m(5) + (m(2) - m(1)))[u]()
                y = y * scale
                q_ref.at[j, u][:, 128 * n:128 * (n + 1)] = _pack(y)
                if n == 1:
                    q_ref.at[j, u][:, 384:] = _pack(pltpu.roll(y, 64, 1))

        def q_piece(j, part):
            if part < 2:
                for n in range(3):
                    q_m(j, (2, 1)[part], n), q_m(j, (4, 3)[part], n)
                for a in (((0, 1, 0), (0, 1, 1), (0, 1, 2), (0, 2, 0)),
                          ((0, 2, 1), (0, 2, 2), (1, 1, 0), (1, 1, 1)),
                          ((1, 1, 2), (1, 2, 0), (1, 2, 1), (1, 2, 2)), ())[2 * j + part]:
                    q_k(*a)
                q_fin(j, 1 + part)
            elif part == 2:
                for n in range(3):
                    q_m(j, 0, n), q_k(j, 0, n), q_k(j, 3, n)
            else:
                for n in range(3):
                    q_m(j, 6, n), q_m(j, 5, n)
                q_fin(j, 0)
                q_fin(j, 3)

        def r_piece(j, part):
            for n in range(3):
                q_m(j, (2, 1)[part], n), q_m(j, (4, 3)[part], n)
            for n in range(3):
                q_k(j, 1 + part, n)
            q_fin(j, 1 + part)

        def x_piece(j):
            if j == 1:
                build_x(1, g)
            else:
                toks.append(_or_tiles(build_x(0, jnp.minimum(g + 1, ng - 1))))

        def kv(j, which, u):
            return tuple(kvbuf[slot, 2 * j + which, u // 2, 2 * (u % 2) + h] for h in range(2))

        def s_piece(j, u):
            s[j, u] = _scores(q_ref.at[j, u], *kv(j, 0, u), lhs)

        def p_piece(j, u):
            def sink(c, *o):
                rows = [slice(h * hq + c * CH // 2, h * hq + (c + 1) * CH // 2) for h in range(2)]
                prev = lambda v: [_unpack(oraw.at[j, v][rows[h], :]).astype(f32) for h in range(2)]
                add = lambda x, y: [x[h] + y[h] for h in range(2)]
                sub = lambda x, y: [x[h] - y[h] for h in range(2)]
                for h in range(2):
                    oraw.at[j, u][rows[h], :] = _pack(o[h])
                new = {1: lambda: {},
                       2: lambda: {3: o, 0: add(prev(1), o)},
                       0: lambda: {4: add(prev(1), o), 6: sub(o, prev(2))},
                       3: lambda: {1: add(o, prev(2)), 5: sub(o, prev(1))}}[u]()
                for k, v in new.items():
                    cs = _lhs_combos(_col(v[0], 0), _col(v[0], 1), _col(v[1], 0), _col(v[1], 1))
                    blocks = [cs[t] for t in (0, 1, 4, 5, 6)]
                    if k != 3:
                        blocks += [cs[2], cs[3], _col(v[0], 2), _col(v[1], 2)]
                    oc.at[j, k][rows[0], :128 * len(blocks)] = _pack(_cat(blocks, 1))

            _attend(s.pop((j, u)), *kv(j, 1, u), pbuf.at[(1, 2, 0, 3).index(u)], zero, lhs, sink)

        def emit(j, i, col, y):
            b = 2 * g + i
            cols = slice(j * d + col, j * d + col + 128)
            if not first:
                y = y + acc[b, :, cols]
            acc[b, :, cols] = y
            if write_out:
                obuf[b, :, cols] = y.astype(bf16)

        def o_w(j, k, t):
            return _unpack(woc.at[j, k][:, 128 * t:128 * (t + 1)])

        def o_m(j, k):
            def blk(t):
                if k == 3 and t in (2, 3, 7, 8):
                    h, kt = {2: (0, 0), 3: (1, 1), 7: (0, 2), 8: (1, 2)}[t]
                    return oraw.at[j, 2][h * hq:(h + 1) * hq, 128 * kt:128 * (kt + 1)]
                pos = (0, 1, 4, 5, 6, 2, 3, 7, 8).index(t)
                return oc.at[j, k][:, 128 * pos:128 * (pos + 1)]

            mm = lambda t: _dot(lhs(blk(t)), o_w(j, k, t))
            kk = lambda h, n: _dot(lhs(blk(7 + h)), o_w(j, k, 7 + n))
            m2, m4, k01, m0 = mm(2), mm(4), kk(0, 1), mm(0)
            m1, m3, k10, m6 = mm(1), mm(3), kk(1, 0), mm(6)
            k00, m5, k11 = kk(0, 0), mm(5), kk(1, 1)
            om[j, k, 0] = _cat([((m0 - m4) + (m3 + m6)) + k00, m1 + m3 + k10], 0)
            om[j, k, 1] = _cat([m2 + m4 + k01, ((m0 + m2) - m1) + (m5 + k11)], 0)

        def o_n(j, i, t, half=None):
            x = oraw.at[j, 2 * i + t // 3][:, 128 * (t % 3):128 * (t % 3 + 1)]
            w = _unpack(wo4.at[j][:, 128 * t:128 * (t + 1)])
            if half is None:
                y = _dot(lhs(x), w)
                parts = {h: y[h * 2 * hq:(h + 1) * 2 * hq] for h in range(2)}
            else:
                parts = {half: _dot(lhs(x[half * hq:(half + 1) * hq]), w)}
            for h, y in parts.items():
                om[j, 'n', i, h] = om[j, 'n', i, h] + y if (j, 'n', i, h) in om else y

        def emit_n(j, i):
            emit(j, i, 512, _cat([om[j, 'n', i, h] for h in range(2)], 0))

        def flush(i):
            if write_out:
                @pl.when(last)
                def _():
                    pltpu.make_async_copy(obuf.at[2 * g + i], out.at[2 * g + i], osem).start()

        def o_piece(j, part):
            m = lambda k, c: om[j, k, c]
            if part == 0:
                for c in range(2):
                    om[j, 2, c] = _dot(lhs(oraw[j, 1]), _cat([o_w(j, 2, 3 * c + t) for t in range(3)], 0))
                o_n(j, 0, 3), o_n(j, 0, 4)
                return
            ka, kb = ((0, 3), (4, 6), (1, 5))[part - 1]
            o_m(j, ka), o_n(j, 1, part - 1, 0)
            o_m(j, kb), o_n(j, 1, part - 1, 1)
            if part == 2:
                for c in range(2):
                    emit(j, 0, 256 + 128 * c, m(2, c) + m(4, c))
                    emit(j, 0, 128 * c, (m(0, c) + m(3, c) - m(4, c)) + m(6, c))
                for t in (5, 0, 1, 2):
                    o_n(j, 0, t)
                emit_n(j, 0)
                if j == 1:
                    flush(0)
            elif part == 3:
                for c in range(2):
                    emit(j, 1, 128 * c, m(1, c) + m(3, c))
                    emit(j, 1, 256 + 128 * c, (m(0, c) + m(2, c) - m(1, c)) + m(5, c))
                if j == 0:
                    for t in (3, 4):
                        o_n(0, 1, t, 0), o_n(0, 1, t, 1)
                else:
                    o_n(0, 1, 5)
                    emit_n(0, 1)
                    for t in (3, 4, 5):
                        o_n(1, 1, t)
                    emit_n(1, 1)
                    flush(1)

        def w_piece(k):
            j = k // 2
            back = (build_wq(j, g, lambda t: rq[slot, j, t], wsets[1 - par]) if k % 2 == 0
                    else build_wo(j, g, lambda t: ro[slot, j, t], wsets[1 - par]))
            toks.append(_or_tiles(back))

        run = {'q': q_piece, 's': s_piece, 'p': p_piece, 'o': o_piece, 'w': w_piece,
               'r': r_piece, 'x': x_piece}
        for tok in seq.split():
            run[tok[0]](*(int(ch) for ch in tok[1:]))

    def run_pass(p, par, first, slot0):
        def step(g, slot):
            fetch_wait(slot)

            wrap = g + 2 >= ng
            fetch(jnp.minimum(jnp.where(wrap, p + 1, p), npass - 1),
                  jnp.where(wrap, g + 2 - ng, g + 2), jnp.where(slot == 0, NKV - 1, slot - 1))

            if first:
                compute(_SEQ_NOQ, g, slot, par, qall.at[g], True, False)
            else:
                compute(_SEQ_FULL, g, slot, par, qbuf, False, par == 1, p == npass - 1)
            return jnp.where(slot == NKV - 1, 0, slot + 1)

        jax.lax.fori_loop(0, ng, step, slot0)

    def init_weights(build, raw):
        def body(gg, carry):
            rows = pl.ds(pl.multiple_of(gg * wr, 16), wr)
            for j in range(2):
                build(j, gg, lambda t: raw.at[j, t][rows, :], wsets[0])
            return carry

        jax.lax.fori_loop(0, ng, body, 0)

    zref[0] = 0
    x_copy(0, 0).start()
    for j in range(2):
        pltpu.make_async_copy(wqs[j].at[:, :, pl.ds(0, gw)], rq0.at[j], isem.at[0]).start()
    x_copy(0, 0).wait()
    build_x(0, 0)
    wait_all(rq0, isem.at[0])
    for gg in range(ng):
        x_copy(1, gg).start()
        if gg + 1 < ng:
            x_copy(0, gg + 1).start()
    init_weights(build_wq, rq0)

    def q_step(g, carry):
        x_copy(1, g).wait()

        @pl.when(g + 1 < ng)
        def _():
            x_copy(0, g + 1).wait()

        @pl.when(g == 1)
        def _():
            for j in range(2):
                pltpu.make_async_copy(wos[j].at[0], ro0.at[j], isem.at[1]).start()
            fetch(0, 0, 0)

        @pl.when(g == 4)
        def _():
            fetch(0, 1, 1)

        compute(_SEQ_Q, g, 0, 0, qall.at[g], True, False)
        return carry

    jax.lax.fori_loop(0, ng, q_step, 0)
    wait_all(ro0, isem.at[1])
    init_weights(build_wo, ro0)

    run_pass(0, 0, True, 0)

    def pass_pair(pp, carry):
        run_pass(2 * pp + 1, 1, False, ((2 * pp + 1) * ng) % NKV)

        @pl.when(2 * pp + 2 < npass)
        def _():
            run_pass(2 * pp + 2, 0, False, ((2 * pp + 2) * ng) % NKV)

        return carry

    jax.lax.fori_loop(0, npass // 2, pass_pair, 0)
    fetch_wait(nsteps % NKV)
    fetch_wait((nsteps + 1) % NKV)
    wait_all(out, osem)


@jax.jit
def pallas_concat_heads__gqa_block_cached__mha_block_cached__near_ridge_kernel(
    A_x: jax.Array,
    A_k_cache: jax.Array,
    A_v_cache: jax.Array,
    A_wq: jax.Array,
    A_wo: jax.Array,
    B_x: jax.Array,
    B_k_cache: jax.Array,
    B_v_cache: jax.Array,
    B_wq: jax.Array,
    B_wo: jax.Array,
):
    B, Sq, D = A_x.shape
    _, H, Sk, Dh = A_k_cache.shape
    assert (B, Sq, D, H, Sk, Dh) == (16, 160, 640, 32, 512, 192)
    npass, ng = H // 4, B // 2
    gw, hw = 4 * Dh, 2 * Dh
    scale = (Dh ** -0.5) * math.log2(math.e)

    akt, avt, bkt, bvt = (jnp.swapaxes(t, 2, 3) for t in
                          (A_k_cache, A_v_cache, B_k_cache, B_v_cache))
    awq, bwq = (w.reshape(5, 128, H * Dh) for w in (A_wq, B_wq))
    awo, bwo = (w.reshape(npass, 6, 128, D) for w in (A_wo, B_wo))
    any_spec = pl.BlockSpec(memory_space=pl.ANY)
    wset = [
        pltpu.VMEM((2, 7, 64, 2 * hw), i32),
        pltpu.VMEM((2, 64, gw), i32),
        pltpu.VMEM((2, 7, 64, 9 * 128), i32),
        pltpu.VMEM((2, 64, 6 * 128), i32),
    ]

    return pl.pallas_call(
        functools.partial(_kernel, scale=scale, d=D, sq=Sq, nbatch=B, npass=npass, dh=Dh),
        in_specs=[any_spec] * 10,
        out_specs=any_spec,
        out_shape=jax.ShapeDtypeStruct((B, Sq, 2 * D), A_x.dtype),
        scratch_shapes=[
            pltpu.VMEM((2, ng, 2, Sq, D), bf16),
            pltpu.VMEM((ng, 7, Sq // 2, 256), i32),
            pltpu.VMEM((ng, 7, Sq // 2, 256), i32),
            pltpu.VMEM((ng, Sq // 2, 256), i32),
            pltpu.VMEM((ng, Sq // 2, 256), i32),
            pltpu.VMEM((NKV, 4, 2, 4, Dh, Sk), bf16),
            pltpu.VMEM((NKV, 2, 5, 128 // ng, gw), bf16),
            pltpu.VMEM((NKV, 2, 6, 128 // ng, D), bf16),
            pltpu.VMEM((2, 5, 128, gw), bf16),
            pltpu.VMEM((2, 6, 128, D), bf16),
            *wset, *wset,
            pltpu.VMEM((B, Sq, 2 * D), f32),
            pltpu.VMEM((B, Sq, 2 * D), bf16),
            pltpu.VMEM((NPS, 2, Sq // 2, 768), i32),
            pltpu.VMEM((2, 4, Sq // 2, 512), i32),
            pltpu.VMEM((ng, 2, 4, Sq // 2, 512), i32),
            pltpu.VMEM((2, 7, Sq // 4, 9 * 128), i32),
            pltpu.VMEM((2, 4, Sq // 2, hw), i32),
            pltpu.SMEM((1,), i32),
            pltpu.SemaphoreType.DMA((2, ng)),
            pltpu.SemaphoreType.DMA((NKV,)),
            pltpu.SemaphoreType.DMA((NKV,)),
            pltpu.SemaphoreType.DMA((NKV,)),
            pltpu.SemaphoreType.DMA((2,)),
            pltpu.SemaphoreType.DMA(()),
        ],
        compiler_params=pltpu.CompilerParams(
            vmem_limit_bytes=116 * 1024 * 1024,
            disable_bounds_checks=True,
        ),
    )(A_x, akt, avt, awq, awo, B_x, bkt, bvt, bwq, bwo)
```

```python
import functools
import math

import jax
import jax.numpy as jnp
import jax.experimental.pallas as pl
import jax.experimental.pallas.tpu as pltpu

_NN = (((1,), (0,)), ((), ()))
_NT = (((1,), (1,)), ((), ()))
bf16 = jnp.bfloat16
f32 = jnp.float32
i32 = jnp.int32

CH = 16
DEP = 3
NKV = 3
NPS = 4

_SEQ_FULL = ('q00 w0 q01 s01 w1 q02 p01 w2 s02 w3 q03 p02 s00 p00 q10 s03 q11 o01 '
             's11 q12 q13 p03 o00 o02 p11 s12 o03 s10 o10 p12 s13 p10 o11 p13 o12 o13')
_SEQ_NOQ = ('s01 s02 p01 w1 s00 p02 p00 s03 o01 w0 s11 w2 p03 s12 p11 p12 o00 o02 '
            's10 o11 w3 p10 s13 o03 p13 o10 o12 o13')
_SEQ_Q = 'x1 r00 v0 r01 q02 v1 q03 r10 r11 x0 q12 q13'


def _dot(a, b, dims=_NN):
    return jax.lax.dot_general(a, b, dims, preferred_element_type=f32)


def _recip(l):
    r = pl.reciprocal(l, approx=True)
    return r * (2.0 - l * r)


def _col(x, i):
    return x[:, 128 * i:128 * (i + 1)]


def _pack(x):
    return pltpu.bitcast(x.astype(bf16), i32)


def _unpack(x):
    return pltpu.bitcast(x, bf16)


def _cat(xs, axis):
    return jnp.concatenate(list(xs), axis=axis)


def _or_tiles(vals):
    t = None
    for v in vals:
        for r in range(0, v.shape[0], 8):
            for c in range(0, v.shape[1], 128):
                x = v[r:r + 8, c:c + 128]
                t = x if t is None else t | x
    return t


def _lane_lo(rows):
    return jax.lax.broadcasted_iota(i32, (rows, 128), 1) < 64


def _lhs_combos(a11, a12, a21, a22):
    return (a11 + a22, a21 + a22, a11, a22, a11 + a12, a21 - a11, a12 - a22)


def _rhs_combos(b11, b12, b21, b22):
    return (b11 + b22, b11, b12 - b22, b21 - b11, b22, b11 + b12, b21 + b22)


def _weights(xa, xb, xc):
    h = xa.shape[1] // 2
    xa, xb, xc = xa.astype(f32), xb.astype(f32), xc.astype(f32)
    return (_cat([xa[:, :h], xb[:, :h] - xb[:, h:]], 0),
            _cat([xa[:, h:], xc[:, h:] - xc[:, :h]], 0),
            _cat([xc[:, :h], xb[:, h:]], 0))


def _pair_weights(t0, t1):
    return (_weights(t0[:64], t0[64:128], t0[128:]), _weights(t1[64:128], t1[128:], t1[:64]))


def _scores(q_ref, kt0, kt1, lhs):
    t0, t1, t2, rot = (q_ref[:, 128 * k:128 * (k + 1)] for k in range(4))
    lo = _lane_lo(t0.shape[0])
    q = ((t0, jnp.where(lo, t0, rot), jnp.where(lo, t1, t0)),
         (t2, jnp.where(lo, t2, t1), jnp.where(lo, rot, t2)))
    w = _pair_weights(kt0, kt1)
    p = {}

    def run(h, k, i):
        y = _dot(lhs(q[h][k]), _col(w[h][k], i).astype(bf16))
        p[h, k, i] = y if k == 2 else y + p[h, 2, i]

    for t, (h, i) in enumerate(((0, 0), (0, 1), (1, 0))):
        run(h, 2, i), run(h, 0, i), run(h, 1, i), run(1, (2, 0, 1)[t], 1)
    return tuple(_cat([p[h, 0, 0], p[h, 0, 1], p[h, 1, 0], p[h, 1, 1]], 1) for h in range(2))


def _softmax_terms(s, p_ref, zero):
    ls, toks = [], []
    for c in range(s.shape[0] // CH):
        sc = s[c * CH:(c + 1) * CH]
        m = jnp.broadcast_to(jnp.max(sc, axis=-1, keepdims=True), (CH, 128))
        if c >= DEP:
            t = toks[c - DEP] & zero
            m = pltpu.bitcast(pltpu.bitcast(m, i32) | _cat([t, t], 0), f32)
        e = [jnp.exp2(_col(sc, k) - m) for k in range(4)]
        t0, t1 = e[0] + e[2], e[1] + e[3]
        ls.append(jnp.broadcast_to(jnp.sum(t0 + t1, axis=-1, keepdims=True), (CH, 128)))
        rows = slice(c * CH // 2, (c + 1) * CH // 2)
        for k, x in enumerate(e + [t0, t1]):
            p_ref[rows, 128 * k:128 * (k + 1)] = _pack(x)
        toks.append(_or_tiles([p_ref[rows, :]]))
    return ls


def _attend(s, vt0, vt1, p_ref, zero, lhs, sink):
    ls = [_softmax_terms(s[h], p_ref.at[h], zero) for h in range(2)]
    w = _pair_weights(vt0, vt1)
    r = {}
    for h, k in ((0, 0), (0, 1), (0, 2), (1, 1), (1, 2), (1, 0)):
        r[h, k] = _dot(lhs(p_ref.at[h][:, 256 * k:256 * (k + 1)]), w[h][k].astype(bf16), _NT)
    lo = _lane_lo(CH)

    def rows(c):
        p1, p2, p3, u1, u2, u3 = (r[h, k][c * CH:(c + 1) * CH] for h in range(2) for k in range(3))
        r0, r1 = _recip(ls[0][c]), _recip(ls[1][c])
        o_lo = p1 + jnp.where(lo, p2, p3)
        o_hi = u1 + jnp.where(lo, u2, u3)
        mid = jnp.where(lo, p3, u2) + pltpu.roll(jnp.where(lo, u3, p2), 64, 1)
        return _cat([o_lo * r0, mid * jnp.where(lo, r0, r1), o_hi * r1], 1)

    n = len(ls[0]) // 2
    for c in range(n):
        sink(c, rows(c), rows(c + n))


def _kernel(ax, akt, avt, awq, awo, bx, bkt, bvt, bwq, bwo, out,
            xbuf, xca, xcb, x4a, x4b, kvbuf, rq, ro, rq0, ro0,
            wqc0, wq40, woc0, wo40, wqc1, wq41, woc1, wo41,
            acc, obuf, pbuf, qbuf, qall, oc, oraw, zref,
            xsem, kvsem, rqsem, rosem, isem, vsem, osem,
            *, scale, d, sq, nbatch, npass, dh):
    ng = nbatch // 2
    nsteps = npass * ng
    gw, hw = 4 * dh, 2 * dh
    wr = 128 // ng
    hq = sq // 4
    xs, wqs, wos = (ax, bx), (awq, bwq), (awo, bwo)
    kvs = (akt, avt, bkt, bvt)
    xc, x4 = (xca, xcb), (x4a, x4b)
    wsets = ((wqc0, wq40, woc0, wo40), (wqc1, wq41, woc1, wo41))

    def wait_all(ref, sem):
        pltpu.make_async_copy(ref, ref, sem).wait()

    def fetch(pp, gg, slot):
        for t in range(4):
            pltpu.make_async_copy(kvs[t].at[pl.ds(gg * 2, 2), pl.ds(4 * pp, 4)],
                                  kvbuf.at[slot, t], kvsem.at[slot]).start()
        pw = jnp.minimum(pp + 1, npass - 1)
        rows = pl.ds(pl.multiple_of(gg * wr, 16), wr)
        for j in range(2):
            for t in range(5):
                pltpu.make_async_copy(wqs[j].at[t, rows, pl.ds(pl.multiple_of(pw * gw, 128), gw)],
                                      rq.at[slot, j, t], rqsem.at[slot]).start()
            pltpu.make_async_copy(wos[j].at[pw, :, rows], ro.at[slot, j], rosem.at[slot]).start()

    def fetch_wait(slot):
        wait_all(kvbuf.at[slot], kvsem.at[slot])
        wait_all(rq.at[slot], rqsem.at[slot])
        wait_all(ro.at[slot], rosem.at[slot])

    def x_copy(j, gg):
        return pltpu.make_async_copy(xs[j].at[pl.ds(gg * 2, 2)], xbuf.at[j, gg], xsem.at[j, gg])

    def build_x(j, gg):
        back = []
        for r in range(0, sq, 32):
            x0 = xbuf.at[j, gg, 0][r:r + 32, :].astype(f32)
            x1 = xbuf.at[j, gg, 1][r:r + 32, :].astype(f32)
            rows = slice(r // 2, r // 2 + 16)
            cs = _lhs_combos(x0[:, :256], x0[:, 256:512], x1[:, :256], x1[:, 256:512])
            for k, c in enumerate(cs):
                xc[j].at[gg, k][rows, :] = _pack(c)
            x4[j].at[gg][rows, :] = _pack(_cat([x0[:, 512:], x1[:, 512:]], 1))
            back += [xc[j].at[gg, k][rows, :] for k in range(7)] + [x4[j].at[gg][rows, :]]
        return back

    def build_wq(j, gg, raw, wset):
        wqc, wq4, _, _ = wset
        kt = [raw(t).astype(f32) for t in range(5)]
        l1 = [_rhs_combos(kt[t][:, :hw], kt[t][:, hw:], kt[2 + t][:, :hw], kt[2 + t][:, hw:])
              for t in range(2)]
        rows = pl.ds(pl.multiple_of(gg * (wr // 2), 8), wr // 2)
        for k in range(7):
            wqc.at[j, k][rows, :] = _pack(_cat([l1[0][k], l1[1][k]], 1))
        wq4.at[j][rows, :] = _pack(kt[4])
        return [wqc.at[j, k][rows, :] for k in range(7)] + [wq4.at[j][rows, :]]

    def build_wo(j, gg, raw, wset):
        _, _, woc, wo4 = wset
        kt = [raw(t).astype(f32) for t in range(6)]
        l1 = [_rhs_combos(kt[3 + t][:, :256], kt[3 + t][:, 256:512], kt[t][:, :256], kt[t][:, 256:512])
              for t in range(3)]
        rows = pl.ds(pl.multiple_of(gg * (wr // 2), 8), wr // 2)
        back = []
        for k in range(7):
            b = [[_col(l1[t][k], n) for n in range(2)] for t in range(3)]
            if k == 2:
                tiles = [b[t][n] for n in range(2) for t in range(3)]
            else:
                tiles = list(_rhs_combos(b[0][0], b[0][1], b[1][0], b[1][1])) + b[2]
            cols = slice(0, 128 * len(tiles))
            woc.at[j, k][rows, cols] = _pack(_cat(tiles, 1))
            back.append(woc.at[j, k][rows, cols])
        wo4.at[j][rows, :] = _pack(_cat([x[:, 512:] for x in kt], 1))
        return back + [wo4.at[j][rows, :]]

    def compute(seq, g, slot, par, q_ref, first, write_out, last=None):
        wqc, wq4, woc, wo4 = wsets[par]
        s, qm, om, toks = {}, {}, {}, []
        zero = jnp.full((8, 128), zref[0], i32)

        def lhs(x):
            if toks:
                t = toks.pop(0) & zero
                x = _cat([x[:8] | _cat([t] * (x.shape[1] // 128), 1), x[8:]], 0)
            return _unpack(x)

        def q_m(j, k, n):
            x, w = xc[j].at[g, k], wqc.at[j, k]
            qm[j, k, n] = (_dot(lhs(x[:, :128]), _unpack(w[:, 128 * n:128 * (n + 1)]))
                           + _dot(lhs(x[:, 128:]), _unpack(w[:, hw + 128 * n:hw + 128 * (n + 1)])))

        def q_k(j, u, n):
            col = (u % 2) * hw + 128 * n
            qm[j, 'k', u, n] = _dot(lhs(x4[j].at[g][:, 128 * (u // 2):128 * (u // 2 + 1)]),
                                    _unpack(wq4.at[j][:, col:col + 128]))

        def q_fin(j, u):
            for n in range(3):
                m = lambda k: qm[j, k, n]
                kk = qm[j, 'k', u, n]
                y = (lambda: (m(0) + kk) + m(6) + (m(3) - m(4)), lambda: m(2) + m(4) + kk,
                     lambda: m(1) + m(3) + kk, lambda: (m(0) + kk) + m(5) + (m(2) - m(1)))[u]()
                y = y * scale
                q_ref.at[j, u][:, 128 * n:128 * (n + 1)] = _pack(y)
                if n == 1:
                    q_ref.at[j, u][:, 384:] = _pack(pltpu.roll(y, 64, 1))

        def q_piece(j, part):
            if part < 2:
                for n in range(3):
                    q_m(j, (2, 1)[part], n), q_m(j, (4, 3)[part], n)
                for a in (((0, 1, 0), (0, 1, 1), (0, 1, 2), (0, 2, 0)),
                          ((0, 2, 1), (0, 2, 2), (1, 1, 0), (1, 1, 1)),
                          ((1, 1, 2), (1, 2, 0), (1, 2, 1), (1, 2, 2)), ())[2 * j + part]:
                    q_k(*a)
                q_fin(j, 1 + part)
            elif part == 2:
                for n in range(3):
                    q_m(j, 0, n), q_k(j, 0, n), q_k(j, 3, n)
            else:
                for n in range(3):
                    q_m(j, 6, n), q_m(j, 5, n)
                q_fin(j, 0)
                q_fin(j, 3)

        def r_piece(j, part):
            for n in range(3):
                q_m(j, (2, 1)[part], n), q_m(j, (4, 3)[part], n)
            for n in range(3):
                q_k(j, 1 + part, n)
            q_fin(j, 1 + part)

        def x_piece(j):
            if j == 1:
                build_x(1, g)
            else:
                toks.append(_or_tiles(build_x(0, jnp.minimum(g + 1, ng - 1))))

        def v_piece(j):
            toks.append(_or_tiles(build_wo(j, g, lambda t: ro0[g, j, t], wsets[0])))

        def kv(j, which, u):
            return tuple(kvbuf[slot, 2 * j + which, u // 2, 2 * (u % 2) + h] for h in range(2))

        def s_piece(j, u):
            s[j, u] = _scores(q_ref.at[j, u], *kv(j, 0, u), lhs)

        def p_piece(j, u):
            def sink(c, *o):
                rows = [slice(h * hq + c * CH // 2, h * hq + (c + 1) * CH // 2) for h in range(2)]
                prev = lambda v: [_unpack(oraw.at[j, v][rows[h], :]).astype(f32) for h in range(2)]
                add = lambda x, y: [x[h] + y[h] for h in range(2)]
                sub = lambda x, y: [x[h] - y[h] for h in range(2)]
                for h in range(2):
                    oraw.at[j, u][rows[h], :] = _pack(o[h])
                new = {1: lambda: {},
                       2: lambda: {3: o, 0: add(prev(1), o)},
                       0: lambda: {4: add(prev(1), o), 6: sub(o, prev(2))},
                       3: lambda: {1: add(o, prev(2)), 5: sub(o, prev(1))}}[u]()
                for k, v in new.items():
                    cs = _lhs_combos(_col(v[0], 0), _col(v[0], 1), _col(v[1], 0), _col(v[1], 1))
                    blocks = [cs[t] for t in (0, 1, 4, 5, 6)]
                    if k != 3:
                        blocks += [cs[2], cs[3], _col(v[0], 2), _col(v[1], 2)]
                    oc.at[j, k][rows[0], :128 * len(blocks)] = _pack(_cat(blocks, 1))

            _attend(s.pop((j, u)), *kv(j, 1, u), pbuf.at[(1, 2, 0, 3).index(u)], zero, lhs, sink)

        def emit(j, i, col, y):
            b = 2 * g + i
            cols = slice(j * d + col, j * d + col + 128)
            if not first:
                y = y + acc[b, :, cols]
            acc[b, :, cols] = y
            if write_out:
                obuf[b, :, cols] = y.astype(bf16)

        def o_w(j, k, t):
            return _unpack(woc.at[j, k][:, 128 * t:128 * (t + 1)])

        def o_m(j, k):
            def blk(t):
                if k == 3 and t in (2, 3, 7, 8):
                    h, kt = {2: (0, 0), 3: (1, 1), 7: (0, 2), 8: (1, 2)}[t]
                    return oraw.at[j, 2][h * hq:(h + 1) * hq, 128 * kt:128 * (kt + 1)]
                pos = (0, 1, 4, 5, 6, 2, 3, 7, 8).index(t)
                return oc.at[j, k][:, 128 * pos:128 * (pos + 1)]

            mm = lambda t: _dot(lhs(blk(t)), o_w(j, k, t))
            kk = lambda h, n: _dot(lhs(blk(7 + h)), o_w(j, k, 7 + n))
            m2, m4, k01, m0 = mm(2), mm(4), kk(0, 1), mm(0)
            m1, m3, k10, m6 = mm(1), mm(3), kk(1, 0), mm(6)
            k00, m5, k11 = kk(0, 0), mm(5), kk(1, 1)
            om[j, k, 0] = _cat([((m0 - m4) + (m3 + m6)) + k00, m1 + m3 + k10], 0)
            om[j, k, 1] = _cat([m2 + m4 + k01, ((m0 + m2) - m1) + (m5 + k11)], 0)

        def o_n(j, i, t, half=None):
            x = oraw.at[j, 2 * i + t // 3][:, 128 * (t % 3):128 * (t % 3 + 1)]
            w = _unpack(wo4.at[j][:, 128 * t:128 * (t + 1)])
            if half is None:
                y = _dot(lhs(x), w)
                parts = {h: y[h * 2 * hq:(h + 1) * 2 * hq] for h in range(2)}
            else:
                parts = {half: _dot(lhs(x[half * hq:(half + 1) * hq]), w)}
            for h, y in parts.items():
                om[j, 'n', i, h] = om[j, 'n', i, h] + y if (j, 'n', i, h) in om else y

        def emit_n(j, i):
            emit(j, i, 512, _cat([om[j, 'n', i, h] for h in range(2)], 0))

        def flush(i):
            if write_out:
                @pl.when(last)
                def _():
                    pltpu.make_async_copy(obuf.at[2 * g + i], out.at[2 * g + i], osem).start()

        def o_piece(j, part):
            m = lambda k, c: om[j, k, c]
            if part == 0:
                for c in range(2):
                    om[j, 2, c] = _dot(lhs(oraw[j, 1]), _cat([o_w(j, 2, 3 * c + t) for t in range(3)], 0))
                o_n(j, 0, 3), o_n(j, 0, 4)
                return
            ka, kb = ((0, 3), (4, 6), (1, 5))[part - 1]
            o_m(j, ka), o_n(j, 1, part - 1, 0)
            o_m(j, kb), o_n(j, 1, part - 1, 1)
            if part == 2:
                for c in range(2):
                    emit(j, 0, 256 + 128 * c, m(2, c) + m(4, c))
                    emit(j, 0, 128 * c, (m(0, c) + m(3, c) - m(4, c)) + m(6, c))
                for t in (5, 0, 1, 2):
                    o_n(j, 0, t)
                emit_n(j, 0)
                if j == 1:
                    flush(0)
            elif part == 3:
                for c in range(2):
                    emit(j, 1, 128 * c, m(1, c) + m(3, c))
                    emit(j, 1, 256 + 128 * c, (m(0, c) + m(2, c) - m(1, c)) + m(5, c))
                if j == 0:
                    for t in (3, 4):
                        o_n(0, 1, t, 0), o_n(0, 1, t, 1)
                else:
                    o_n(0, 1, 5)
                    emit_n(0, 1)
                    for t in (3, 4, 5):
                        o_n(1, 1, t)
                    emit_n(1, 1)
                    flush(1)

        def w_piece(k):
            j = k // 2
            back = (build_wq(j, g, lambda t: rq[slot, j, t], wsets[1 - par]) if k % 2 == 0
                    else build_wo(j, g, lambda t: ro[slot, j, t], wsets[1 - par]))
            toks.append(_or_tiles(back))

        run = {'q': q_piece, 's': s_piece, 'p': p_piece, 'o': o_piece, 'w': w_piece,
               'r': r_piece, 'x': x_piece, 'v': v_piece}
        for tok in seq.split():
            run[tok[0]](*(int(ch) for ch in tok[1:]))

    def run_pass(p, par, first, slot0):
        def step(g, slot):
            fetch_wait(slot)

            wrap = g + 2 >= ng
            fetch(jnp.minimum(jnp.where(wrap, p + 1, p), npass - 1),
                  jnp.where(wrap, g + 2 - ng, g + 2), jnp.where(slot == 0, NKV - 1, slot - 1))

            if first:
                compute(_SEQ_NOQ, g, slot, par, qall.at[g], True, False)
            else:
                compute(_SEQ_FULL, g, slot, par, qbuf, False, par == 1, p == npass - 1)
            return jnp.where(slot == NKV - 1, 0, slot + 1)

        jax.lax.fori_loop(0, ng, step, slot0)

    def wq_init(j):
        return pltpu.make_async_copy(wqs[j].at[:, :, pl.ds(0, gw)], rq0.at[j], isem.at[j])

    zref[0] = 0
    x_copy(0, 0).start()
    wq_init(0).start()
    x_copy(0, 0).wait()
    wq_init(1).start()
    build_x(0, 0)
    for j in range(2):
        wq_init(j).wait()
        if j == 0:
            for gg in range(ng):
                x_copy(1, gg).start()
                for jj in range(2):
                    pltpu.make_async_copy(wos[jj].at[0, :, pl.ds(gg * wr, wr)], ro0.at[gg, jj],
                                          vsem.at[gg]).start()
                if gg + 1 < ng:
                    x_copy(0, gg + 1).start()

        def init_wq(gg, carry, j=j):
            rows = pl.ds(pl.multiple_of(gg * wr, 16), wr)
            build_wq(j, gg, lambda t: rq0.at[j, t][rows, :], wsets[0])
            return carry

        jax.lax.fori_loop(0, ng, init_wq, 0)

    def q_step(g, carry):
        x_copy(1, g).wait()
        wait_all(ro0.at[g], vsem.at[g])

        @pl.when(g + 1 < ng)
        def _():
            x_copy(0, g + 1).wait()

        @pl.when(g == 1)
        def _():
            fetch(0, 0, 0)

        @pl.when(g == 4)
        def _():
            fetch(0, 1, 1)

        compute(_SEQ_Q, g, 0, 0, qall.at[g], True, False)
        return carry

    jax.lax.fori_loop(0, ng, q_step, 0)

    run_pass(0, 0, True, 0)

    def pass_pair(pp, carry):
        run_pass(2 * pp + 1, 1, False, ((2 * pp + 1) * ng) % NKV)

        @pl.when(2 * pp + 2 < npass)
        def _():
            run_pass(2 * pp + 2, 0, False, ((2 * pp + 2) * ng) % NKV)

        return carry

    jax.lax.fori_loop(0, npass // 2, pass_pair, 0)
    fetch_wait(nsteps % NKV)
    fetch_wait((nsteps + 1) % NKV)
    wait_all(out, osem)


@jax.jit
def pallas_concat_heads__gqa_block_cached__mha_block_cached__near_ridge_kernel(
    A_x: jax.Array,
    A_k_cache: jax.Array,
    A_v_cache: jax.Array,
    A_wq: jax.Array,
    A_wo: jax.Array,
    B_x: jax.Array,
    B_k_cache: jax.Array,
    B_v_cache: jax.Array,
    B_wq: jax.Array,
    B_wo: jax.Array,
):
    B, Sq, D = A_x.shape
    _, H, Sk, Dh = A_k_cache.shape
    assert (B, Sq, D, H, Sk, Dh) == (16, 160, 640, 32, 512, 192)
    npass, ng = H // 4, B // 2
    gw, hw = 4 * Dh, 2 * Dh
    scale = (Dh ** -0.5) * math.log2(math.e)

    akt, avt, bkt, bvt = (jnp.swapaxes(t, 2, 3) for t in
                          (A_k_cache, A_v_cache, B_k_cache, B_v_cache))
    awq, bwq = (w.reshape(5, 128, H * Dh) for w in (A_wq, B_wq))
    awo, bwo = (w.reshape(npass, 6, 128, D) for w in (A_wo, B_wo))
    any_spec = pl.BlockSpec(memory_space=pl.ANY)
    wset = [
        pltpu.VMEM((2, 7, 64, 2 * hw), i32),
        pltpu.VMEM((2, 64, gw), i32),
        pltpu.VMEM((2, 7, 64, 9 * 128), i32),
        pltpu.VMEM((2, 64, 6 * 128), i32),
    ]

    return pl.pallas_call(
        functools.partial(_kernel, scale=scale, d=D, sq=Sq, nbatch=B, npass=npass, dh=Dh),
        in_specs=[any_spec] * 10,
        out_specs=any_spec,
        out_shape=jax.ShapeDtypeStruct((B, Sq, 2 * D), A_x.dtype),
        scratch_shapes=[
            pltpu.VMEM((2, ng, 2, Sq, D), bf16),
            pltpu.VMEM((ng, 7, Sq // 2, 256), i32),
            pltpu.VMEM((ng, 7, Sq // 2, 256), i32),
            pltpu.VMEM((ng, Sq // 2, 256), i32),
            pltpu.VMEM((ng, Sq // 2, 256), i32),
            pltpu.VMEM((NKV, 4, 2, 4, Dh, Sk), bf16),
            pltpu.VMEM((NKV, 2, 5, 128 // ng, gw), bf16),
            pltpu.VMEM((NKV, 2, 6, 128 // ng, D), bf16),
            pltpu.VMEM((2, 5, 128, gw), bf16),
            pltpu.VMEM((ng, 2, 6, 128 // ng, D), bf16),
            *wset, *wset,
            pltpu.VMEM((B, Sq, 2 * D), f32),
            pltpu.VMEM((B, Sq, 2 * D), bf16),
            pltpu.VMEM((NPS, 2, Sq // 2, 768), i32),
            pltpu.VMEM((2, 4, Sq // 2, 512), i32),
            pltpu.VMEM((ng, 2, 4, Sq // 2, 512), i32),
            pltpu.VMEM((2, 7, Sq // 4, 9 * 128), i32),
            pltpu.VMEM((2, 4, Sq // 2, hw), i32),
            pltpu.SMEM((1,), i32),
            pltpu.SemaphoreType.DMA((2, ng)),
            pltpu.SemaphoreType.DMA((NKV,)),
            pltpu.SemaphoreType.DMA((NKV,)),
            pltpu.SemaphoreType.DMA((NKV,)),
            pltpu.SemaphoreType.DMA((2,)),
            pltpu.SemaphoreType.DMA((ng,)),
            pltpu.SemaphoreType.DMA(()),
        ],
        compiler_params=pltpu.CompilerParams(
            vmem_limit_bytes=116 * 1024 * 1024,
            disable_bounds_checks=True,
        ),
    )(A_x, akt, avt, awq, awo, B_x, bkt, bvt, bwq, bwo)
```

```python
import functools
import math

import jax
import jax.numpy as jnp
import jax.experimental.pallas as pl
import jax.experimental.pallas.tpu as pltpu

_NN = (((1,), (0,)), ((), ()))
_NT = (((1,), (1,)), ((), ()))
bf16 = jnp.bfloat16
f32 = jnp.float32
i32 = jnp.int32

CH = 16
DEP = 3
NKV = 3
NPS = 4

_SEQ_FULL = ('q00 w0 q01 s01 w1 q02 p01 w2 s02 w3 q03 p02 s00 p00 q10 s03 q11 o01 '
             's11 q12 q13 p03 o00 o02 p11 s12 o03 s10 o10 p12 s13 p10 o11 p13 o12 o13')
_SEQ_NOQ = ('s01 s02 p01 w1 s00 p02 p00 s03 o01 w0 s11 w2 p03 s12 p11 p12 o00 o02 '
            's10 o11 w3 p10 s13 o03 p13 o10 o12 o13')
_SEQ_Q = 'x1 r00 v0 r01 q02 v1 q03 r10 r11 x0 q12 q13'


def _dot(a, b, dims=_NN):
    return jax.lax.dot_general(a, b, dims, preferred_element_type=f32)


def _recip(l):
    r = pl.reciprocal(l, approx=True)
    return r * (2.0 - l * r)


def _col(x, i):
    return x[:, 128 * i:128 * (i + 1)]


def _pack(x):
    return pltpu.bitcast(x.astype(bf16), i32)


def _unpack(x):
    return pltpu.bitcast(x, bf16)


def _cat(xs, axis):
    return jnp.concatenate(list(xs), axis=axis)


def _or_tiles(vals):
    t = None
    for v in vals:
        for r in range(0, v.shape[0], 8):
            for c in range(0, v.shape[1], 128):
                x = v[r:r + 8, c:c + 128]
                t = x if t is None else t | x
    return t


def _lane_lo(rows):
    return jax.lax.broadcasted_iota(i32, (rows, 128), 1) < 64


def _lhs_combos(a11, a12, a21, a22):
    return (a11 + a22, a21 + a22, a11, a22, a11 + a12, a21 - a11, a12 - a22)


def _rhs_combos(b11, b12, b21, b22):
    return (b11 + b22, b11, b12 - b22, b21 - b11, b22, b11 + b12, b21 + b22)


def _weights(xa, xb, xc):
    h = xa.shape[1] // 2
    xa, xb, xc = xa.astype(f32), xb.astype(f32), xc.astype(f32)
    return (_cat([xa[:, :h], xb[:, :h] - xb[:, h:]], 0),
            _cat([xa[:, h:], xc[:, h:] - xc[:, :h]], 0),
            _cat([xc[:, :h], xb[:, h:]], 0))


def _pair_weights(t0, t1):
    return (_weights(t0[:64], t0[64:128], t0[128:]), _weights(t1[64:128], t1[128:], t1[:64]))


def _scores(q_ref, kt0, kt1, lhs):
    t0, t1, t2, rot = (q_ref[:, 128 * k:128 * (k + 1)] for k in range(4))
    lo = _lane_lo(t0.shape[0])
    q = ((t0, jnp.where(lo, t0, rot), jnp.where(lo, t1, t0)),
         (t2, jnp.where(lo, t2, t1), jnp.where(lo, rot, t2)))
    w = _pair_weights(kt0, kt1)
    p = {}

    def run(h, k, i):
        y = _dot(lhs(q[h][k]), _col(w[h][k], i).astype(bf16))
        p[h, k, i] = y if k == 2 else y + p[h, 2, i]

    for t, (h, i) in enumerate(((0, 0), (0, 1), (1, 0))):
        run(h, 2, i), run(h, 0, i), run(h, 1, i), run(1, (2, 0, 1)[t], 1)
    return tuple(_cat([p[h, 0, 0], p[h, 0, 1], p[h, 1, 0], p[h, 1, 1]], 1) for h in range(2))


def _softmax_terms(s, p_ref, zero):
    ls, toks = [], []
    for c in range(s.shape[0] // CH):
        sc = s[c * CH:(c + 1) * CH]
        m = jnp.broadcast_to(jnp.max(sc, axis=-1, keepdims=True), (CH, 128))
        if c >= DEP:
            t = toks[c - DEP] & zero
            m = pltpu.bitcast(pltpu.bitcast(m, i32) | _cat([t, t], 0), f32)
        e = [jnp.exp2(_col(sc, k) - m) for k in range(4)]
        t0, t1 = e[0] + e[2], e[1] + e[3]
        ls.append(jnp.broadcast_to(jnp.sum(t0 + t1, axis=-1, keepdims=True), (CH, 128)))
        rows = slice(c * CH // 2, (c + 1) * CH // 2)
        for k, x in enumerate(e + [t0, t1]):
            p_ref[rows, 128 * k:128 * (k + 1)] = _pack(x)
        toks.append(_or_tiles([p_ref[rows, :]]))
    return ls


def _attend(s, vt0, vt1, p_ref, zero, lhs, sink):
    ls = [_softmax_terms(s[h], p_ref.at[h], zero) for h in range(2)]
    w = _pair_weights(vt0, vt1)
    r = {}
    for h, k in ((0, 0), (0, 1), (0, 2), (1, 1), (1, 2), (1, 0)):
        r[h, k] = _dot(lhs(p_ref.at[h][:, 256 * k:256 * (k + 1)]), w[h][k].astype(bf16), _NT)
    lo = _lane_lo(CH)

    def rows(c):
        p1, p2, p3, u1, u2, u3 = (r[h, k][c * CH:(c + 1) * CH] for h in range(2) for k in range(3))
        r0, r1 = _recip(ls[0][c]), _recip(ls[1][c])
        o_lo = p1 + jnp.where(lo, p2, p3)
        o_hi = u1 + jnp.where(lo, u2, u3)
        mid = jnp.where(lo, p3, u2) + pltpu.roll(jnp.where(lo, u3, p2), 64, 1)
        return _cat([o_lo * r0, mid * jnp.where(lo, r0, r1), o_hi * r1], 1)

    n = len(ls[0]) // 2
    for c in range(n):
        sink(c, rows(c), rows(c + n))


def _kernel(ax, akt, avt, awq, awo, bx, bkt, bvt, bwq, bwo, out,
            xbuf, xca, xcb, x4a, x4b, kvbuf, rq, ro, rq0, ro0,
            wqc0, wq40, woc0, wo40, wqc1, wq41, woc1, wo41,
            acc, obuf, pbuf, qbuf, qall, oc, oraw, zref,
            xsem, kvsem, rqsem, rosem, isem, vsem, osem,
            *, scale, d, sq, nbatch, npass, dh):
    ng = nbatch // 2
    nsteps = npass * ng
    gw, hw = 4 * dh, 2 * dh
    wr = 128 // ng
    hq = sq // 4
    xs, wqs, wos = (ax, bx), (awq, bwq), (awo, bwo)
    kvs = (akt, avt, bkt, bvt)
    xc, x4 = (xca, xcb), (x4a, x4b)
    wsets = ((wqc0, wq40, woc0, wo40), (wqc1, wq41, woc1, wo41))

    def wait_all(ref, sem):
        pltpu.make_async_copy(ref, ref, sem).wait()

    def fetch(pp, gg, slot, live=True):
        def start(src, dst, sem):
            pl.when(live)(lambda: pltpu.make_async_copy(src, dst, sem).start())

        for t in range(4):
            start(kvs[t].at[pl.ds(gg * 2, 2), pl.ds(4 * pp, 4)], kvbuf.at[slot, t], kvsem.at[slot])
        pw = jnp.minimum(pp + 1, npass - 1)
        rows = pl.ds(pl.multiple_of(gg * wr, 16), wr)
        for j in range(2):
            for t in range(5):
                start(wqs[j].at[t, rows, pl.ds(pl.multiple_of(pw * gw, 128), gw)],
                      rq.at[slot, j, t], rqsem.at[slot])
            start(wos[j].at[pw, :, rows], ro.at[slot, j], rosem.at[slot])

    def fetch_wait(slot):
        wait_all(kvbuf.at[slot], kvsem.at[slot])
        wait_all(rq.at[slot], rqsem.at[slot])
        wait_all(ro.at[slot], rosem.at[slot])

    def x_copy(j, gg):
        return pltpu.make_async_copy(xs[j].at[pl.ds(gg * 2, 2)], xbuf.at[j, gg], xsem.at[j, gg])

    def build_x(j, gg):
        back = []
        for r in range(0, sq, 32):
            x0 = xbuf.at[j, gg, 0][r:r + 32, :].astype(f32)
            x1 = xbuf.at[j, gg, 1][r:r + 32, :].astype(f32)
            rows = slice(r // 2, r // 2 + 16)
            cs = _lhs_combos(x0[:, :256], x0[:, 256:512], x1[:, :256], x1[:, 256:512])
            for k, c in enumerate(cs):
                xc[j].at[gg, k][rows, :] = _pack(c)
            x4[j].at[gg][rows, :] = _pack(_cat([x0[:, 512:], x1[:, 512:]], 1))
            back += [xc[j].at[gg, k][rows, :] for k in range(7)] + [x4[j].at[gg][rows, :]]
        return back

    def build_wq(j, gg, raw, wset):
        wqc, wq4, _, _ = wset
        kt = [raw(t).astype(f32) for t in range(5)]
        l1 = [_rhs_combos(kt[t][:, :hw], kt[t][:, hw:], kt[2 + t][:, :hw], kt[2 + t][:, hw:])
              for t in range(2)]
        rows = pl.ds(pl.multiple_of(gg * (wr // 2), 8), wr // 2)
        for k in range(7):
            wqc.at[j, k][rows, :] = _pack(_cat([l1[0][k], l1[1][k]], 1))
        wq4.at[j][rows, :] = _pack(kt[4])
        return [wqc.at[j, k][rows, :] for k in range(7)] + [wq4.at[j][rows, :]]

    def build_wo(j, gg, raw, wset):
        _, _, woc, wo4 = wset
        kt = [raw(t).astype(f32) for t in range(6)]
        l1 = [_rhs_combos(kt[3 + t][:, :256], kt[3 + t][:, 256:512], kt[t][:, :256], kt[t][:, 256:512])
              for t in range(3)]
        rows = pl.ds(pl.multiple_of(gg * (wr // 2), 8), wr // 2)
        back = []
        for k in range(7):
            b = [[_col(l1[t][k], n) for n in range(2)] for t in range(3)]
            if k == 2:
                tiles = [b[t][n] for n in range(2) for t in range(3)]
            else:
                tiles = list(_rhs_combos(b[0][0], b[0][1], b[1][0], b[1][1])) + b[2]
            cols = slice(0, 128 * len(tiles))
            woc.at[j, k][rows, cols] = _pack(_cat(tiles, 1))
            back.append(woc.at[j, k][rows, cols])
        wo4.at[j][rows, :] = _pack(_cat([x[:, 512:] for x in kt], 1))
        return back + [wo4.at[j][rows, :]]

    def compute(seq, g, slot, par, q_ref, first, write_out, last=None):
        wqc, wq4, woc, wo4 = wsets[par]
        s, qm, om, toks = {}, {}, {}, []
        zero = jnp.full((8, 128), zref[0], i32)

        def lhs(x):
            if toks:
                t = toks.pop(0) & zero
                x = _cat([x[:8] | _cat([t] * (x.shape[1] // 128), 1), x[8:]], 0)
            return _unpack(x)

        def q_m(j, k, n):
            x, w = xc[j].at[g, k], wqc.at[j, k]
            qm[j, k, n] = (_dot(lhs(x[:, :128]), _unpack(w[:, 128 * n:128 * (n + 1)]))
                           + _dot(lhs(x[:, 128:]), _unpack(w[:, hw + 128 * n:hw + 128 * (n + 1)])))

        def q_k(j, u, n):
            col = (u % 2) * hw + 128 * n
            qm[j, 'k', u, n] = _dot(lhs(x4[j].at[g][:, 128 * (u // 2):128 * (u // 2 + 1)]),
                                    _unpack(wq4.at[j][:, col:col + 128]))

        def q_fin(j, u):
            for n in range(3):
                m = lambda k: qm[j, k, n]
                kk = qm[j, 'k', u, n]
                y = (lambda: (m(0) + kk) + m(6) + (m(3) - m(4)), lambda: m(2) + m(4) + kk,
                     lambda: m(1) + m(3) + kk, lambda: (m(0) + kk) + m(5) + (m(2) - m(1)))[u]()
                y = y * scale
                q_ref.at[j, u][:, 128 * n:128 * (n + 1)] = _pack(y)
                if n == 1:
                    q_ref.at[j, u][:, 384:] = _pack(pltpu.roll(y, 64, 1))

        def q_piece(j, part):
            if part < 2:
                for n in range(3):
                    q_m(j, (2, 1)[part], n), q_m(j, (4, 3)[part], n)
                for a in (((0, 1, 0), (0, 1, 1), (0, 1, 2), (0, 2, 0)),
                          ((0, 2, 1), (0, 2, 2), (1, 1, 0), (1, 1, 1)),
                          ((1, 1, 2), (1, 2, 0), (1, 2, 1), (1, 2, 2)), ())[2 * j + part]:
                    q_k(*a)
                q_fin(j, 1 + part)
            elif part == 2:
                for n in range(3):
                    q_m(j, 0, n), q_k(j, 0, n), q_k(j, 3, n)
            else:
                for n in range(3):
                    q_m(j, 6, n), q_m(j, 5, n)
                q_fin(j, 0)
                q_fin(j, 3)

        def r_piece(j, part):
            for n in range(3):
                q_m(j, (2, 1)[part], n), q_m(j, (4, 3)[part], n)
            for n in range(3):
                q_k(j, 1 + part, n)
            q_fin(j, 1 + part)

        def x_piece(j):
            if j == 1:
                build_x(1, g)
            else:
                toks.append(_or_tiles(build_x(0, jnp.minimum(g + 1, ng - 1))))

        def v_piece(j):
            toks.append(_or_tiles(build_wo(j, g, lambda t: ro0[g, j, t], wsets[0])))

        def kv(j, which, u):
            return tuple(kvbuf[slot, 2 * j + which, u // 2, 2 * (u % 2) + h] for h in range(2))

        def s_piece(j, u):
            s[j, u] = _scores(q_ref.at[j, u], *kv(j, 0, u), lhs)

        def p_piece(j, u):
            def sink(c, *o):
                rows = [slice(h * hq + c * CH // 2, h * hq + (c + 1) * CH // 2) for h in range(2)]
                prev = lambda v: [_unpack(oraw.at[j, v][rows[h], :]).astype(f32) for h in range(2)]
                add = lambda x, y: [x[h] + y[h] for h in range(2)]
                sub = lambda x, y: [x[h] - y[h] for h in range(2)]
                for h in range(2):
                    oraw.at[j, u][rows[h], :] = _pack(o[h])
                new = {1: lambda: {},
                       2: lambda: {3: o, 0: add(prev(1), o)},
                       0: lambda: {4: add(prev(1), o), 6: sub(o, prev(2))},
                       3: lambda: {1: add(o, prev(2)), 5: sub(o, prev(1))}}[u]()
                for k, v in new.items():
                    cs = _lhs_combos(_col(v[0], 0), _col(v[0], 1), _col(v[1], 0), _col(v[1], 1))
                    blocks = [cs[t] for t in (0, 1, 4, 5, 6)]
                    if k != 3:
                        blocks += [cs[2], cs[3], _col(v[0], 2), _col(v[1], 2)]
                    oc.at[j, k][rows[0], :128 * len(blocks)] = _pack(_cat(blocks, 1))

            _attend(s.pop((j, u)), *kv(j, 1, u), pbuf.at[(1, 2, 0, 3).index(u)], zero, lhs, sink)

        def emit(j, i, col, y):
            b = 2 * g + i
            cols = slice(j * d + col, j * d + col + 128)
            if not first:
                y = y + acc[b, :, cols]
            acc[b, :, cols] = y
            if write_out:
                obuf[b, :, cols] = y.astype(bf16)

        def o_w(j, k, t):
            return _unpack(woc.at[j, k][:, 128 * t:128 * (t + 1)])

        def o_m(j, k):
            def blk(t):
                if k == 3 and t in (2, 3, 7, 8):
                    h, kt = {2: (0, 0), 3: (1, 1), 7: (0, 2), 8: (1, 2)}[t]
                    return oraw.at[j, 2][h * hq:(h + 1) * hq, 128 * kt:128 * (kt + 1)]
                pos = (0, 1, 4, 5, 6, 2, 3, 7, 8).index(t)
                return oc.at[j, k][:, 128 * pos:128 * (pos + 1)]

            mm = lambda t: _dot(lhs(blk(t)), o_w(j, k, t))
            kk = lambda h, n: _dot(lhs(blk(7 + h)), o_w(j, k, 7 + n))
            m2, m4, k01, m0 = mm(2), mm(4), kk(0, 1), mm(0)
            m1, m3, k10, m6 = mm(1), mm(3), kk(1, 0), mm(6)
            k00, m5, k11 = kk(0, 0), mm(5), kk(1, 1)
            om[j, k, 0] = _cat([((m0 - m4) + (m3 + m6)) + k00, m1 + m3 + k10], 0)
            om[j, k, 1] = _cat([m2 + m4 + k01, ((m0 + m2) - m1) + (m5 + k11)], 0)

        def o_n(j, i, t, half=None):
            x = oraw.at[j, 2 * i + t // 3][:, 128 * (t % 3):128 * (t % 3 + 1)]
            w = _unpack(wo4.at[j][:, 128 * t:128 * (t + 1)])
            if half is None:
                y = _dot(lhs(x), w)
                parts = {h: y[h * 2 * hq:(h + 1) * 2 * hq] for h in range(2)}
            else:
                parts = {half: _dot(lhs(x[half * hq:(half + 1) * hq]), w)}
            for h, y in parts.items():
                om[j, 'n', i, h] = om[j, 'n', i, h] + y if (j, 'n', i, h) in om else y

        def emit_n(j, i):
            emit(j, i, 512, _cat([om[j, 'n', i, h] for h in range(2)], 0))

        def flush(i):
            if write_out:
                @pl.when(last)
                def _():
                    pltpu.make_async_copy(obuf.at[2 * g + i], out.at[2 * g + i], osem).start()

        def o_piece(j, part):
            m = lambda k, c: om[j, k, c]
            if part == 0:
                for c in range(2):
                    om[j, 2, c] = _dot(lhs(oraw[j, 1]), _cat([o_w(j, 2, 3 * c + t) for t in range(3)], 0))
                o_n(j, 0, 3), o_n(j, 0, 4)
                return
            ka, kb = ((0, 3), (4, 6), (1, 5))[part - 1]
            o_m(j, ka), o_n(j, 1, part - 1, 0)
            o_m(j, kb), o_n(j, 1, part - 1, 1)
            if part == 2:
                for c in range(2):
                    emit(j, 0, 256 + 128 * c, m(2, c) + m(4, c))
                    emit(j, 0, 128 * c, (m(0, c) + m(3, c) - m(4, c)) + m(6, c))
                for t in (5, 0, 1, 2):
                    o_n(j, 0, t)
                emit_n(j, 0)
                if j == 1:
                    flush(0)
            elif part == 3:
                for c in range(2):
                    emit(j, 1, 128 * c, m(1, c) + m(3, c))
                    emit(j, 1, 256 + 128 * c, (m(0, c) + m(2, c) - m(1, c)) + m(5, c))
                if j == 0:
                    for t in (3, 4):
                        o_n(0, 1, t, 0), o_n(0, 1, t, 1)
                else:
                    o_n(0, 1, 5)
                    emit_n(0, 1)
                    for t in (3, 4, 5):
                        o_n(1, 1, t)
                    emit_n(1, 1)
                    flush(1)

        def w_piece(k):
            j = k // 2
            back = (build_wq(j, g, lambda t: rq[slot, j, t], wsets[1 - par]) if k % 2 == 0
                    else build_wo(j, g, lambda t: ro[slot, j, t], wsets[1 - par]))
            toks.append(_or_tiles(back))

        run = {'q': q_piece, 's': s_piece, 'p': p_piece, 'o': o_piece, 'w': w_piece,
               'r': r_piece, 'x': x_piece, 'v': v_piece}
        for tok in seq.split():
            run[tok[0]](*(int(ch) for ch in tok[1:]))

    def run_pass(p, par, first, slot0):
        def step(g, slot):
            fetch_wait(slot)

            wrap = g + 2 >= ng
            fetch(jnp.minimum(jnp.where(wrap, p + 1, p), npass - 1),
                  jnp.where(wrap, g + 2 - ng, g + 2), jnp.where(slot == 0, NKV - 1, slot - 1),
                  p * ng + g + 2 < nsteps)

            if first:
                compute(_SEQ_NOQ, g, slot, par, qall.at[g], True, False)
            else:
                compute(_SEQ_FULL, g, slot, par, qbuf, False, par == 1, p == npass - 1)
            return jnp.where(slot == NKV - 1, 0, slot + 1)

        jax.lax.fori_loop(0, ng, step, slot0)

    def wq_init(j):
        return pltpu.make_async_copy(wqs[j].at[:, :, pl.ds(0, gw)], rq0.at[j], isem.at[j])

    zref[0] = 0
    x_copy(0, 0).start()
    wq_init(0).start()
    x_copy(0, 0).wait()
    wq_init(1).start()
    build_x(0, 0)
    for j in range(2):
        wq_init(j).wait()
        if j == 0:
            for gg in range(ng):
                x_copy(1, gg).start()
                for jj in range(2):
                    pltpu.make_async_copy(wos[jj].at[0, :, pl.ds(gg * wr, wr)], ro0.at[gg, jj],
                                          vsem.at[gg]).start()
                if gg + 1 < ng:
                    x_copy(0, gg + 1).start()

        def init_wq(gg, carry, j=j):
            rows = pl.ds(pl.multiple_of(gg * wr, 16), wr)
            build_wq(j, gg, lambda t: rq0.at[j, t][rows, :], wsets[0])
            return carry

        jax.lax.fori_loop(0, ng, init_wq, 0)

    def q_step(g, carry):
        x_copy(1, g).wait()
        wait_all(ro0.at[g], vsem.at[g])

        @pl.when(g + 1 < ng)
        def _():
            x_copy(0, g + 1).wait()

        @pl.when(g == 1)
        def _():
            fetch(0, 0, 0)

        @pl.when(g == 4)
        def _():
            fetch(0, 1, 1)

        compute(_SEQ_Q, g, 0, 0, qall.at[g], True, False)
        return carry

    jax.lax.fori_loop(0, ng, q_step, 0)

    run_pass(0, 0, True, 0)

    def pass_pair(pp, carry):
        run_pass(2 * pp + 1, 1, False, ((2 * pp + 1) * ng) % NKV)

        @pl.when(2 * pp + 2 < npass)
        def _():
            run_pass(2 * pp + 2, 0, False, ((2 * pp + 2) * ng) % NKV)

        return carry

    jax.lax.fori_loop(0, npass // 2, pass_pair, 0)
    wait_all(out, osem)


@jax.jit
def pallas_concat_heads__gqa_block_cached__mha_block_cached__near_ridge_kernel(
    A_x: jax.Array,
    A_k_cache: jax.Array,
    A_v_cache: jax.Array,
    A_wq: jax.Array,
    A_wo: jax.Array,
    B_x: jax.Array,
    B_k_cache: jax.Array,
    B_v_cache: jax.Array,
    B_wq: jax.Array,
    B_wo: jax.Array,
):
    B, Sq, D = A_x.shape
    _, H, Sk, Dh = A_k_cache.shape
    assert (B, Sq, D, H, Sk, Dh) == (16, 160, 640, 32, 512, 192)
    npass, ng = H // 4, B // 2
    gw, hw = 4 * Dh, 2 * Dh
    scale = (Dh ** -0.5) * math.log2(math.e)

    akt, avt, bkt, bvt = (jnp.swapaxes(t, 2, 3) for t in
                          (A_k_cache, A_v_cache, B_k_cache, B_v_cache))
    awq, bwq = (w.reshape(5, 128, H * Dh) for w in (A_wq, B_wq))
    awo, bwo = (w.reshape(npass, 6, 128, D) for w in (A_wo, B_wo))
    any_spec = pl.BlockSpec(memory_space=pl.ANY)
    wset = [
        pltpu.VMEM((2, 7, 64, 2 * hw), i32),
        pltpu.VMEM((2, 64, gw), i32),
        pltpu.VMEM((2, 7, 64, 9 * 128), i32),
        pltpu.VMEM((2, 64, 6 * 128), i32),
    ]

    return pl.pallas_call(
        functools.partial(_kernel, scale=scale, d=D, sq=Sq, nbatch=B, npass=npass, dh=Dh),
        in_specs=[any_spec] * 10,
        out_specs=any_spec,
        out_shape=jax.ShapeDtypeStruct((B, Sq, 2 * D), A_x.dtype),
        scratch_shapes=[
            pltpu.VMEM((2, ng, 2, Sq, D), bf16),
            pltpu.VMEM((ng, 7, Sq // 2, 256), i32),
            pltpu.VMEM((ng, 7, Sq // 2, 256), i32),
            pltpu.VMEM((ng, Sq // 2, 256), i32),
            pltpu.VMEM((ng, Sq // 2, 256), i32),
            pltpu.VMEM((NKV, 4, 2, 4, Dh, Sk), bf16),
            pltpu.VMEM((NKV, 2, 5, 128 // ng, gw), bf16),
            pltpu.VMEM((NKV, 2, 6, 128 // ng, D), bf16),
            pltpu.VMEM((2, 5, 128, gw), bf16),
            pltpu.VMEM((ng, 2, 6, 128 // ng, D), bf16),
            *wset, *wset,
            pltpu.VMEM((B, Sq, 2 * D), f32),
            pltpu.VMEM((B, Sq, 2 * D), bf16),
            pltpu.VMEM((NPS, 2, Sq // 2, 768), i32),
            pltpu.VMEM((2, 4, Sq // 2, 512), i32),
            pltpu.VMEM((ng, 2, 4, Sq // 2, 512), i32),
            pltpu.VMEM((2, 7, Sq // 4, 9 * 128), i32),
            pltpu.VMEM((2, 4, Sq // 2, hw), i32),
            pltpu.SMEM((1,), i32),
            pltpu.SemaphoreType.DMA((2, ng)),
            pltpu.SemaphoreType.DMA((NKV,)),
            pltpu.SemaphoreType.DMA((NKV,)),
            pltpu.SemaphoreType.DMA((NKV,)),
            pltpu.SemaphoreType.DMA((2,)),
            pltpu.SemaphoreType.DMA((ng,)),
            pltpu.SemaphoreType.DMA(()),
        ],
        compiler_params=pltpu.CompilerParams(
            vmem_limit_bytes=116 * 1024 * 1024,
            disable_bounds_checks=True,
            disable_semaphore_checks=True,
        ),
    )(A_x, akt, avt, awq, awo, B_x, bkt, bvt, bwq, bwo)
```

```python
import functools
import math

import jax
import jax.numpy as jnp
import jax.experimental.pallas as pl
import jax.experimental.pallas.tpu as pltpu

_NN = (((1,), (0,)), ((), ()))
_NT = (((1,), (1,)), ((), ()))
bf16 = jnp.bfloat16
f32 = jnp.float32
i32 = jnp.int32

CH = 16
DEP = 3
NKV = 3
NPS = 4

_SEQ_FULL = ('q00 w0 q01 q02 w2 w1 s01 p01 s02 q03 q10 p02 w3 q11 s00 p00 q12 s03 '
             'o01 p03 s11 o00 p11 q13 o02 s12 o03 o10 s10 p12 s13 p10 o11 p13 o12 o13')
_SEQ_NOQ = ('s01 s02 p01 w1 s00 p02 p00 s03 o01 w0 s11 w2 p03 s12 p11 p12 o00 o02 '
            's10 o11 w3 p10 s13 o03 p13 o10 o12 o13')
_SEQ_Q = 'x1 r00 v0 r01 r02 v1 r03 r10 r11 x0 r12 r13'


def _dot(a, b, dims=_NN):
    return jax.lax.dot_general(a, b, dims, preferred_element_type=f32)


def _recip(l):
    r = pl.reciprocal(l, approx=True)
    return r * (2.0 - l * r)


def _col(x, i):
    return x[:, 128 * i:128 * (i + 1)]


def _pack(x):
    return pltpu.bitcast(x.astype(bf16), i32)


def _unpack(x):
    return pltpu.bitcast(x, bf16)


def _cat(xs, axis):
    return jnp.concatenate(list(xs), axis=axis)


def _or_tiles(vals):
    t = None
    for v in vals:
        for r in range(0, v.shape[0], 8):
            for c in range(0, v.shape[1], 128):
                x = v[r:r + 8, c:c + 128]
                t = x if t is None else t | x
    return t


def _lane_lo(rows):
    return jax.lax.broadcasted_iota(i32, (rows, 128), 1) < 64


def _lhs_combos(a11, a12, a21, a22):
    return (a11 + a22, a21 + a22, a11, a22, a11 + a12, a21 - a11, a12 - a22)


def _rhs_combos(b11, b12, b21, b22):
    return (b11 + b22, b11, b12 - b22, b21 - b11, b22, b11 + b12, b21 + b22)


_HK = (
    ({(0, 0): 1, (0, 1): 1, (1, 0): -1}, {(1, 0): 1, (0, 1): 1}, {(0, 0): 1, (1, 0): 1, (1, 1): -1}),
    ({(0, 1): 1}, {(0, 1): -1, (1, 1): 1, (1, 2): 1}, {(0, 1): 1}),
    ({(1, 0): 1}, {(0, 0): 1, (2, 0): -1, (0, 1): 1}, {(0, 0): 1, (1, 0): 1}),
    ({(1, 1): 1}, {(1, 0): 1, (1, 1): 1, (2, 1): -1}, {(1, 1): 1}),
    ({(0, 0): 1, (1, 0): -1}, {(0, 0): 1, (1, 0): -1, (0, 2): 1}, {(0, 0): 1}),
    ({(0, 0): 1, (0, 1): 1}, {(0, 1): -1}, {(0, 0): 1, (1, 0): 1, (0, 1): -1, (1, 1): -1}),
    ({(0, 0): 1, (0, 1): 1, (1, 0): -1, (1, 1): -1}, {(1, 0): -1}, {(1, 0): 1, (1, 1): -1}),
    ({(0, 2): 1, (1, 0): 1}, {(2, 0): 1, (0, 2): 1}, {(0, 0): 1, (1, 2): 1}),
    ({(0, 2): 1}, {(2, 1): 1, (0, 2): -1, (2, 2): 1}, {(0, 2): 1, (1, 2): 1}),
    ({(0, 2): 1, (1, 2): -1}, {(2, 0): -1, (1, 2): 1, (2, 2): -1}, {(1, 2): 1}),
    ({(0, 0): 1, (0, 2): 1}, {(0, 2): -1}, {(0, 0): 1, (0, 2): -1}),
    ({(1, 0): 1, (1, 2): 1}, {(2, 0): 1}, {(1, 0): 1, (1, 2): -1}),
    ({(0, 2): 1, (1, 1): -1, (1, 2): -1}, {(2, 1): 1, (1, 2): 1}, {(0, 1): 1, (0, 2): -1, (1, 2): -1}),
    ({(1, 1): 1, (1, 2): 1}, {(2, 1): 1}, {(0, 1): 1, (1, 1): 1, (0, 2): -1, (1, 2): -1}),
    ({(0, 1): 1, (0, 2): 1, (1, 1): -1, (1, 2): -1}, {(1, 2): -1}, {(0, 1): 1, (0, 2): -1}),
)
_HK_ROUNDS = ((0, 2, 5, 6), (4, 7, 10, 11), (12, 13, 14, 1), (3, 8, 9))


def _signed_sum(terms):
    terms = sorted(terms, key=lambda t: -t[0])
    y = terms[0][1] if terms[0][0] > 0 else -terms[0][1]
    for sg, v in terms[1:]:
        y = y + v if sg > 0 else y - v
    return y


def _weights(xa, xb, xc):
    h = xa.shape[1] // 2
    xa, xb, xc = xa.astype(f32), xb.astype(f32), xc.astype(f32)
    return (_cat([xa[:, :h], xb[:, :h] - xb[:, h:]], 0),
            _cat([xa[:, h:], xc[:, h:] - xc[:, :h]], 0),
            _cat([xc[:, :h], xb[:, h:]], 0))


def _pair_weights(t0, t1):
    return (_weights(t0[:64], t0[64:128], t0[128:]), _weights(t1[64:128], t1[128:], t1[:64]))


def _scores(q_ref, kt0, kt1, lhs):
    t0, t1, t2, rot = (q_ref[:, 128 * k:128 * (k + 1)] for k in range(4))
    lo = _lane_lo(t0.shape[0])
    q = ((t0, jnp.where(lo, t0, rot), jnp.where(lo, t1, t0)),
         (t2, jnp.where(lo, t2, t1), jnp.where(lo, rot, t2)))
    w = _pair_weights(kt0, kt1)
    p = {}

    def run(h, k, i):
        y = _dot(lhs(q[h][k]), _col(w[h][k], i).astype(bf16))
        p[h, k, i] = y if k == 2 else y + p[h, 2, i]

    for t, (h, i) in enumerate(((0, 0), (0, 1), (1, 0))):
        run(h, 2, i), run(h, 0, i), run(h, 1, i), run(1, (2, 0, 1)[t], 1)
    return tuple(_cat([p[h, 0, 0], p[h, 0, 1], p[h, 1, 0], p[h, 1, 1]], 1) for h in range(2))


def _softmax_terms(s, p_ref, zero):
    ls, toks = [], []
    for c in range(s.shape[0] // CH):
        sc = s[c * CH:(c + 1) * CH]
        m = jnp.broadcast_to(jnp.max(sc, axis=-1, keepdims=True), (CH, 128))
        if c >= DEP:
            t = toks[c - DEP] & zero
            m = pltpu.bitcast(pltpu.bitcast(m, i32) | _cat([t, t], 0), f32)
        e = [jnp.exp2(_col(sc, k) - m) for k in range(4)]
        t0, t1 = e[0] + e[2], e[1] + e[3]
        ls.append(jnp.broadcast_to(jnp.sum(t0 + t1, axis=-1, keepdims=True), (CH, 128)))
        rows = slice(c * CH // 2, (c + 1) * CH // 2)
        for k, x in enumerate(e + [t0, t1]):
            p_ref[rows, 128 * k:128 * (k + 1)] = _pack(x)
        toks.append(_or_tiles([p_ref[rows, :]]))
    return ls


def _attend(s, vt0, vt1, p_ref, zero, lhs, sink):
    ls = [_softmax_terms(s[h], p_ref.at[h], zero) for h in range(2)]
    w = _pair_weights(vt0, vt1)
    r = {}
    for h, k in ((0, 0), (0, 1), (0, 2), (1, 1), (1, 2), (1, 0)):
        r[h, k] = _dot(lhs(p_ref.at[h][:, 256 * k:256 * (k + 1)]), w[h][k].astype(bf16), _NT)
    lo = _lane_lo(CH)

    def rows(c):
        p1, p2, p3, u1, u2, u3 = (r[h, k][c * CH:(c + 1) * CH] for h in range(2) for k in range(3))
        r0, r1 = _recip(ls[0][c]), _recip(ls[1][c])
        o_lo = p1 + jnp.where(lo, p2, p3)
        o_hi = u1 + jnp.where(lo, u2, u3)
        mid = jnp.where(lo, p3, u2) + pltpu.roll(jnp.where(lo, u3, p2), 64, 1)
        return _cat([o_lo * r0, mid * jnp.where(lo, r0, r1), o_hi * r1], 1)

    n = len(ls[0]) // 2
    for c in range(n):
        sink(c, rows(c), rows(c + n))


def _kernel(ax, akt, avt, awq, awo, bx, bkt, bvt, bwq, bwo, out,
            xbuf, xca, xcb, kvbuf, rq, ro, rq0, ro0,
            wqc0, woc0, wo40, wqc1, woc1, wo41,
            acc, obuf, pbuf, qbuf, qall, oc, oraw, zref,
            xsem, kvsem, rqsem, rosem, isem, vsem, osem,
            *, scale, d, sq, nbatch, npass, dh):
    ng = nbatch // 2
    nsteps = npass * ng
    gw, hw = 4 * dh, 2 * dh
    wr = 128 // ng
    hq = sq // 4
    xs, wqs, wos = (ax, bx), (awq, bwq), (awo, bwo)
    kvs = (akt, avt, bkt, bvt)
    xc = (xca, xcb)
    wsets = ((wqc0, woc0, wo40), (wqc1, woc1, wo41))

    def wait_all(ref, sem):
        pltpu.make_async_copy(ref, ref, sem).wait()

    def fetch(pp, gg, slot, live=True):
        def start(src, dst, sem):
            pl.when(live)(lambda: pltpu.make_async_copy(src, dst, sem).start())

        for t in range(4):
            start(kvs[t].at[pl.ds(gg * 2, 2), pl.ds(4 * pp, 4)], kvbuf.at[slot, t], kvsem.at[slot])
        pw = jnp.minimum(pp + 1, npass - 1)
        rows = pl.ds(pl.multiple_of(gg * wr, 16), wr)
        for j in range(2):
            for t in range(5):
                start(wqs[j].at[t, rows, pl.ds(pl.multiple_of(pw * gw, 128), gw)],
                      rq.at[slot, j, t], rqsem.at[slot])
            start(wos[j].at[pw, :, rows], ro.at[slot, j], rosem.at[slot])

    def fetch_wait(slot):
        wait_all(kvbuf.at[slot], kvsem.at[slot])
        wait_all(rq.at[slot], rqsem.at[slot])
        wait_all(ro.at[slot], rosem.at[slot])

    def x_copy(j, gg):
        return pltpu.make_async_copy(xs[j].at[pl.ds(gg * 2, 2)], xbuf.at[j, gg], xsem.at[j, gg])

    def build_x(j, gg):
        back = []
        for r in range(0, sq, 16):
            x = [xbuf.at[j, gg, i][r:r + 16, :].astype(f32) for i in range(2)]
            tiles = list(_lhs_combos(_col(x[0], 0), _col(x[0], 1), _col(x[1], 0), _col(x[1], 1)))
            tiles += [_signed_sum([(sg, _col(x[i], 2 + k)) for (i, k), sg in h[0].items()]) for h in _HK]
            rows = slice(r // 2, r // 2 + 8)
            xc[j].at[gg][rows, :] = _pack(_cat(tiles, 1))
            back.append(xc[j].at[gg][rows, :])
        return back

    def build_wq(j, gg, raw, wset):
        wqc = wset[0]
        kt = [raw(t).astype(f32) for t in range(5)]
        tiles = list(_rhs_combos(kt[0][:, :hw], kt[0][:, hw:], kt[1][:, :hw], kt[1][:, hw:]))
        tiles += [_signed_sum([(sg, _col(kt[2 + k], 3 * t + n)) for (k, n), sg in h[1].items()])
                  for t in range(2) for h in _HK]
        rows = pl.ds(pl.multiple_of(gg * (wr // 2), 8), wr // 2)
        wqc.at[j][rows, :] = _pack(_cat(tiles, 1))
        return [wqc.at[j][rows, :]]

    def build_wo(j, gg, raw, wset):
        _, woc, wo4 = wset
        kt = [raw(t).astype(f32) for t in range(6)]
        l1 = [_rhs_combos(kt[3 + t][:, :256], kt[3 + t][:, 256:512], kt[t][:, :256], kt[t][:, 256:512])
              for t in range(3)]
        rows = pl.ds(pl.multiple_of(gg * (wr // 2), 8), wr // 2)
        back = []
        for k in range(7):
            b = [[_col(l1[t][k], n) for n in range(2)] for t in range(3)]
            if k == 2:
                tiles = [b[t][n] for n in range(2) for t in range(3)]
            else:
                tiles = list(_rhs_combos(b[0][0], b[0][1], b[1][0], b[1][1])) + b[2]
            cols = slice(0, 128 * len(tiles))
            woc.at[j, k][rows, cols] = _pack(_cat(tiles, 1))
            back.append(woc.at[j, k][rows, cols])
        wo4.at[j][rows, :] = _pack(_cat([x[:, 512:] for x in kt], 1))
        return back + [wo4.at[j][rows, :]]

    def compute(seq, g, slot, par, q_ref, first, write_out, last=None):
        wqc, woc, wo4 = wsets[par]
        s, qm, om, toks = {}, {}, {}, []
        zero = jnp.full((8, 128), zref[0], i32)

        def lhs(x):
            if toks:
                t = toks.pop(0) & zero
                x = _cat([x[:8] | _cat([t] * (x.shape[1] // 128), 1), x[8:]], 0)
            return _unpack(x)

        def q_dot(j, xt, wt, split=False):
            x = xc[j].at[g][:, 128 * xt:128 * (xt + 1)]
            w = _unpack(wqc.at[j][:, 128 * wt:128 * (wt + 1)])
            if split:
                return _cat([_dot(lhs(x[h * hq:(h + 1) * hq]), w) for h in range(2)], 0)
            return _dot(lhs(x), w)

        def q_m(j, k, n, split=False):
            qm[j, k, n] = q_dot(j, k, 3 * k + n, split)

        def q_h(j, t, rnd):
            res = {m: q_dot(j, 7 + m, 21 + 15 * t + m) for m in _HK_ROUNDS[rnd]}
            for i in range(2):
                for n in range(3):
                    terms = [(_HK[m][2][i, n], y) for m, y in res.items() if (i, n) in _HK[m][2]]
                    if terms:
                        y = _signed_sum(terms)
                        key = (j, 'h', 2 * i + t, n)
                        qm[key] = qm[key] + y if key in qm else y

        def q_fin(j, u):
            for n in range(3):
                m = lambda k: qm[j, k, n]
                hh = qm[j, 'h', u, n]
                y = (lambda: (hh + (m(3) - m(4))) + (m(0) + m(6)), lambda: (m(2) + m(4)) + hh,
                     lambda: (m(1) + m(3)) + hh, lambda: (hh + (m(2) - m(1))) + (m(0) + m(5)))[u]()
                y = y * scale
                q_ref.at[j, u][:, 128 * n:128 * (n + 1)] = _pack(y)
                if n == 1:
                    q_ref.at[j, u][:, 384:] = _pack(pltpu.roll(y, 64, 1))

        def q_piece(j, part, shift=None):
            order = [(2, 0), (4, 0), (2, 1), (4, 1), (2, 2), (4, 2), (1, 0), (3, 0), (1, 1), (3, 1), (1, 2),
                     (3, 2), (0, 0), (6, 0), (5, 0), (0, 1), (6, 1), (5, 1), (0, 2), (6, 2), (5, 2)]
            o = j if shift is None else shift
            if part == 0:
                for k, n in order[o:o + 8]:
                    q_m(j, k, n)
            elif part == 1:
                for rnd in range(4):
                    q_h(j, 1, rnd)
                q_m(j, *order[o + 8])
                q_fin(j, 1)
            elif part == 2:
                for k, n in order[o + 9:o + 13]:
                    q_m(j, k, n)
                for rnd in range(4):
                    q_h(j, 0, rnd)
                q_m(j, *order[o + 13])
                q_fin(j, 2)
            else:
                rest = order[o + 14:]
                for c, (k, n) in enumerate(rest):
                    q_m(j, k, n, split=(o == 1 and c >= 4))
                if j == 0 and shift is None:
                    q_m(1, *order[0])
                q_fin(j, 0)
                q_fin(j, 3)

        def r_piece(j, part):
            q_piece(j, part, 0)

        def x_piece(j):
            if j == 1:
                build_x(1, g)
            else:
                toks.append(_or_tiles(build_x(0, jnp.minimum(g + 1, ng - 1))))

        def v_piece(j):
            toks.append(_or_tiles(build_wo(j, g, lambda t: ro0[g, j, t], wsets[0])))

        def kv(j, which, u):
            return tuple(kvbuf[slot, 2 * j + which, u // 2, 2 * (u % 2) + h] for h in range(2))

        def s_piece(j, u):
            s[j, u] = _scores(q_ref.at[j, u], *kv(j, 0, u), lhs)

        def p_piece(j, u):
            def sink(c, *o):
                rows = [slice(h * hq + c * CH // 2, h * hq + (c + 1) * CH // 2) for h in range(2)]
                prev = lambda v: [_unpack(oraw.at[j, v][rows[h], :]).astype(f32) for h in range(2)]
                add = lambda x, y: [x[h] + y[h] for h in range(2)]
                sub = lambda x, y: [x[h] - y[h] for h in range(2)]
                for h in range(2):
                    oraw.at[j, u][rows[h], :] = _pack(o[h])
                new = {1: lambda: {},
                       2: lambda: {3: o, 0: add(prev(1), o)},
                       0: lambda: {4: add(prev(1), o), 6: sub(o, prev(2))},
                       3: lambda: {1: add(o, prev(2)), 5: sub(o, prev(1))}}[u]()
                for k, v in new.items():
                    cs = _lhs_combos(_col(v[0], 0), _col(v[0], 1), _col(v[1], 0), _col(v[1], 1))
                    blocks = [cs[t] for t in (0, 1, 4, 5, 6)]
                    if k != 3:
                        blocks += [cs[2], cs[3], _col(v[0], 2), _col(v[1], 2)]
                    oc.at[j, k][rows[0], :128 * len(blocks)] = _pack(_cat(blocks, 1))

            _attend(s.pop((j, u)), *kv(j, 1, u), pbuf.at[(1, 2, 0, 3).index(u)], zero, lhs, sink)

        def emit(j, i, col, y):
            b = 2 * g + i
            cols = slice(j * d + col, j * d + col + 128)
            if not first:
                y = y + acc[b, :, cols]
            acc[b, :, cols] = y
            if write_out:
                obuf[b, :, cols] = y.astype(bf16)

        def o_w(j, k, t):
            return _unpack(woc.at[j, k][:, 128 * t:128 * (t + 1)])

        def o_m(j, k):
            def blk(t):
                if k == 3 and t in (2, 3, 7, 8):
                    h, kt = {2: (0, 0), 3: (1, 1), 7: (0, 2), 8: (1, 2)}[t]
                    return oraw.at[j, 2][h * hq:(h + 1) * hq, 128 * kt:128 * (kt + 1)]
                pos = (0, 1, 4, 5, 6, 2, 3, 7, 8).index(t)
                return oc.at[j, k][:, 128 * pos:128 * (pos + 1)]

            mm = lambda t: _dot(lhs(blk(t)), o_w(j, k, t))
            kk = lambda h, n: _dot(lhs(blk(7 + h)), o_w(j, k, 7 + n))
            m2, m4, k01, m0 = mm(2), mm(4), kk(0, 1), mm(0)
            m1, m3, k10, m6 = mm(1), mm(3), kk(1, 0), mm(6)
            k00, m5, k11 = kk(0, 0), mm(5), kk(1, 1)
            om[j, k, 0] = _cat([((m0 - m4) + (m3 + m6)) + k00, m1 + m3 + k10], 0)
            om[j, k, 1] = _cat([m2 + m4 + k01, ((m0 + m2) - m1) + (m5 + k11)], 0)

        def o_n(j, i, t, half=None):
            x = oraw.at[j, 2 * i + t // 3][:, 128 * (t % 3):128 * (t % 3 + 1)]
            w = _unpack(wo4.at[j][:, 128 * t:128 * (t + 1)])
            if half is None:
                y = _dot(lhs(x), w)
                parts = {h: y[h * 2 * hq:(h + 1) * 2 * hq] for h in range(2)}
            else:
                parts = {half: _dot(lhs(x[half * hq:(half + 1) * hq]), w)}
            for h, y in parts.items():
                om[j, 'n', i, h] = om[j, 'n', i, h] + y if (j, 'n', i, h) in om else y

        def emit_n(j, i):
            emit(j, i, 512, _cat([om[j, 'n', i, h] for h in range(2)], 0))

        def flush(i):
            if write_out:
                @pl.when(last)
                def _():
                    pltpu.make_async_copy(obuf.at[2 * g + i], out.at[2 * g + i], osem).start()

        def o_piece(j, part):
            m = lambda k, c: om[j, k, c]
            if part == 0:
                for c in range(2):
                    om[j, 2, c] = _dot(lhs(oraw[j, 1]), _cat([o_w(j, 2, 3 * c + t) for t in range(3)], 0))
                o_n(j, 0, 3), o_n(j, 0, 4)
                return
            ka, kb = ((0, 3), (4, 6), (1, 5))[part - 1]
            o_m(j, ka), o_n(j, 1, part - 1, 0)
            o_m(j, kb), o_n(j, 1, part - 1, 1)
            if part == 2:
                for c in range(2):
                    emit(j, 0, 256 + 128 * c, m(2, c) + m(4, c))
                    emit(j, 0, 128 * c, (m(0, c) + m(3, c) - m(4, c)) + m(6, c))
                for t in (5, 0, 1, 2):
                    o_n(j, 0, t)
                emit_n(j, 0)
                if j == 1:
                    flush(0)
            elif part == 3:
                for c in range(2):
                    emit(j, 1, 128 * c, m(1, c) + m(3, c))
                    emit(j, 1, 256 + 128 * c, (m(0, c) + m(2, c) - m(1, c)) + m(5, c))
                if j == 0:
                    for t in (3, 4):
                        o_n(0, 1, t, 0), o_n(0, 1, t, 1)
                else:
                    o_n(0, 1, 5)
                    emit_n(0, 1)
                    for t in (3, 4, 5):
                        o_n(1, 1, t)
                    emit_n(1, 1)
                    flush(1)

        def w_piece(k):
            j = k // 2
            back = (build_wq(j, g, lambda t: rq[slot, j, t], wsets[1 - par]) if k % 2 == 0
                    else build_wo(j, g, lambda t: ro[slot, j, t], wsets[1 - par]))
            toks.append(_or_tiles(back))

        run = {'q': q_piece, 's': s_piece, 'p': p_piece, 'o': o_piece, 'w': w_piece,
               'r': r_piece, 'x': x_piece, 'v': v_piece}
        for tok in seq.split():
            run[tok[0]](*(int(ch) for ch in tok[1:]))

    def run_pass(p, par, first, slot0):
        def step(g, slot):
            fetch_wait(slot)

            wrap = g + 2 >= ng
            fetch(jnp.minimum(jnp.where(wrap, p + 1, p), npass - 1),
                  jnp.where(wrap, g + 2 - ng, g + 2), jnp.where(slot == 0, NKV - 1, slot - 1),
                  p * ng + g + 2 < nsteps)

            if first:
                compute(_SEQ_NOQ, g, slot, par, qall.at[g], True, False)
            else:
                compute(_SEQ_FULL, g, slot, par, qbuf, False, par == 1, p == npass - 1)
            return jnp.where(slot == NKV - 1, 0, slot + 1)

        jax.lax.fori_loop(0, ng, step, slot0)

    def wq_init(j):
        return pltpu.make_async_copy(wqs[j].at[:, :, pl.ds(0, gw)], rq0.at[j], isem.at[j])

    zref[0] = 0
    x_copy(0, 0).start()
    wq_init(0).start()
    x_copy(0, 0).wait()
    wq_init(1).start()
    build_x(0, 0)
    for j in range(2):
        wq_init(j).wait()
        if j == 0:
            for gg in range(ng):
                x_copy(1, gg).start()
                for jj in range(2):
                    pltpu.make_async_copy(wos[jj].at[0, :, pl.ds(gg * wr, wr)], ro0.at[gg, jj],
                                          vsem.at[gg]).start()
                if gg + 1 < ng:
                    x_copy(0, gg + 1).start()

        def init_wq(gg, carry, j=j):
            rows = pl.ds(pl.multiple_of(gg * wr, 16), wr)
            build_wq(j, gg, lambda t: rq0.at[j, t][rows, :], wsets[0])
            return carry

        jax.lax.fori_loop(0, ng, init_wq, 0)

    def q_step(g, carry):
        x_copy(1, g).wait()
        wait_all(ro0.at[g], vsem.at[g])

        @pl.when(g + 1 < ng)
        def _():
            x_copy(0, g + 1).wait()

        @pl.when(g == 1)
        def _():
            fetch(0, 0, 0)

        @pl.when(g == 4)
        def _():
            fetch(0, 1, 1)

        compute(_SEQ_Q, g, 0, 0, qall.at[g], True, False)
        return carry

    jax.lax.fori_loop(0, ng, q_step, 0)

    run_pass(0, 0, True, 0)

    def pass_pair(pp, carry):
        run_pass(2 * pp + 1, 1, False, ((2 * pp + 1) * ng) % NKV)

        @pl.when(2 * pp + 2 < npass)
        def _():
            run_pass(2 * pp + 2, 0, False, ((2 * pp + 2) * ng) % NKV)

        return carry

    jax.lax.fori_loop(0, npass // 2, pass_pair, 0)
    wait_all(out, osem)


@jax.jit
def pallas_concat_heads__gqa_block_cached__mha_block_cached__near_ridge_kernel(
    A_x: jax.Array,
    A_k_cache: jax.Array,
    A_v_cache: jax.Array,
    A_wq: jax.Array,
    A_wo: jax.Array,
    B_x: jax.Array,
    B_k_cache: jax.Array,
    B_v_cache: jax.Array,
    B_wq: jax.Array,
    B_wo: jax.Array,
):
    B, Sq, D = A_x.shape
    _, H, Sk, Dh = A_k_cache.shape
    assert (B, Sq, D, H, Sk, Dh) == (16, 160, 640, 32, 512, 192)
    npass, ng = H // 4, B // 2
    gw, hw = 4 * Dh, 2 * Dh
    scale = (Dh ** -0.5) * math.log2(math.e)

    akt, avt, bkt, bvt = (jnp.swapaxes(t, 2, 3) for t in
                          (A_k_cache, A_v_cache, B_k_cache, B_v_cache))
    awq, bwq = (w.reshape(5, 128, H * Dh) for w in (A_wq, B_wq))
    awo, bwo = (w.reshape(npass, 6, 128, D) for w in (A_wo, B_wo))
    any_spec = pl.BlockSpec(memory_space=pl.ANY)
    wset = [
        pltpu.VMEM((2, 64, 51 * 128), i32),
        pltpu.VMEM((2, 7, 64, 9 * 128), i32),
        pltpu.VMEM((2, 64, 6 * 128), i32),
    ]

    return pl.pallas_call(
        functools.partial(_kernel, scale=scale, d=D, sq=Sq, nbatch=B, npass=npass, dh=Dh),
        in_specs=[any_spec] * 10,
        out_specs=any_spec,
        out_shape=jax.ShapeDtypeStruct((B, Sq, 2 * D), A_x.dtype),
        scratch_shapes=[
            pltpu.VMEM((2, ng, 2, Sq, D), bf16),
            pltpu.VMEM((ng, Sq // 2, 22 * 128), i32),
            pltpu.VMEM((ng, Sq // 2, 22 * 128), i32),
            pltpu.VMEM((NKV, 4, 2, 4, Dh, Sk), bf16),
            pltpu.VMEM((NKV, 2, 5, 128 // ng, gw), bf16),
            pltpu.VMEM((NKV, 2, 6, 128 // ng, D), bf16),
            pltpu.VMEM((2, 5, 128, gw), bf16),
            pltpu.VMEM((ng, 2, 6, 128 // ng, D), bf16),
            *wset, *wset,
            pltpu.VMEM((B, Sq, 2 * D), f32),
            pltpu.VMEM((B, Sq, 2 * D), bf16),
            pltpu.VMEM((NPS, 2, Sq // 2, 768), i32),
            pltpu.VMEM((2, 4, Sq // 2, 512), i32),
            pltpu.VMEM((ng, 2, 4, Sq // 2, 512), i32),
            pltpu.VMEM((2, 7, Sq // 4, 9 * 128), i32),
            pltpu.VMEM((2, 4, Sq // 2, hw), i32),
            pltpu.SMEM((1,), i32),
            pltpu.SemaphoreType.DMA((2, ng)),
            pltpu.SemaphoreType.DMA((NKV,)),
            pltpu.SemaphoreType.DMA((NKV,)),
            pltpu.SemaphoreType.DMA((NKV,)),
            pltpu.SemaphoreType.DMA((2,)),
            pltpu.SemaphoreType.DMA((ng,)),
            pltpu.SemaphoreType.DMA(()),
        ],
        compiler_params=pltpu.CompilerParams(
            vmem_limit_bytes=116 * 1024 * 1024,
            disable_bounds_checks=True,
            disable_semaphore_checks=True,
        ),
    )(A_x, akt, avt, awq, awo, B_x, bkt, bvt, bwq, bwo)
```

```python
import functools
import math

import jax
import jax.numpy as jnp
import jax.experimental.pallas as pl
import jax.experimental.pallas.tpu as pltpu

_NN = (((1,), (0,)), ((), ()))
_NT = (((1,), (1,)), ((), ()))
bf16 = jnp.bfloat16
f32 = jnp.float32
i32 = jnp.int32

CH = 16
DEP = 3
XPAD = 46
NKV = 3
NPS = 4

_SEQ_FULL = ('q00 w0 q01 q02 w2 w1 s01 p01 s02 q03 p02 q10 s00 q11 p00 w3 s03 p03 '
             'q12 o00 q13 s11 o01 o02 p11 s12 o03 s10 p12 s13 p10 o10 o11 p13 o12 o13')
_SEQ_NOQ = ('s01 s02 p01 s00 p02 o00 p00 s03 w1 o01 s11 w2 p03 s12 w0 p11 p12 o02 '
            's10 w3 o10 o11 p10 s13 o03 p13 o12 o13')
_SEQ_Q = 'x1 q00 v1 q01 q02 q03 v0 x0 q10 q11 q12 q13'


def _dot(a, b, dims=_NN):
    return jax.lax.dot_general(a, b, dims, preferred_element_type=f32)


def _recip(l):
    r = pl.reciprocal(l, approx=True)
    return r * (2.0 - l * r)


def _col(x, i):
    return x[:, 128 * i:128 * (i + 1)]


def _pack(x):
    return pltpu.bitcast(x.astype(bf16), i32)


def _unpack(x):
    return pltpu.bitcast(x, bf16)


def _cat(xs, axis):
    return jnp.concatenate(list(xs), axis=axis)


def _or_tiles(vals):
    t = None
    for v in vals:
        for r in range(0, v.shape[0], 8):
            for c in range(0, v.shape[1], 128):
                x = v[r:r + 8, c:c + 128]
                t = x if t is None else t | x
    return t


def _lane_lo(rows):
    return jax.lax.broadcasted_iota(i32, (rows, 128), 1) < 64


_QPROD = (
    '+00-10 +03+05+04 +03', '+10 +03-43-23 +03+13', '+00-10 -00-02-01 +10',
    '+00 +00-30-10 +00+10', '+01-11 -13-12 +13', '+01 +13-33 +03+13',
    '+01-11 +11+15+14+10 +01', '+11 +11-41-21-01 +01+11', '+02-12 +20+25 +00',
    '+12 +20-40 +00+10', '+02-12 -24-23-22-21 +14', '+02 +24-04-34-14 +04+14',
    '+13 +31 +11', '+03 +31 +01', '+03-13 +32+35+33+30+34 +02',
    '+13 +32-42-12-02-22 +02+12', '+14 +44 +14', '+04 +44 +04',
    '+04-14 -45-40-43-41-42 +15', '+04 +45-25-05-15-35 +05+15', '+04+12 +40+25 +00+15',
    '+02+04 -25 +00-05', '+12+14 +40 +10-15', '+04+10 +43+05 +03+15',
    '+00+04 -05 +03-05', '+10+14 +43 +13-15', '+04+11 +41+15 +01+15',
    '+01+04 -15 +01-05', '+11+14 +41 +11-15', '+04+13 +42+35 +02+15',
    '+03+04 -35 +02-05', '+13+14 +42 +12-15', '+02+10 +23+04 +03+14',
    '+00+02 -04 +03-04', '+10+12 +23 +13-14', '+01+13 +33+12 +02+13',
    '+01+03 +33 +03-02', '+11+13 -12 +13-12', '+00+13 +30+02 +02+10',
    '+00+03 +30 +00-02', '+10+13 -02 +10-12', '+02+13 +34+22 +02+14',
    '+02+03 +34 +04-02', '+12+13 -22 +14-12', '+02+11 +21+14 +01+14',
    '+01+02 -14 +01-04', '+11+12 +21 +11-14', '+00+11 +10+01 +01+10',
    '+00+01 +10 +00-01', '+10+11 -01 +10-11',
)
_QROUNDS = (
    ((~5, ~15, 43, ~36), (~27, ~38, ~30, ~45), (~17, 0, 33, 1), (11, 32, 41, 42), (21, 19, 23, 24),
     (~39, ~46, 22, ~37), (~9, ~8, ~28, ~3), (18, ~2, 40, 31), (49, 7, 47, 12), (48, ~20, 6, 26),
     (~14, 29, ~25, 35), (44, 10, 16, ~13), (4, 34)),
    ((~21, ~5), (~23, ~26, ~11, ~32), (43, ~19, ~46, ~34), (~33, ~17, 45, 0), (~27, ~42, ~1, ~44),
     (36, 30, ~37, 24), (2, 47, 40, 7), (12, 22, 28, 49), (29, 14, 31, 15), (3, ~38, ~9, 39),
     (41, ~16, 10, ~20), (35, 18, ~25, 4), (48, 8, ~13, 6)),
)
_OPROD = (
    '+00 +00+20+10 +00-10', '+00+10 +00-02-04 +10', '+13 -30-40-50 +00-10',
    '+03+13 +30-33-31 +00', '+10 -01-41 +01-11', '+00+10 +01-03 +01',
    '+05 +51+31+21+11 +01-11', '+05+15 +51-50-52-54 +11', '+03 +32+12 +02-12',
    '+03+13 +32-34 +12', '+12 -22-42-52-02 +02-12', '+02+12 +22-23-21-20 +02',
    '+04 +43+03+33+23+13 +03-13', '+04+14 +43-41-40-42-44 +13', '+15 +53 +13',
    '+05 +53 +03', '+11 -14-44-54-34-04 +04-14', '+01+11 +14-13-11-12-10 +04',
    '+12 +24 +14', '+02 +24 +04', '+04+10 +03+41 +01+13',
    '+00-04 +03 +01+03', '+10-14 -41 +11+13', '+04+13 +33+40 +00+13',
    '+03-04 +33 +00+03', '+13-14 -40 +10+13', '+05+13 +31+50 +00+11',
    '+03-05 +31 +00+01', '+13-15 -50 +10+11', '+04+12 +23+42 +02+13',
    '+02-04 +23 +02+03', '+12-14 -42 +12+13', '+05+12 +52+21 +02+11',
    '+05-02 -21 +01+02', '+15-12 +52 +11+12', '+00+12 +02+20 +02+10',
    '+00-02 -20 +00+02', '+10-12 +02 +10+12', '+04+11 +44+13 +04+13',
    '+04-01 -13 +03+04', '+14-11 +44 +13+14', '+05+11 +54+11 +04+11',
    '+05-01 -11 +01+04', '+15-11 +54 +11+14', '+03+11 +34+12 +04+12',
    '+03-01 -12 +02+04', '+13-11 +34 +12+14', '+00+11 +04+10 +04+10',
    '+00-01 -10 +00+04', '+10-11 +04 +10+14',
)
_OROUNDS = (
    ((~8, ~6, ~24, 15), (~38, ~10, ~44, ~29), (~16, ~12, ~49, ~4), (~37, ~20, ~32, ~41), (45, ~17, 11, ~19),
     (21, 36, 30, 33), (~39, ~0, ~47, ~35), (42, 27, 5, 48), (43, 34, ~22, 40), (9, 7, 14, 26),
     (~18, 31, ~46, 13), (25, 3, 2, 23), (1, ~28)),
    ((8, ~6), (12, ~27, ~24, ~15), (~20, ~4, ~41, ~16), (~44, ~10, 18, ~32), (~38, 29, ~37, ~49),
     (~21, ~33, ~48, ~47), (0, 1, 11, 36), (39, ~5, 42, 19), (17, 30, 45, 35), (~26, ~22, ~28, ~40),
     (9, 14, 13, 31), (2, 23, 25, 3), (7, 34, ~46, 43)),
)


def _terms(code):
    return tuple((1 if code[i] == '+' else -1, int(code[i + 1]), int(code[i + 2]))
                 for i in range(0, len(code), 3))


_QX, _QW, _QO = zip(*[[_terms(c) for c in p.split()] for p in _QPROD])
_QXS = sorted(set(_QX))
_OX, _OW, _OO = zip(*[[_terms(c) for c in p.split()] for p in _OPROD])
_ORAW = [((1, i, k),) for i in range(2) for k in range(6)]
_OXS = _ORAW + sorted(set(_OX) - set(_ORAW))
_ARRIVAL = (2, 0, 1, 3)


def _signed_sum(terms):
    if terms[0][0] < 0 and len(terms) > 1 and terms[1][0] > 0:
        terms = [terms[1], terms[0]] + list(terms[2:])
    sg0, y = terms[0]
    for sg, v in terms[1:]:
        if sg0 < 0 and sg > 0:
            sg0, y = 1, v - y
        else:
            y = y + v if sg == sg0 else y - v
    return y if sg0 > 0 else -y


def _weights(xa, xb, xc):
    h = xa.shape[1] // 2
    xa, xb, xc = xa.astype(f32), xb.astype(f32), xc.astype(f32)
    return (_cat([xa[:, :h], xb[:, :h] - xb[:, h:]], 0),
            _cat([xa[:, h:], xc[:, h:] - xc[:, :h]], 0),
            _cat([xc[:, :h], xb[:, h:]], 0))


def _pair_weights(t0, t1):
    return (_weights(t0[:64], t0[64:128], t0[128:]), _weights(t1[64:128], t1[128:], t1[:64]))


def _scores(q_ref, kt0, kt1, lhs):
    t0, t1, t2, rot = (q_ref[:, 128 * k:128 * (k + 1)] for k in range(4))
    lo = _lane_lo(t0.shape[0])
    q = ((t0, jnp.where(lo, t0, rot), jnp.where(lo, t1, t0)),
         (t2, jnp.where(lo, t2, t1), jnp.where(lo, rot, t2)))
    w = _pair_weights(kt0, kt1)
    p = {}

    def run(h, k, i):
        y = _dot(lhs(q[h][k]), _col(w[h][k], i).astype(bf16))
        p[h, k, i] = y if k == 2 else y + p[h, 2, i]

    for t, (h, i) in enumerate(((0, 0), (0, 1), (1, 0))):
        run(h, 2, i), run(h, 0, i), run(h, 1, i), run(1, (2, 0, 1)[t], 1)
    return tuple(_cat([p[h, 0, 0], p[h, 0, 1], p[h, 1, 0], p[h, 1, 1]], 1) for h in range(2))


def _softmax_terms(s, p_ref, zero):
    ls, toks = [], []
    for c in range(s.shape[0] // CH):
        sc = s[c * CH:(c + 1) * CH]
        m = jnp.broadcast_to(jnp.max(sc, axis=-1, keepdims=True), (CH, 128))
        if c >= DEP:
            t = toks[c - DEP] & zero
            m = pltpu.bitcast(pltpu.bitcast(m, i32) | _cat([t, t], 0), f32)
        e = [jnp.exp2(_col(sc, k) - m) for k in range(4)]
        t0, t1 = e[0] + e[2], e[1] + e[3]
        ls.append(jnp.broadcast_to(jnp.sum(t0 + t1, axis=-1, keepdims=True), (CH, 128)))
        rows = slice(c * CH // 2, (c + 1) * CH // 2)
        for k, x in enumerate(e + [t0, t1]):
            p_ref[rows, 128 * k:128 * (k + 1)] = _pack(x)
        toks.append(_or_tiles([p_ref[rows, :]]))
    return ls


def _attend(s, vt0, vt1, p_ref, zero, lhs, sink):
    ls = [_softmax_terms(s[h], p_ref.at[h], zero) for h in range(2)]
    w = _pair_weights(vt0, vt1)
    r = {}
    for h, k in ((0, 0), (0, 1), (0, 2), (1, 1), (1, 2), (1, 0)):
        r[h, k] = _dot(lhs(p_ref.at[h][:, 256 * k:256 * (k + 1)]), w[h][k].astype(bf16), _NT)
    lo = _lane_lo(CH)

    def rows(c):
        p1, p2, p3, u1, u2, u3 = (r[h, k][c * CH:(c + 1) * CH] for h in range(2) for k in range(3))
        r0, r1 = _recip(ls[0][c]), _recip(ls[1][c])
        o_lo = p1 + jnp.where(lo, p2, p3)
        o_hi = u1 + jnp.where(lo, u2, u3)
        mid = jnp.where(lo, p3, u2) + pltpu.roll(jnp.where(lo, u3, p2), 64, 1)
        return _cat([o_lo * r0, mid * jnp.where(lo, r0, r1), o_hi * r1], 1)

    for c in range(len(ls[0])):
        sink(c, rows(c))


def _kernel(ax, akt, avt, awq, awo, bx, bkt, bvt, bwq, bwo, out,
            xbuf, xca, xcb, kvbuf, rq, ro, rq0, ro0,
            wqc0, woc0, wqc1, woc1,
            acc, obuf, pbuf, qbuf, qall, oc, zref,
            xsem, kvsem, rqsem, rosem, isem, vsem, osem,
            *, scale, d, sq, nbatch, npass, dh):
    ng = nbatch // 2
    nsteps = npass * ng
    gw = 4 * dh
    wr = 128 // ng
    xs, wqs, wos = (ax, bx), (awq, bwq), (awo, bwo)
    kvs = (akt, avt, bkt, bvt)
    xc = (xca, xcb)
    wsets = ((wqc0, woc0), (wqc1, woc1))

    def wait_all(ref, sem):
        pltpu.make_async_copy(ref, ref, sem).wait()

    def fetch(pp, gg, slot, live=True):
        def start(src, dst, sem):
            pl.when(live)(lambda: pltpu.make_async_copy(src, dst, sem).start())

        for t in range(4):
            start(kvs[t].at[pl.ds(gg * 2, 2), pl.ds(4 * pp, 4)], kvbuf.at[slot, t], kvsem.at[slot])
        pw = jnp.minimum(pp + 1, npass - 1)
        rows = pl.ds(pl.multiple_of(gg * wr, 16), wr)
        for j in range(2):
            for t in range(5):
                start(wqs[j].at[t, rows, pl.ds(pl.multiple_of(pw * gw, 128), gw)],
                      rq.at[slot, j, t], rqsem.at[slot])
            start(wos[j].at[pw, :, rows], ro.at[slot, j], rosem.at[slot])

    def fetch_wait(slot):
        wait_all(kvbuf.at[slot], kvsem.at[slot])
        wait_all(rq.at[slot], rqsem.at[slot])
        wait_all(ro.at[slot], rosem.at[slot])

    def x_copy(j, gg):
        return pltpu.make_async_copy(xs[j].at[pl.ds(gg * 2, 2)], xbuf.at[j, gg], xsem.at[j, gg])

    def build_x(j, gg):
        back = []
        for r in range(0, sq, 16):
            x = [xbuf.at[j, gg, i][r:r + 16, :].astype(f32) for i in range(2)]
            tiles = [_signed_sum([(sg, _col(x[i], k)) for sg, i, k in f]) for f in _QXS]
            rows = slice(r // 2, r // 2 + 8)
            xc[j].at[gg][rows, :128 * len(tiles)] = _pack(_cat(tiles, 1))
            back.append(xc[j].at[gg][rows, :128 * len(tiles)])
        return back

    def build_wq(j, gg, raw, wset):
        wqc = wset[0]
        kt = [raw(t).astype(f32) for t in range(5)]
        tiles = [_signed_sum([(sg, _col(kt[k], n)) for sg, k, n in f]) for f in _QW]
        rows = pl.ds(pl.multiple_of(gg * (wr // 2), 8), wr // 2)
        wqc.at[j][rows, :] = _pack(_cat(tiles, 1))
        return [wqc.at[j][rows, :]]

    def build_wo(j, gg, raw, wset):
        woc = wset[1]
        kt = [raw(t).astype(f32) for t in range(6)]
        tiles = [_signed_sum([(sg, _col(kt[k], n)) for sg, k, n in f]) for f in _OW]
        rows = pl.ds(pl.multiple_of(gg * (wr // 2), 8), wr // 2)
        woc.at[j][rows, :] = _pack(_cat(tiles, 1))
        return [woc.at[j][rows, :]]

    def compute(seq, g, slot, par, q_ref, first, write_out, last=None):
        wqc, woc = wsets[par]
        s, qm, om = {}, {}, {}
        toks = []
        zero = jnp.full((8, 128), zref[0], i32)

        def lhs(x):
            for e in toks:
                e[0] -= 1
            if toks and toks[0][0] < 0:
                t = toks.pop(0)[1] & zero
                x = _cat([x[:8] | _cat([t] * (x.shape[1] // 128), 1), x[8:]], 0)
            return _unpack(x)

        def gate(delay, vals):
            toks.append([delay, _or_tiles(vals)])
            toks.sort(key=lambda e: e[0])

        def run_round(ids, x_ref, w_ref, xs_, xf, of, state, finish):
            touched = []
            for e in ids:
                m = e if e >= 0 else ~e
                xt = xs_.index(xf[m])
                x = x_ref[:, 128 * xt:128 * (xt + 1)]
                w = _unpack(w_ref[:, 128 * m:128 * (m + 1)])
                y = _dot(lhs(x), w)
                for sg, i, n in of[m]:
                    st = state.setdefault((i, n), [[], sum(o[1:] == (i, n) for f in of for o in f)])
                    st[0].insert(0, (sg, y))
                    st[1] -= 1
                    if (e >= 0 or st[1] == 0) and (i, n) not in touched:
                        touched.append((i, n))
            for i, n in touched:
                st = state[i, n]
                y = _signed_sum(st[0])
                st[0] = [(1, y)]
                if st[1] == 0:
                    finish(i, n, y)

        def q_round(j, ids):
            def finish(i, n, y):
                y = y * scale
                dst = q_ref.at[j, 2 * i + n // 3]
                dst[:, 128 * (n % 3):128 * (n % 3 + 1)] = _pack(y)
                if n % 3 == 1:
                    dst[:, 384:] = _pack(pltpu.roll(y, 64, 1))

            run_round(ids, xc[j].at[g], wqc.at[j], _QXS, _QX, _QO, qm.setdefault(j, {}), finish)

        def q_piece(j, part):
            rounds = _QROUNDS[j]
            cuts = [j + c for c in (0, 2, 5, 9)] + [len(rounds)]
            for r in range(cuts[part], cuts[part + 1]):
                q_round(j, rounds[r])
            if part == 3 and j == 0:
                q_round(1, _QROUNDS[1][0])

        def x_piece(j):
            back = build_x(1, g) if j == 1 else build_x(0, jnp.minimum(g + 1, ng - 1))
            for c, v in enumerate(back):
                gate(9 + 4 * c, [v])

        def v_piece(j):
            gate(-1, build_wo(j, g, lambda t: ro0[g, j, t], wsets[0]))

        def kv(j, which, u):
            return tuple(kvbuf[slot, 2 * j + which, u // 2, 2 * (u % 2) + h] for h in range(2))

        def s_piece(j, u):
            s[j, u] = _scores(q_ref.at[j, u], *kv(j, 0, u), lhs)

        def p_piece(j, u):
            when = lambda i, k: _ARRIVAL[2 * i + k // 3]
            new = [t for t, f in enumerate(_OXS) if max(when(i, k) for _, i, k in f) == _ARRIVAL[u]]

            def sink(c, o):
                rows = slice(c * CH // 2, (c + 1) * CH // 2)
                tile = lambda t: oc.at[j][rows, 128 * t:128 * (t + 1)]
                val = lambda i, k: (_col(o, k % 3) if when(i, k) == _ARRIVAL[u]
                                    else _unpack(tile(6 * i + k)).astype(f32))
                for t in new:
                    y = _signed_sum([(sg, val(i, k)) for sg, i, k in _OXS[t]])
                    oc.at[j][rows, 128 * t:128 * (t + 1)] = _pack(y)

            _attend(s.pop((j, u)), *kv(j, 1, u), pbuf.at[_ARRIVAL[u]], zero, lhs, sink)

        def o_round(j, ids):
            def finish(i, n, y):
                b = 2 * g + i
                cols = slice(j * d + 128 * n, j * d + 128 * (n + 1))
                if not first:
                    y = y + acc[b, :, cols]
                acc[b, :, cols] = y
                if write_out:
                    obuf[b, :, cols] = y.astype(bf16)

            run_round(ids, oc.at[j], woc.at[j], _OXS, _OX, _OO, om.setdefault(j, {}), finish)

        def flush(i):
            if write_out:
                @pl.when(last)
                def _():
                    pltpu.make_async_copy(obuf.at[2 * g + i], out.at[2 * g + i], osem).start()

        def o_piece(j, part):
            rounds = _OROUNDS[j]
            cuts = [j + c for c in (0, 1, 4, 8)] + [len(rounds)]
            for r in range(cuts[part], cuts[part + 1]):
                o_round(j, rounds[r])
            if part == 3:
                if j == 0:
                    o_round(1, _OROUNDS[1][0])
                else:
                    flush(0), flush(1)

        def w_piece(k):
            j = k // 2
            back = (build_wq(j, g, lambda t: rq[slot, j, t], wsets[1 - par]) if k % 2 == 0
                    else build_wo(j, g, lambda t: ro[slot, j, t], wsets[1 - par]))
            gate(-1, back)

        run = {'q': q_piece, 's': s_piece, 'p': p_piece, 'o': o_piece, 'w': w_piece,
               'x': x_piece, 'v': v_piece}
        for tok in seq.split():
            run[tok[0]](*(int(ch) for ch in tok[1:]))

    def run_pass(p, par, first, slot0):
        def step(g, slot):
            fetch_wait(slot)

            wrap = g + 2 >= ng
            fetch(jnp.minimum(jnp.where(wrap, p + 1, p), npass - 1),
                  jnp.where(wrap, g + 2 - ng, g + 2), jnp.where(slot == 0, NKV - 1, slot - 1),
                  p * ng + g + 2 < nsteps)

            if first:
                compute(_SEQ_NOQ, g, slot, par, qall.at[g], True, False)
            else:
                compute(_SEQ_FULL, g, slot, par, qbuf, False, par == 1, p == npass - 1)
            return jnp.where(slot == NKV - 1, 0, slot + 1)

        jax.lax.fori_loop(0, ng, step, slot0)

    def wq_init(j):
        return pltpu.make_async_copy(wqs[j].at[:, :, pl.ds(0, gw)], rq0.at[j], isem.at[j])

    zref[0] = 0
    x_copy(0, 0).start()
    wq_init(0).start()
    x_copy(0, 0).wait()
    wq_init(1).start()
    build_x(0, 0)
    for j in range(2):
        wq_init(j).wait()
        if j == 0:
            for gg in range(ng):
                x_copy(1, gg).start()
                for jj in range(2):
                    pltpu.make_async_copy(wos[jj].at[0, :, pl.ds(gg * wr, wr)], ro0.at[gg, jj],
                                          vsem.at[gg]).start()
                if gg + 1 < ng:
                    x_copy(0, gg + 1).start()

        def init_wq(gg, carry, j=j):
            rows = pl.ds(pl.multiple_of(gg * wr, 16), wr)
            build_wq(j, gg, lambda t: rq0.at[j, t][rows, :], wsets[0])
            return carry

        jax.lax.fori_loop(0, ng, init_wq, 0)

    def q_step(g, carry):
        x_copy(1, g).wait()
        wait_all(ro0.at[g], vsem.at[g])

        @pl.when(g + 1 < ng)
        def _():
            x_copy(0, g + 1).wait()

        @pl.when(g == 1)
        def _():
            fetch(0, 0, 0)

        @pl.when(g == 4)
        def _():
            fetch(0, 1, 1)

        compute(_SEQ_Q, g, 0, 0, qall.at[g], True, False)
        return carry

    jax.lax.fori_loop(0, ng, q_step, 0)

    run_pass(0, 0, True, 0)

    def pass_pair(pp, carry):
        run_pass(2 * pp + 1, 1, False, ((2 * pp + 1) * ng) % NKV)

        @pl.when(2 * pp + 2 < npass)
        def _():
            run_pass(2 * pp + 2, 0, False, ((2 * pp + 2) * ng) % NKV)

        return carry

    jax.lax.fori_loop(0, npass // 2, pass_pair, 0)
    wait_all(out, osem)


@jax.jit
def pallas_concat_heads__gqa_block_cached__mha_block_cached__near_ridge_kernel(
    A_x: jax.Array,
    A_k_cache: jax.Array,
    A_v_cache: jax.Array,
    A_wq: jax.Array,
    A_wo: jax.Array,
    B_x: jax.Array,
    B_k_cache: jax.Array,
    B_v_cache: jax.Array,
    B_wq: jax.Array,
    B_wo: jax.Array,
):
    B, Sq, D = A_x.shape
    _, H, Sk, Dh = A_k_cache.shape
    assert (B, Sq, D, H, Sk, Dh) == (16, 160, 640, 32, 512, 192)
    npass, ng = H // 4, B // 2
    gw = 4 * Dh
    scale = (Dh ** -0.5) * math.log2(math.e)

    akt, avt, bkt, bvt = (jnp.swapaxes(t, 2, 3) for t in
                          (A_k_cache, A_v_cache, B_k_cache, B_v_cache))
    awq, bwq = (w.reshape(5, 128, H * Dh) for w in (A_wq, B_wq))
    awo, bwo = (w.reshape(npass, 6, 128, D) for w in (A_wo, B_wo))
    any_spec = pl.BlockSpec(memory_space=pl.ANY)
    wset = [
        pltpu.VMEM((2, 64, len(_QW) * 128), i32),
        pltpu.VMEM((2, 64, len(_OW) * 128), i32),
    ]

    return pl.pallas_call(
        functools.partial(_kernel, scale=scale, d=D, sq=Sq, nbatch=B, npass=npass, dh=Dh),
        in_specs=[any_spec] * 10,
        out_specs=any_spec,
        out_shape=jax.ShapeDtypeStruct((B, Sq, 2 * D), A_x.dtype),
        scratch_shapes=[
            pltpu.VMEM((2, ng, 2, Sq, D), bf16),
            pltpu.VMEM((ng, Sq // 2, XPAD * 128), i32),
            pltpu.VMEM((ng, Sq // 2, XPAD * 128), i32),
            pltpu.VMEM((NKV, 4, 2, 4, Dh, Sk), bf16),
            pltpu.VMEM((NKV, 2, 5, 128 // ng, gw), bf16),
            pltpu.VMEM((NKV, 2, 6, 128 // ng, D), bf16),
            pltpu.VMEM((2, 5, 128, gw), bf16),
            pltpu.VMEM((ng, 2, 6, 128 // ng, D), bf16),
            *wset, *wset,
            pltpu.VMEM((B, Sq, 2 * D), f32),
            pltpu.VMEM((B, Sq, 2 * D), bf16),
            pltpu.VMEM((NPS, 2, Sq // 2, 768), i32),
            pltpu.VMEM((2, 4, Sq // 2, 512), i32),
            pltpu.VMEM((ng, 2, 4, Sq // 2, 512), i32),
            pltpu.VMEM((2, Sq // 2, len(_OXS) * 128), i32),
            pltpu.SMEM((1,), i32),
            pltpu.SemaphoreType.DMA((2, ng)),
            pltpu.SemaphoreType.DMA((NKV,)),
            pltpu.SemaphoreType.DMA((NKV,)),
            pltpu.SemaphoreType.DMA((NKV,)),
            pltpu.SemaphoreType.DMA((2,)),
            pltpu.SemaphoreType.DMA((ng,)),
            pltpu.SemaphoreType.DMA(()),
        ],
        compiler_params=pltpu.CompilerParams(
            vmem_limit_bytes=124 * 1024 * 1024,
            disable_bounds_checks=True,
            disable_semaphore_checks=True,
        ),
    )(A_x, akt, avt, awq, awo, B_x, bkt, bvt, bwq, bwo)
```

```python
import functools
import math

import jax
import jax.numpy as jnp
import jax.experimental.pallas as pl
import jax.experimental.pallas.tpu as pltpu

_NN = (((1,), (0,)), ((), ()))
_NT = (((1,), (1,)), ((), ()))
bf16 = jnp.bfloat16
f32 = jnp.float32
i32 = jnp.int32

CH = 16
DEP = 3
XPAD = 46
NKV = 3
NPS = 4

_SEQ_FULL = ('q00 w0 q01 q02 w2 w1 s01 q03 p01 s02 p02 q10 s00 q11 p00 w3 s03 p03 '
             'q12 o00 q13 s11 o01 o02 p11 s12 o03 s10 p12 s13 p10 o10 o11 p13 o12 o13')
_SEQ_NOQ = ('s01 s02 s00 p01 p02 p00 w1 o00 s03 o01 s11 p03 s12 o02 w2 p11 w0 p12 '
            's10 o10 o11 s13 p10 w3 o03 p13 o12 o13')
_SEQ_Q = 'x1 q00 v1 q01 q02 q03 v0 x0 q10 q11 q12 q13'


def _dot(a, b, dims=_NN):
    return jax.lax.dot_general(a, b, dims, preferred_element_type=f32)


def _recip(l):
    r = pl.reciprocal(l, approx=True)
    return r * (2.0 - l * r)


def _col(x, i):
    return x[:, 128 * i:128 * (i + 1)]


def _pack(x):
    return pltpu.bitcast(x.astype(bf16), i32)


def _unpack(x):
    return pltpu.bitcast(x, bf16)


def _cat(xs, axis):
    return jnp.concatenate(list(xs), axis=axis)


def _or_tiles(vals):
    t = None
    for v in vals:
        for r in range(0, v.shape[0], 8):
            for c in range(0, v.shape[1], 128):
                x = v[r:r + 8, c:c + 128]
                t = x if t is None else t | x
    return t


def _lane_lo(rows):
    return jax.lax.broadcasted_iota(i32, (rows, 128), 1) < 64


_QPROD = (
    '+00-10 +03+05+04 +03', '+10 +03-43-23 +03+13', '+00-10 -00-02-01 +10',
    '+00 +00-30-10 +00+10', '+01-11 -13-12 +13', '+01 +13-33 +03+13',
    '+01-11 +11+15+14+10 +01', '+11 +11-41-21-01 +01+11', '+02-12 +20+25 +00',
    '+12 +20-40 +00+10', '+02-12 -24-23-22-21 +14', '+02 +24-04-34-14 +04+14',
    '+13 +31 +11', '+03 +31 +01', '+03-13 +32+35+33+30+34 +02',
    '+13 +32-42-12-02-22 +02+12', '+14 +44 +14', '+04 +44 +04',
    '+04-14 -45-40-43-41-42 +15', '+04 +45-25-05-15-35 +05+15', '+04+12 +40+25 +00+15',
    '+02+04 -25 +00-05', '+12+14 +40 +10-15', '+04+10 +43+05 +03+15',
    '+00+04 -05 +03-05', '+10+14 +43 +13-15', '+04+11 +41+15 +01+15',
    '+01+04 -15 +01-05', '+11+14 +41 +11-15', '+04+13 +42+35 +02+15',
    '+03+04 -35 +02-05', '+13+14 +42 +12-15', '+02+10 +23+04 +03+14',
    '+00+02 -04 +03-04', '+10+12 +23 +13-14', '+01+13 +33+12 +02+13',
    '+01+03 +33 +03-02', '+11+13 -12 +13-12', '+00+13 +30+02 +02+10',
    '+00+03 +30 +00-02', '+10+13 -02 +10-12', '+02+13 +34+22 +02+14',
    '+02+03 +34 +04-02', '+12+13 -22 +14-12', '+02+11 +21+14 +01+14',
    '+01+02 -14 +01-04', '+11+12 +21 +11-14', '+00+11 +10+01 +01+10',
    '+00+01 +10 +00-01', '+10+11 -01 +10-11',
)
_QROUNDS = (
    ((~5, ~15, 43, ~36), (~27, ~38, ~30, ~45), (11, 32, 41, ~42), (~17, 0, ~33, 1), (21, 19, 23, 24),
     (~39, ~46, 22, ~37), (~9, ~8, ~28, ~3), (49, 7, 47, 12), (18, ~2, 40, 31), (48, 20, 6, 26),
     (~44, ~10, ~16, 34), (~14, 29, 25, 35), (4, 13)),
    ((~32, ~5), (~23, ~26, ~11, 21), (43, ~17, ~46, ~34), (33, ~19, 45, 0), (~27, ~42, ~1, ~44),
     (36, 30, ~37, 24), (2, 47, 40, 7), (12, 22, ~28, ~49), (3, ~38, ~9, 39), (29, 14, 31, 15),
     (41, 16, 10, ~20), (35, 18, 25, 4), (48, 6, 8, ~13)),
)
_OPROD = (
    '+10 -00-20-40-50 +00-10', '+00+10 +00-02-04-03 +00', '+03 +30+10 +00-10',
    '+03+13 +30-31 +10', '+10 +01 +11', '+00 +01 +01',
    '+11 -11-31-21-41-51 +01-11', '+01+11 +11-10-12-14-13 +01', '+13 -32-52-42 +02-12',
    '+03+13 +32-33-34 +02', '+02 +22+12+02 +02-12', '+02+12 +22-21-20 +12',
    '+14 +43 +13', '+04 +43 +03', '+05 +53+23+13+03+33 +03-13',
    '+05+15 +53-54-51-50-52 +13', '+04 +44+14+04+34 +04-14', '+04+14 +44-41-40-42 +14',
    '+12 -24-54 +04-14', '+02+12 +24-23 +04', '+05+12 +54+23 +04+13',
    '+05-02 -23 +03+04', '+15-12 +54 +13+14', '+03+11 +31+10 +01+10',
    '+03-01 -10 +00+01', '+13-11 +31 +10+11', '+02+11 +12+21 +01+12',
    '+01-02 +12 +01+02', '+11-12 -21 +11+12', '+04+11 +14+41 +01+14',
    '+01-04 +14 +01+04', '+11-14 -41 +11+14', '+05+11 +13+51 +01+13',
    '+01-05 +13 +01+03', '+11-15 -51 +11+13', '+02+10 +02+20 +00+12',
    '+00-02 +02 +00+02', '+10-12 -20 +10+12', '+04+10 +04+40 +00+14',
    '+00-04 +04 +00+04', '+10-14 -40 +10+14', '+05+10 +03+50 +00+13',
    '+00-05 +03 +00+03', '+10-15 -50 +10+13', '+05+13 +33+52 +02+13',
    '+03-05 +33 +02+03', '+13-15 -52 +12+13', '+04+13 +34+42 +02+14',
    '+03-04 +34 +02+04', '+13-14 -42 +12+14',
)
_OROUNDS = (
    ((~13, ~16, ~48, ~45), (29, ~18, 4, ~37), (~14, ~32, ~6, ~41), (~20, ~23, ~38, ~2), (30, 7, 19, ~5),
     (26, 42, ~27, ~0), (1, 39, 21, ~36), (~33, 11, ~24, ~35), (49, 17, 31, 28), (47, 25, 34, 43),
     (~9, 46, 10, ~8), (44, ~12, 15, 22), (3, 40)),
    ((14, 13), (~45, ~16, ~2, ~48), (~37, ~0, ~32, 28), (~20, ~38, 4, ~23), (~29, 6, ~41, ~18),
     (~10, ~35, ~39, ~42), (5, 11, 26, 7), (33, 30, 19, 21), (~24, 27, 36, 1), (~47, ~34, ~22, ~49),
     (46, 44, 9, 8), (40, ~31, 25, 17), (43, ~15, 12, 3)),
)


def _terms(code):
    return tuple((1 if code[i] == '+' else -1, int(code[i + 1]), int(code[i + 2]))
                 for i in range(0, len(code), 3))


_QX, _QW, _QO = zip(*[[_terms(c) for c in p.split()] for p in _QPROD])
_QXS = sorted(set(_QX))
_OX, _OW, _OO = zip(*[[_terms(c) for c in p.split()] for p in _OPROD])
_ORAW = [((1, i, k),) for i in range(2) for k in range(6)]
_OXS = _ORAW + sorted(set(_OX) - set(_ORAW))
_ARRIVAL = (2, 0, 1, 3)


def _signed_sum(terms):
    if terms[0][0] < 0 and len(terms) > 1 and terms[1][0] > 0:
        terms = [terms[1], terms[0]] + list(terms[2:])
    sg0, y = terms[0]
    for sg, v in terms[1:]:
        if sg0 < 0 and sg > 0:
            sg0, y = 1, v - y
        else:
            y = y + v if sg == sg0 else y - v
    return y if sg0 > 0 else -y


def _weights(xa, xb, xc):
    h = xa.shape[1] // 2
    xa, xb, xc = xa.astype(f32), xb.astype(f32), xc.astype(f32)
    return (_cat([xa[:, :h], xb[:, :h] - xb[:, h:]], 0),
            _cat([xa[:, h:], xc[:, h:] - xc[:, :h]], 0),
            _cat([xc[:, :h], xb[:, h:]], 0))


def _pair_weights(t0, t1):
    return (_weights(t0[:64], t0[64:128], t0[128:]), _weights(t1[64:128], t1[128:], t1[:64]))


def _scores(q_ref, kt0, kt1, lhs):
    t0, t1, t2, rot = (q_ref[:, 128 * k:128 * (k + 1)] for k in range(4))
    lo = _lane_lo(t0.shape[0])
    q = ((t0, jnp.where(lo, t0, rot), jnp.where(lo, t1, t0)),
         (t2, jnp.where(lo, t2, t1), jnp.where(lo, rot, t2)))
    w = _pair_weights(kt0, kt1)
    p = {}

    def run(h, k, i):
        y = _dot(lhs(q[h][k]), _col(w[h][k], i).astype(bf16))
        p[h, k, i] = y if k == 2 else y + p[h, 2, i]

    for t, (h, i) in enumerate(((0, 0), (0, 1), (1, 0))):
        run(h, 2, i), run(h, 0, i), run(h, 1, i), run(1, (2, 0, 1)[t], 1)
    return tuple(_cat([p[h, 0, 0], p[h, 0, 1], p[h, 1, 0], p[h, 1, 1]], 1) for h in range(2))


def _softmax_terms(s, p_ref, zero):
    ls, toks = [], []
    for c in range(s.shape[0] // CH):
        sc = s[c * CH:(c + 1) * CH]
        m = jnp.broadcast_to(jnp.max(sc, axis=-1, keepdims=True), (CH, 128))
        if c >= DEP:
            t = toks[c - DEP] & zero
            m = pltpu.bitcast(pltpu.bitcast(m, i32) | _cat([t, t], 0), f32)
        e = [jnp.exp2(_col(sc, k) - m) for k in range(4)]
        t0, t1 = e[0] + e[2], e[1] + e[3]
        ls.append(jnp.broadcast_to(jnp.sum(t0 + t1, axis=-1, keepdims=True), (CH, 128)))
        rows = slice(c * CH // 2, (c + 1) * CH // 2)
        for k, x in enumerate(e + [t0, t1]):
            p_ref[rows, 128 * k:128 * (k + 1)] = _pack(x)
        toks.append(_or_tiles([p_ref[rows, :]]))
    return ls


def _attend(s, vt0, vt1, p_ref, zero, lhs, sink):
    ls = [_softmax_terms(s[h], p_ref.at[h], zero) for h in range(2)]
    w = _pair_weights(vt0, vt1)
    r = {}
    for h, k in ((0, 0), (0, 1), (0, 2), (1, 1), (1, 2), (1, 0)):
        r[h, k] = _dot(lhs(p_ref.at[h][:, 256 * k:256 * (k + 1)]), w[h][k].astype(bf16), _NT)
    lo = _lane_lo(CH)

    def rows(c):
        p1, p2, p3, u1, u2, u3 = (r[h, k][c * CH:(c + 1) * CH] for h in range(2) for k in range(3))
        r0, r1 = _recip(ls[0][c]), _recip(ls[1][c])
        o_lo = p1 + jnp.where(lo, p2, p3)
        o_hi = u1 + jnp.where(lo, u2, u3)
        mid = jnp.where(lo, p3, u2) + pltpu.roll(jnp.where(lo, u3, p2), 64, 1)
        return _cat([o_lo * r0, mid * jnp.where(lo, r0, r1), o_hi * r1], 1)

    for c in range(len(ls[0])):
        sink(c, rows(c))


def _kernel(ax, akt, avt, awq, awo, bx, bkt, bvt, bwq, bwo, out,
            xbuf, xca, xcb, kvbuf, rq, ro, rq0, ro0,
            wqc0, woc0, wqc1, woc1,
            acc, obuf, pbuf, qbuf, qall, oc, zref,
            xsem, kvsem, rqsem, rosem, isem, vsem, osem,
            *, scale, d, sq, nbatch, npass, dh):
    ng = nbatch // 2
    nsteps = npass * ng
    gw = 4 * dh
    wr = 128 // ng
    xs, wqs, wos = (ax, bx), (awq, bwq), (awo, bwo)
    kvs = (akt, avt, bkt, bvt)
    xc = (xca, xcb)
    wsets = ((wqc0, woc0), (wqc1, woc1))

    def wait_all(ref, sem):
        pltpu.make_async_copy(ref, ref, sem).wait()

    def fetch(pp, gg, slot, live=True):
        def start(src, dst, sem):
            pl.when(live)(lambda: pltpu.make_async_copy(src, dst, sem).start())

        for t in range(4):
            start(kvs[t].at[pl.ds(gg * 2, 2), pl.ds(4 * pp, 4)], kvbuf.at[slot, t], kvsem.at[slot])
        pw = jnp.minimum(pp + 1, npass - 1)
        rows = pl.ds(pl.multiple_of(gg * wr, 16), wr)
        for j in range(2):
            for t in range(5):
                start(wqs[j].at[t, rows, pl.ds(pl.multiple_of(pw * gw, 128), gw)],
                      rq.at[slot, j, t], rqsem.at[slot])
            start(wos[j].at[pw, :, rows], ro.at[slot, j], rosem.at[slot])

    def fetch_wait(slot):
        wait_all(kvbuf.at[slot], kvsem.at[slot])
        wait_all(rq.at[slot], rqsem.at[slot])
        wait_all(ro.at[slot], rosem.at[slot])

    def x_copy(j, gg):
        return pltpu.make_async_copy(xs[j].at[pl.ds(gg * 2, 2)], xbuf.at[j, gg], xsem.at[j, gg])

    def build_x(j, gg):
        back = []
        for r in range(0, sq, 16):
            x = [xbuf.at[j, gg, i][r:r + 16, :].astype(f32) for i in range(2)]
            tiles = [_signed_sum([(sg, _col(x[i], k)) for sg, i, k in f]) for f in _QXS]
            rows = slice(r // 2, r // 2 + 8)
            xc[j].at[gg][rows, :128 * len(tiles)] = _pack(_cat(tiles, 1))
            back.append(xc[j].at[gg][rows, :128 * len(tiles)])
        return back

    def build_wq(j, gg, raw, wset):
        wqc = wset[0]
        kt = [raw(t).astype(f32) for t in range(5)]
        tiles = [_signed_sum([(sg, _col(kt[k], n)) for sg, k, n in f]) for f in _QW]
        rows = pl.ds(pl.multiple_of(gg * (wr // 2), 8), wr // 2)
        wqc.at[j][rows, :] = _pack(_cat(tiles, 1))
        return [wqc.at[j][rows, :]]

    def build_wo(j, gg, raw, wset):
        woc = wset[1]
        kt = [raw(t).astype(f32) for t in range(6)]
        tiles = [_signed_sum([(sg, _col(kt[k], n)) for sg, k, n in f]) for f in _OW]
        rows = pl.ds(pl.multiple_of(gg * (wr // 2), 8), wr // 2)
        woc.at[j][rows, :] = _pack(_cat(tiles, 1))
        return [woc.at[j][rows, :]]

    def compute(seq, g, slot, par, q_ref, first, write_out, last=None):
        wqc, woc = wsets[par]
        s, qm, om = {}, {}, {}
        toks = []
        zero = jnp.full((8, 128), zref[0], i32)

        def lhs(x):
            for e in toks:
                e[0] -= 1
            if toks and toks[0][0] < 0:
                t = toks.pop(0)[1] & zero
                x = _cat([x[:8] | _cat([t] * (x.shape[1] // 128), 1), x[8:]], 0)
            return _unpack(x)

        def gate(delay, vals):
            toks.append([delay, _or_tiles(vals)])
            toks.sort(key=lambda e: e[0])

        def run_round(ids, x_ref, w_ref, xs_, xf, of, state, finish):
            touched = []
            for e in ids:
                m = e if e >= 0 else ~e
                xt = xs_.index(xf[m])
                x = x_ref[:, 128 * xt:128 * (xt + 1)]
                w = _unpack(w_ref[:, 128 * m:128 * (m + 1)])
                y = _dot(lhs(x), w)
                for sg, i, n in of[m]:
                    st = state.setdefault((i, n), [[], sum(o[1:] == (i, n) for f in of for o in f)])
                    st[0].insert(0, (sg, y))
                    st[1] -= 1
                    if (e >= 0 or st[1] == 0) and (i, n) not in touched:
                        touched.append((i, n))
            for i, n in touched:
                st = state[i, n]
                y = _signed_sum(st[0])
                st[0] = [(1, y)]
                if st[1] == 0:
                    finish(i, n, y)

        def q_round(j, ids):
            def finish(i, n, y):
                y = y * scale
                dst = q_ref.at[j, 2 * i + n // 3]
                dst[:, 128 * (n % 3):128 * (n % 3 + 1)] = _pack(y)
                if n % 3 == 1:
                    dst[:, 384:] = _pack(pltpu.roll(y, 64, 1))

            run_round(ids, xc[j].at[g], wqc.at[j], _QXS, _QX, _QO, qm.setdefault(j, {}), finish)

        def q_piece(j, part):
            rounds = _QROUNDS[j]
            cuts = [j + c for c in (0, 2, 5, 9)] + [len(rounds)]
            for r in range(cuts[part], cuts[part + 1]):
                q_round(j, rounds[r])
            if part == 3 and j == 0:
                q_round(1, _QROUNDS[1][0])

        def x_piece(j):
            back = build_x(1, g) if j == 1 else build_x(0, jnp.minimum(g + 1, ng - 1))
            for c, v in enumerate(back):
                gate(9 + 4 * c, [v])

        def v_piece(j):
            gate(-1, build_wo(j, g, lambda t: ro0[g, j, t], wsets[0]))

        def kv(j, which, u):
            return tuple(kvbuf[slot, 2 * j + which, u // 2, 2 * (u % 2) + h] for h in range(2))

        def s_piece(j, u):
            s[j, u] = _scores(q_ref.at[j, u], *kv(j, 0, u), lhs)

        def p_piece(j, u):
            when = lambda i, k: _ARRIVAL[2 * i + k // 3]
            new = [t for t, f in enumerate(_OXS) if max(when(i, k) for _, i, k in f) == _ARRIVAL[u]]

            def sink(c, o):
                rows = slice(c * CH // 2, (c + 1) * CH // 2)
                tile = lambda t: oc.at[j][rows, 128 * t:128 * (t + 1)]
                val = lambda i, k: (_col(o, k % 3) if when(i, k) == _ARRIVAL[u]
                                    else _unpack(tile(6 * i + k)).astype(f32))
                for t in new:
                    y = _signed_sum([(sg, val(i, k)) for sg, i, k in _OXS[t]])
                    oc.at[j][rows, 128 * t:128 * (t + 1)] = _pack(y)

            _attend(s.pop((j, u)), *kv(j, 1, u), pbuf.at[_ARRIVAL[u]], zero, lhs, sink)

        def o_round(j, ids):
            def finish(i, n, y):
                b = 2 * g + i
                cols = slice(j * d + 128 * n, j * d + 128 * (n + 1))
                if not first:
                    y = y + acc[b, :, cols]
                acc[b, :, cols] = y
                if write_out:
                    obuf[b, :, cols] = y.astype(bf16)

            run_round(ids, oc.at[j], woc.at[j], _OXS, _OX, _OO, om.setdefault(j, {}), finish)

        def flush(i):
            if write_out:
                @pl.when(last)
                def _():
                    pltpu.make_async_copy(obuf.at[2 * g + i], out.at[2 * g + i], osem).start()

        def o_piece(j, part):
            rounds = _OROUNDS[j]
            cuts = [j + c for c in (0, 1, 4, 8)] + [len(rounds)]
            for r in range(cuts[part], cuts[part + 1]):
                o_round(j, rounds[r])
            if part == 3:
                if j == 0:
                    o_round(1, _OROUNDS[1][0])
                else:
                    flush(0), flush(1)

        def w_piece(k):
            j = k // 2
            back = (build_wq(j, g, lambda t: rq[slot, j, t], wsets[1 - par]) if k % 2 == 0
                    else build_wo(j, g, lambda t: ro[slot, j, t], wsets[1 - par]))
            gate(-1, back)

        run = {'q': q_piece, 's': s_piece, 'p': p_piece, 'o': o_piece, 'w': w_piece,
               'x': x_piece, 'v': v_piece}
        for tok in seq.split():
            run[tok[0]](*(int(ch) for ch in tok[1:]))

    def run_pass(p, par, first, slot0):
        def step(g, slot):
            fetch_wait(slot)

            wrap = g + 2 >= ng
            fetch(jnp.minimum(jnp.where(wrap, p + 1, p), npass - 1),
                  jnp.where(wrap, g + 2 - ng, g + 2), jnp.where(slot == 0, NKV - 1, slot - 1),
                  p * ng + g + 2 < nsteps)

            if first:
                compute(_SEQ_NOQ, g, slot, par, qall.at[g], True, False)
            else:
                compute(_SEQ_FULL, g, slot, par, qbuf, False, par == 1, p == npass - 1)
            return jnp.where(slot == NKV - 1, 0, slot + 1)

        jax.lax.fori_loop(0, ng, step, slot0)

    def wq_init(j):
        return pltpu.make_async_copy(wqs[j].at[:, :, pl.ds(0, gw)], rq0.at[j], isem.at[j])

    zref[0] = 0
    x_copy(0, 0).start()
    wq_init(0).start()
    x_copy(0, 0).wait()
    wq_init(1).start()
    build_x(0, 0)
    for j in range(2):
        wq_init(j).wait()
        if j == 0:
            for gg in range(ng):
                x_copy(1, gg).start()
                for jj in range(2):
                    pltpu.make_async_copy(wos[jj].at[0, :, pl.ds(gg * wr, wr)], ro0.at[gg, jj],
                                          vsem.at[gg]).start()
                if gg + 1 < ng:
                    x_copy(0, gg + 1).start()

        def init_wq(gg, carry, j=j):
            rows = pl.ds(pl.multiple_of(gg * wr, 16), wr)
            build_wq(j, gg, lambda t: rq0.at[j, t][rows, :], wsets[0])
            return carry

        jax.lax.fori_loop(0, ng, init_wq, 0)

    def q_step(g, carry):
        x_copy(1, g).wait()
        wait_all(ro0.at[g], vsem.at[g])

        @pl.when(g + 1 < ng)
        def _():
            x_copy(0, g + 1).wait()

        @pl.when(g == 1)
        def _():
            fetch(0, 0, 0)

        @pl.when(g == 4)
        def _():
            fetch(0, 1, 1)

        compute(_SEQ_Q, g, 0, 0, qall.at[g], True, False)
        return carry

    jax.lax.fori_loop(0, ng, q_step, 0)

    run_pass(0, 0, True, 0)

    def pass_pair(pp, carry):
        run_pass(2 * pp + 1, 1, False, ((2 * pp + 1) * ng) % NKV)

        @pl.when(2 * pp + 2 < npass)
        def _():
            run_pass(2 * pp + 2, 0, False, ((2 * pp + 2) * ng) % NKV)

        return carry

    jax.lax.fori_loop(0, npass // 2, pass_pair, 0)
    wait_all(out, osem)


@jax.jit
def pallas_concat_heads__gqa_block_cached__mha_block_cached__near_ridge_kernel(
    A_x: jax.Array,
    A_k_cache: jax.Array,
    A_v_cache: jax.Array,
    A_wq: jax.Array,
    A_wo: jax.Array,
    B_x: jax.Array,
    B_k_cache: jax.Array,
    B_v_cache: jax.Array,
    B_wq: jax.Array,
    B_wo: jax.Array,
):
    B, Sq, D = A_x.shape
    _, H, Sk, Dh = A_k_cache.shape
    assert (B, Sq, D, H, Sk, Dh) == (16, 160, 640, 32, 512, 192)
    npass, ng = H // 4, B // 2
    gw = 4 * Dh
    scale = (Dh ** -0.5) * math.log2(math.e)

    akt, avt, bkt, bvt = (jnp.swapaxes(t, 2, 3) for t in
                          (A_k_cache, A_v_cache, B_k_cache, B_v_cache))
    awq, bwq = (w.reshape(5, 128, H * Dh) for w in (A_wq, B_wq))
    awo, bwo = (w.reshape(npass, 6, 128, D) for w in (A_wo, B_wo))
    any_spec = pl.BlockSpec(memory_space=pl.ANY)
    wset = [
        pltpu.VMEM((2, 64, len(_QW) * 128), i32),
        pltpu.VMEM((2, 64, len(_OW) * 128), i32),
    ]

    return pl.pallas_call(
        functools.partial(_kernel, scale=scale, d=D, sq=Sq, nbatch=B, npass=npass, dh=Dh),
        in_specs=[any_spec] * 10,
        out_specs=any_spec,
        out_shape=jax.ShapeDtypeStruct((B, Sq, 2 * D), A_x.dtype),
        scratch_shapes=[
            pltpu.VMEM((2, ng, 2, Sq, D), bf16),
            pltpu.VMEM((ng, Sq // 2, XPAD * 128), i32),
            pltpu.VMEM((ng, Sq // 2, XPAD * 128), i32),
            pltpu.VMEM((NKV, 4, 2, 4, Dh, Sk), bf16),
            pltpu.VMEM((NKV, 2, 5, 128 // ng, gw), bf16),
            pltpu.VMEM((NKV, 2, 6, 128 // ng, D), bf16),
            pltpu.VMEM((2, 5, 128, gw), bf16),
            pltpu.VMEM((ng, 2, 6, 128 // ng, D), bf16),
            *wset, *wset,
            pltpu.VMEM((B, Sq, 2 * D), f32),
            pltpu.VMEM((B, Sq, 2 * D), bf16),
            pltpu.VMEM((NPS, 2, Sq // 2, 768), i32),
            pltpu.VMEM((2, 4, Sq // 2, 512), i32),
            pltpu.VMEM((ng, 2, 4, Sq // 2, 512), i32),
            pltpu.VMEM((2, Sq // 2, len(_OXS) * 128), i32),
            pltpu.SMEM((1,), i32),
            pltpu.SemaphoreType.DMA((2, ng)),
            pltpu.SemaphoreType.DMA((NKV,)),
            pltpu.SemaphoreType.DMA((NKV,)),
            pltpu.SemaphoreType.DMA((NKV,)),
            pltpu.SemaphoreType.DMA((2,)),
            pltpu.SemaphoreType.DMA((ng,)),
            pltpu.SemaphoreType.DMA(()),
        ],
        compiler_params=pltpu.CompilerParams(
            vmem_limit_bytes=124 * 1024 * 1024,
            disable_bounds_checks=True,
            disable_semaphore_checks=True,
        ),
    )(A_x, akt, avt, awq, awo, B_x, bkt, bvt, bwq, bwo)
```

```python
import functools
import math

import jax
import jax.numpy as jnp
import jax.experimental.pallas as pl
import jax.experimental.pallas.tpu as pltpu

_NN = (((1,), (0,)), ((), ()))
_NT = (((1,), (1,)), ((), ()))
bf16 = jnp.bfloat16
f32 = jnp.float32
i32 = jnp.int32

CH = 16
DEP = 3
XPAD = 46
NKV = 3
NPS = 4

_SEQ_FULL = ('q00 w0 q01 q02 w2 w1 s01 q03 p01 s02 p02 q10 s00 q11 p00 w3 s03 p03 '
             'q12 o00 q13 s11 o01 o02 p11 s12 o03 s10 o10 p12 s13 p10 o11 p13 o12 o13')
_SEQ_NOQ = ('s01 s02 s00 p01 p02 p00 w1 o00 s03 o01 s11 p03 s12 o02 w2 p11 w0 p12 '
            's10 o10 o11 s13 p10 w3 o03 p13 o12 o13')
_SEQ_Q = 'x1 q00 v1 q01 q02 q03 v0 x0 q10 q11 q12 q13'


def _dot(a, b, dims=_NN):
    return jax.lax.dot_general(a, b, dims, preferred_element_type=f32)


def _recip(l):
    r = pl.reciprocal(l, approx=True)
    return r * (2.0 - l * r)


def _col(x, i):
    return x[:, 128 * i:128 * (i + 1)]


def _pack(x):
    return pltpu.bitcast(x.astype(bf16), i32)


def _unpack(x):
    return pltpu.bitcast(x, bf16)


def _cat(xs, axis):
    return jnp.concatenate(list(xs), axis=axis)


def _or_tiles(vals):
    t = None
    for v in vals:
        for r in range(0, v.shape[0], 8):
            for c in range(0, v.shape[1], 128):
                x = v[r:r + 8, c:c + 128]
                t = x if t is None else t | x
    return t


def _lane_lo(rows):
    return jax.lax.broadcasted_iota(i32, (rows, 128), 1) < 64


_QPROD = (
    '+00-10 +03+05+04 +03', '+10 +03-43-23 +03+13', '+00-10 -00-02-01 +10',
    '+00 +00-30-10 +00+10', '+01-11 -13-12 +13', '+01 +13-33 +03+13',
    '+01-11 +11+15+14+10 +01', '+11 +11-41-21-01 +01+11', '+02-12 +20+25 +00',
    '+12 +20-40 +00+10', '+02-12 -24-23-22-21 +14', '+02 +24-04-34-14 +04+14',
    '+13 +31 +11', '+03 +31 +01', '+03-13 +32+35+33+30+34 +02',
    '+13 +32-42-12-02-22 +02+12', '+14 +44 +14', '+04 +44 +04',
    '+04-14 -45-40-43-41-42 +15', '+04 +45-25-05-15-35 +05+15', '+04+12 +40+25 +00+15',
    '+02+04 -25 +00-05', '+12+14 +40 +10-15', '+04+10 +43+05 +03+15',
    '+00+04 -05 +03-05', '+10+14 +43 +13-15', '+04+11 +41+15 +01+15',
    '+01+04 -15 +01-05', '+11+14 +41 +11-15', '+04+13 +42+35 +02+15',
    '+03+04 -35 +02-05', '+13+14 +42 +12-15', '+02+10 +23+04 +03+14',
    '+00+02 -04 +03-04', '+10+12 +23 +13-14', '+01+13 +33+12 +02+13',
    '+01+03 +33 +03-02', '+11+13 -12 +13-12', '+00+13 +30+02 +02+10',
    '+00+03 +30 +00-02', '+10+13 -02 +10-12', '+02+13 +34+22 +02+14',
    '+02+03 +34 +04-02', '+12+13 -22 +14-12', '+02+11 +21+14 +01+14',
    '+01+02 -14 +01-04', '+11+12 +21 +11-14', '+00+11 +10+01 +01+10',
    '+00+01 +10 +00-01', '+10+11 -01 +10-11',
)
_QROUNDS = (
    ((~5, ~15, 43, ~36), (~27, ~38, ~30, ~45), (11, 32, 41, ~42), (17, 0, 33, 1), (21, 19, 23, 24),
     (~39, ~46, 22, ~37), (~2, ~8, 28, ~3), (49, 7, 47, 12), (18, ~9, 40, 31), (48, ~20, 6, 26),
     (~44, ~10, ~16, 34), (~14, 29, 25, 35), (4, 13)),
    ((~32, ~5), (~23, ~26, ~11, 21), (43, ~17, ~46, ~34), (33, ~19, 45, 0), (~27, ~42, ~1, ~44),
     (36, 30, ~37, ~24), (2, 47, 40, 7), (12, 22, ~28, 49), (3, ~38, ~9, 39), (29, 14, 31, ~15),
     (41, 16, 10, ~20), (35, 18, 25, 4), (~48, ~6, ~8, ~13)),
)
_OPROD = (
    '+10 -00-20-40-50 +00-10', '+00+10 +00-02-04-03 +00', '+03 +30+10 +00-10',
    '+03+13 +30-31 +10', '+10 +01 +11', '+00 +01 +01',
    '+11 -11-31-21-41-51 +01-11', '+01+11 +11-10-12-14-13 +01', '+13 -32-52-42 +02-12',
    '+03+13 +32-33-34 +02', '+02 +22+12+02 +02-12', '+02+12 +22-21-20 +12',
    '+14 +43 +13', '+04 +43 +03', '+05 +53+23+13+03+33 +03-13',
    '+05+15 +53-54-51-50-52 +13', '+04 +44+14+04+34 +04-14', '+04+14 +44-41-40-42 +14',
    '+12 -24-54 +04-14', '+02+12 +24-23 +04', '+05+12 +54+23 +04+13',
    '+05-02 -23 +03+04', '+15-12 +54 +13+14', '+03+11 +31+10 +01+10',
    '+03-01 -10 +00+01', '+13-11 +31 +10+11', '+02+11 +12+21 +01+12',
    '+01-02 +12 +01+02', '+11-12 -21 +11+12', '+04+11 +14+41 +01+14',
    '+01-04 +14 +01+04', '+11-14 -41 +11+14', '+05+11 +13+51 +01+13',
    '+01-05 +13 +01+03', '+11-15 -51 +11+13', '+02+10 +02+20 +00+12',
    '+00-02 +02 +00+02', '+10-12 -20 +10+12', '+04+10 +04+40 +00+14',
    '+00-04 +04 +00+04', '+10-14 -40 +10+14', '+05+10 +03+50 +00+13',
    '+00-05 +03 +00+03', '+10-15 -50 +10+13', '+05+13 +33+52 +02+13',
    '+03-05 +33 +02+03', '+13-15 -52 +12+13', '+04+13 +34+42 +02+14',
    '+03-04 +34 +02+04', '+13-14 -42 +12+14',
)
_OROUNDS = (
    ((~13, ~16, ~48, ~45), (29, ~18, 4, ~37), (~14, ~32, ~38, ~41), (~20, ~23, ~6, ~2), (30, 7, 19, ~5),
     (26, 42, ~27, ~0), (1, 39, 21, ~36), (~33, 11, ~24, ~35), (49, 17, 31, 28), (47, 25, 34, 43),
     (~9, 46, 10, ~8), (44, 12, ~15, 22), (3, 40)),
    ((14, 13), (~45, ~16, ~2, ~48), (~37, ~0, ~29, 28), (~20, ~38, ~4, ~23), (~32, ~6, ~41, ~18),
     (~10, ~35, ~39, ~42), (5, 11, 26, ~7), (33, 30, 19, 21), (~24, 27, 36, 1), (~47, ~34, ~22, ~49),
     (40, ~31, 25, 17), (46, 44, 9, 8), (~15, 43, 12, 3)),
)


def _terms(code):
    return tuple((1 if code[i] == '+' else -1, int(code[i + 1]), int(code[i + 2]))
                 for i in range(0, len(code), 3))


_QX, _QW, _QO = zip(*[[_terms(c) for c in p.split()] for p in _QPROD])
_QXS = sorted(set(_QX))
_OX, _OW, _OO = zip(*[[_terms(c) for c in p.split()] for p in _OPROD])
_ORAW = [((1, i, k),) for i in range(2) for k in range(6)]
_OXS = _ORAW + sorted(set(_OX) - set(_ORAW))
_ARRIVAL = (2, 0, 1, 3)


def _signed_sum(terms):
    if terms[0][0] < 0 and len(terms) > 1 and terms[1][0] > 0:
        terms = [terms[1], terms[0]] + list(terms[2:])
    sg0, y = terms[0]
    for sg, v in terms[1:]:
        if sg0 < 0 and sg > 0:
            sg0, y = 1, v - y
        else:
            y = y + v if sg == sg0 else y - v
    return y if sg0 > 0 else -y


def _weights(xa, xb, xc):
    h = xa.shape[1] // 2
    xa, xb, xc = xa.astype(f32), xb.astype(f32), xc.astype(f32)
    return (_cat([xa[:, :h], xb[:, :h] - xb[:, h:]], 0),
            _cat([xa[:, h:], xc[:, h:] - xc[:, :h]], 0),
            _cat([xc[:, :h], xb[:, h:]], 0))


def _pair_weights(t0, t1):
    return (_weights(t0[:64], t0[64:128], t0[128:]), _weights(t1[64:128], t1[128:], t1[:64]))


def _scores(q_ref, kt0, kt1, lhs):
    t0, t1, t2, rot = (q_ref[:, 128 * k:128 * (k + 1)] for k in range(4))
    lo = _lane_lo(t0.shape[0])
    q = ((t0, jnp.where(lo, t0, rot), jnp.where(lo, t1, t0)),
         (t2, jnp.where(lo, t2, t1), jnp.where(lo, rot, t2)))
    w = _pair_weights(kt0, kt1)
    p = {}

    def run(h, k, i):
        y = _dot(lhs(q[h][k]), _col(w[h][k], i).astype(bf16))
        p[h, k, i] = y if k == 2 else y + p[h, 2, i]

    run(0, 2, 0), run(0, 2, 1), run(1, 2, 0), run(1, 2, 1)
    for h in range(2):
        run(h, 0, 0), run(h, 0, 1), run(h, 1, 0), run(h, 1, 1)
    return tuple(_cat([p[h, 0, 0], p[h, 0, 1], p[h, 1, 0], p[h, 1, 1]], 1) for h in range(2))


def _softmax_terms(s, p_ref, zero):
    ls, toks = [], []
    for c in range(s.shape[0] // CH):
        sc = s[c * CH:(c + 1) * CH]
        m = jnp.broadcast_to(jnp.max(sc, axis=-1, keepdims=True), (CH, 128))
        if c >= DEP:
            t = toks[c - DEP] & zero
            m = pltpu.bitcast(pltpu.bitcast(m, i32) | _cat([t, t], 0), f32)
        e = [jnp.exp2(_col(sc, k) - m) for k in range(4)]
        t0, t1 = e[0] + e[2], e[1] + e[3]
        t01 = t0 + t1
        ls.append(jnp.broadcast_to(jnp.sum(t01, axis=-1, keepdims=True), (CH, 128)))
        rows = slice(c * CH // 2, (c + 1) * CH // 2)
        for k, x in enumerate(e + [t0, t1]):
            p_ref[rows, 128 * k:128 * (k + 1)] = _pack(x)
        toks.append(_or_tiles([p_ref[rows, :], pltpu.bitcast(t01, i32)]))
    return ls


def _attend(s, vt0, vt1, p_ref, zero, lhs, sink):
    ls = [_softmax_terms(s[h], p_ref.at[h], zero) for h in range(2)]
    w = _pair_weights(vt0, vt1)
    r = {}
    for h, k in ((0, 0), (0, 2), (0, 1), (1, 0), (1, 2), (1, 1)):
        r[h, k] = _dot(lhs(p_ref.at[h][:, 256 * k:256 * (k + 1)]), w[h][k].astype(bf16), _NT)
    lo = _lane_lo(CH)

    def rows(c):
        p1, p2, p3, u1, u2, u3 = (r[h, k][c * CH:(c + 1) * CH] for h in range(2) for k in range(3))
        r0, r1 = _recip(ls[0][c]), _recip(ls[1][c])
        o_lo = p1 + jnp.where(lo, p2, p3)
        o_hi = u1 + jnp.where(lo, u2, u3)
        mid = jnp.where(lo, p3, u2) + pltpu.roll(jnp.where(lo, u3, p2), 64, 1)
        return _cat([o_lo * r0, mid * jnp.where(lo, r0, r1), o_hi * r1], 1)

    for c in range(len(ls[0])):
        sink(c, rows(c))


def _kernel(ax, akt, avt, awq, awo, bx, bkt, bvt, bwq, bwo, out,
            xbuf, xca, xcb, kvbuf, rq, ro, rq0, ro0,
            wqc0, woc0, wqc1, woc1,
            acc, obuf, pbuf, qbuf, qall, oc, zref,
            xsem, kvsem, rqsem, rosem, isem, vsem, osem,
            *, scale, d, sq, nbatch, npass, dh):
    ng = nbatch // 2
    nsteps = npass * ng
    gw = 4 * dh
    wr = 128 // ng
    xs, wqs, wos = (ax, bx), (awq, bwq), (awo, bwo)
    kvs = (akt, avt, bkt, bvt)
    xc = (xca, xcb)
    wsets = ((wqc0, woc0), (wqc1, woc1))

    def wait_all(ref, sem):
        pltpu.make_async_copy(ref, ref, sem).wait()

    def fetch(pp, gg, slot, live=True):
        def start(src, dst, sem):
            pl.when(live)(lambda: pltpu.make_async_copy(src, dst, sem).start())

        for t in range(4):
            start(kvs[t].at[pl.ds(gg * 2, 2), pl.ds(4 * pp, 4)], kvbuf.at[slot, t], kvsem.at[slot])
        pw = jnp.minimum(pp + 1, npass - 1)
        rows = pl.ds(pl.multiple_of(gg * wr, 16), wr)
        for j in range(2):
            for t in range(5):
                start(wqs[j].at[t, rows, pl.ds(pl.multiple_of(pw * gw, 128), gw)],
                      rq.at[slot, j, t], rqsem.at[slot])
            start(wos[j].at[pw, :, rows], ro.at[slot, j], rosem.at[slot])

    def fetch_wait(slot):
        wait_all(kvbuf.at[slot], kvsem.at[slot])
        wait_all(rq.at[slot], rqsem.at[slot])
        wait_all(ro.at[slot], rosem.at[slot])

    def x_copy(j, gg):
        return pltpu.make_async_copy(xs[j].at[pl.ds(gg * 2, 2)], xbuf.at[j, gg], xsem.at[j, gg])

    def build_x(j, gg):
        back = []
        for r in range(0, sq, 16):
            x = [xbuf.at[j, gg, i][r:r + 16, :].astype(f32) for i in range(2)]
            tiles = [_signed_sum([(sg, _col(x[i], k)) for sg, i, k in f]) for f in _QXS]
            rows = slice(r // 2, r // 2 + 8)
            xc[j].at[gg][rows, :128 * len(tiles)] = _pack(_cat(tiles, 1))
            back.append(xc[j].at[gg][rows, :128 * len(tiles)])
        return back

    def build_wq(j, gg, raw, wset):
        wqc = wset[0]
        kt = [raw(t).astype(f32) for t in range(5)]
        tiles = [_signed_sum([(sg, _col(kt[k], n)) for sg, k, n in f]) for f in _QW]
        rows = pl.ds(pl.multiple_of(gg * (wr // 2), 8), wr // 2)
        wqc.at[j][rows, :] = _pack(_cat(tiles, 1))
        return [wqc.at[j][rows, :]]

    def build_wo(j, gg, raw, wset):
        woc = wset[1]
        kt = [raw(t).astype(f32) for t in range(6)]
        tiles = [_signed_sum([(sg, _col(kt[k], n)) for sg, k, n in f]) for f in _OW]
        rows = pl.ds(pl.multiple_of(gg * (wr // 2), 8), wr // 2)
        woc.at[j][rows, :] = _pack(_cat(tiles, 1))
        return [woc.at[j][rows, :]]

    def compute(seq, g, slot, par, q_ref, first, write_out, last=None):
        wqc, woc = wsets[par]
        s, qm, om = {}, {}, {}
        toks = []
        zero = jnp.full((8, 128), zref[0], i32)

        def lhs(x):
            for e in toks:
                e[0] -= 1
            if toks and toks[0][0] < 0:
                t = toks.pop(0)[1] & zero
                x = _cat([x[:8] | _cat([t] * (x.shape[1] // 128), 1), x[8:]], 0)
            return _unpack(x)

        def gate(delay, vals):
            toks.append([delay, _or_tiles(vals)])
            toks.sort(key=lambda e: e[0])

        def run_round(ids, x_ref, w_ref, xs_, xf, of, state, finish):
            touched = []
            for e in ids:
                m = e if e >= 0 else ~e
                xt = xs_.index(xf[m])
                x = x_ref[:, 128 * xt:128 * (xt + 1)]
                w = _unpack(w_ref[:, 128 * m:128 * (m + 1)])
                y = _dot(lhs(x), w)
                for sg, i, n in of[m]:
                    st = state.setdefault((i, n), [[], sum(o[1:] == (i, n) for f in of for o in f)])
                    st[0].insert(0, (sg, y))
                    st[1] -= 1
                    if (e >= 0 or st[1] == 0) and (i, n) not in touched:
                        touched.append((i, n))
            for i, n in touched:
                st = state[i, n]
                y = _signed_sum(st[0])
                st[0] = [(1, y)]
                if st[1] == 0:
                    finish(i, n, y)

        def q_round(j, ids):
            def finish(i, n, y):
                y = y * scale
                dst = q_ref.at[j, 2 * i + n // 3]
                dst[:, 128 * (n % 3):128 * (n % 3 + 1)] = _pack(y)
                if n % 3 == 1:
                    dst[:, 384:] = _pack(pltpu.roll(y, 64, 1))

            run_round(ids, xc[j].at[g], wqc.at[j], _QXS, _QX, _QO, qm.setdefault(j, {}), finish)

        def q_piece(j, part):
            rounds = _QROUNDS[j]
            cuts = [j + c for c in (0, 2, 5, 9)] + [len(rounds)]
            for r in range(cuts[part], cuts[part + 1]):
                q_round(j, rounds[r])
            if part == 3 and j == 0:
                q_round(1, _QROUNDS[1][0])

        def x_piece(j):
            back = build_x(1, g) if j == 1 else build_x(0, jnp.minimum(g + 1, ng - 1))
            for c, v in enumerate(back):
                gate(9 + 4 * c, [v])

        def v_piece(j):
            gate(-1, build_wo(j, g, lambda t: ro0[g, j, t], wsets[0]))

        def kv(j, which, u):
            return tuple(kvbuf[slot, 2 * j + which, u // 2, 2 * (u % 2) + h] for h in range(2))

        def s_piece(j, u):
            s[j, u] = _scores(q_ref.at[j, u], *kv(j, 0, u), lhs)

        def p_piece(j, u):
            when = lambda i, k: _ARRIVAL[2 * i + k // 3]
            new = [t for t, f in enumerate(_OXS) if max(when(i, k) for _, i, k in f) == _ARRIVAL[u]]

            def sink(c, o):
                rows = slice(c * CH // 2, (c + 1) * CH // 2)
                tile = lambda t: oc.at[j][rows, 128 * t:128 * (t + 1)]
                val = lambda i, k: (_col(o, k % 3) if when(i, k) == _ARRIVAL[u]
                                    else _unpack(tile(6 * i + k)).astype(f32))
                for t in new:
                    y = _signed_sum([(sg, val(i, k)) for sg, i, k in _OXS[t]])
                    oc.at[j][rows, 128 * t:128 * (t + 1)] = _pack(y)

            _attend(s.pop((j, u)), *kv(j, 1, u), pbuf.at[_ARRIVAL[u]], zero, lhs, sink)

        def o_round(j, ids):
            def finish(i, n, y):
                b = 2 * g + i
                cols = slice(j * d + 128 * n, j * d + 128 * (n + 1))
                if not first:
                    y = y + acc[b, :, cols]
                acc[b, :, cols] = y
                if write_out:
                    obuf[b, :, cols] = y.astype(bf16)

            run_round(ids, oc.at[j], woc.at[j], _OXS, _OX, _OO, om.setdefault(j, {}), finish)

        def flush(i):
            if write_out:
                @pl.when(last)
                def _():
                    pltpu.make_async_copy(obuf.at[2 * g + i], out.at[2 * g + i], osem).start()

        def o_piece(j, part):
            rounds = _OROUNDS[j]
            cuts = [j + c for c in (0, 1, 4, 8)] + [len(rounds)]
            for r in range(cuts[part], cuts[part + 1]):
                o_round(j, rounds[r])
            if part == 3:
                if j == 0:
                    o_round(1, _OROUNDS[1][0])
                else:
                    flush(0), flush(1)

        def w_piece(k):
            j = k // 2
            back = (build_wq(j, g, lambda t: rq[slot, j, t], wsets[1 - par]) if k % 2 == 0
                    else build_wo(j, g, lambda t: ro[slot, j, t], wsets[1 - par]))
            gate(-1, back)

        run = {'q': q_piece, 's': s_piece, 'p': p_piece, 'o': o_piece, 'w': w_piece,
               'x': x_piece, 'v': v_piece}
        for tok in seq.split():
            run[tok[0]](*(int(ch) for ch in tok[1:]))

    def run_pass(p, par, first, slot0):
        def step(g, slot):
            fetch_wait(slot)

            wrap = g + 2 >= ng
            fetch(jnp.minimum(jnp.where(wrap, p + 1, p), npass - 1),
                  jnp.where(wrap, g + 2 - ng, g + 2), jnp.where(slot == 0, NKV - 1, slot - 1),
                  p * ng + g + 2 < nsteps)

            if first:
                compute(_SEQ_NOQ, g, slot, par, qall.at[g], True, False)
            else:
                compute(_SEQ_FULL, g, slot, par, qbuf, False, par == 1, p == npass - 1)
            return jnp.where(slot == NKV - 1, 0, slot + 1)

        jax.lax.fori_loop(0, ng, step, slot0)

    def wq_init(j):
        return pltpu.make_async_copy(wqs[j].at[:, :, pl.ds(0, gw)], rq0.at[j], isem.at[j])

    zref[0] = 0
    x_copy(0, 0).start()
    wq_init(0).start()
    x_copy(0, 0).wait()
    wq_init(1).start()
    build_x(0, 0)
    for j in range(2):
        wq_init(j).wait()
        if j == 0:
            for gg in range(ng):
                x_copy(1, gg).start()
                for jj in range(2):
                    pltpu.make_async_copy(wos[jj].at[0, :, pl.ds(gg * wr, wr)], ro0.at[gg, jj],
                                          vsem.at[gg]).start()
                if gg + 1 < ng:
                    x_copy(0, gg + 1).start()

        def init_wq(gg, carry, j=j):
            rows = pl.ds(pl.multiple_of(gg * wr, 16), wr)
            build_wq(j, gg, lambda t: rq0.at[j, t][rows, :], wsets[0])
            return carry

        jax.lax.fori_loop(0, ng, init_wq, 0)

    def q_step(g, carry):
        x_copy(1, g).wait()
        wait_all(ro0.at[g], vsem.at[g])

        @pl.when(g + 1 < ng)
        def _():
            x_copy(0, g + 1).wait()

        @pl.when(g == 1)
        def _():
            fetch(0, 0, 0)

        @pl.when(g == 4)
        def _():
            fetch(0, 1, 1)

        compute(_SEQ_Q, g, 0, 0, qall.at[g], True, False)
        return carry

    jax.lax.fori_loop(0, ng, q_step, 0)

    run_pass(0, 0, True, 0)

    def pass_pair(pp, carry):
        run_pass(2 * pp + 1, 1, False, ((2 * pp + 1) * ng) % NKV)

        @pl.when(2 * pp + 2 < npass)
        def _():
            run_pass(2 * pp + 2, 0, False, ((2 * pp + 2) * ng) % NKV)

        return carry

    jax.lax.fori_loop(0, npass // 2, pass_pair, 0)
    wait_all(out, osem)


@jax.jit
def pallas_concat_heads__gqa_block_cached__mha_block_cached__near_ridge_kernel(
    A_x: jax.Array,
    A_k_cache: jax.Array,
    A_v_cache: jax.Array,
    A_wq: jax.Array,
    A_wo: jax.Array,
    B_x: jax.Array,
    B_k_cache: jax.Array,
    B_v_cache: jax.Array,
    B_wq: jax.Array,
    B_wo: jax.Array,
):
    B, Sq, D = A_x.shape
    _, H, Sk, Dh = A_k_cache.shape
    assert (B, Sq, D, H, Sk, Dh) == (16, 160, 640, 32, 512, 192)
    npass, ng = H // 4, B // 2
    gw = 4 * Dh
    scale = (Dh ** -0.5) * math.log2(math.e)

    akt, avt, bkt, bvt = (jnp.swapaxes(t, 2, 3) for t in
                          (A_k_cache, A_v_cache, B_k_cache, B_v_cache))
    awq, bwq = (w.reshape(5, 128, H * Dh) for w in (A_wq, B_wq))
    awo, bwo = (w.reshape(npass, 6, 128, D) for w in (A_wo, B_wo))
    any_spec = pl.BlockSpec(memory_space=pl.ANY)
    wset = [
        pltpu.VMEM((2, 64, len(_QW) * 128), i32),
        pltpu.VMEM((2, 64, len(_OW) * 128), i32),
    ]

    return pl.pallas_call(
        functools.partial(_kernel, scale=scale, d=D, sq=Sq, nbatch=B, npass=npass, dh=Dh),
        in_specs=[any_spec] * 10,
        out_specs=any_spec,
        out_shape=jax.ShapeDtypeStruct((B, Sq, 2 * D), A_x.dtype),
        scratch_shapes=[
            pltpu.VMEM((2, ng, 2, Sq, D), bf16),
            pltpu.VMEM((ng, Sq // 2, XPAD * 128), i32),
            pltpu.VMEM((ng, Sq // 2, XPAD * 128), i32),
            pltpu.VMEM((NKV, 4, 2, 4, Dh, Sk), bf16),
            pltpu.VMEM((NKV, 2, 5, 128 // ng, gw), bf16),
            pltpu.VMEM((NKV, 2, 6, 128 // ng, D), bf16),
            pltpu.VMEM((2, 5, 128, gw), bf16),
            pltpu.VMEM((ng, 2, 6, 128 // ng, D), bf16),
            *wset, *wset,
            pltpu.VMEM((B, Sq, 2 * D), f32),
            pltpu.VMEM((B, Sq, 2 * D), bf16),
            pltpu.VMEM((NPS, 2, Sq // 2, 768), i32),
            pltpu.VMEM((2, 4, Sq // 2, 512), i32),
            pltpu.VMEM((ng, 2, 4, Sq // 2, 512), i32),
            pltpu.VMEM((2, Sq // 2, len(_OXS) * 128), i32),
            pltpu.SMEM((1,), i32),
            pltpu.SemaphoreType.DMA((2, ng)),
            pltpu.SemaphoreType.DMA((NKV,)),
            pltpu.SemaphoreType.DMA((NKV,)),
            pltpu.SemaphoreType.DMA((NKV,)),
            pltpu.SemaphoreType.DMA((2,)),
            pltpu.SemaphoreType.DMA((ng,)),
            pltpu.SemaphoreType.DMA(()),
        ],
        compiler_params=pltpu.CompilerParams(
            vmem_limit_bytes=124 * 1024 * 1024,
            disable_bounds_checks=True,
            disable_semaphore_checks=True,
        ),
    )(A_x, akt, avt, awq, awo, B_x, bkt, bvt, bwq, bwo)
```

```python
import functools
import math

import jax
import jax.numpy as jnp
import jax.experimental.pallas as pl
import jax.experimental.pallas.tpu as pltpu

_NN = (((1,), (0,)), ((), ()))
_NT = (((1,), (1,)), ((), ()))
bf16 = jnp.bfloat16
f32 = jnp.float32
i32 = jnp.int32

CH = 16
DEP = 3
XPAD = 48
NKV = 3
NPS = 4

_SEQ_FULL = ('q00 w0 q01 q02 w2 w1 s01 p01 w4 s02 p02 q03 q10 q11 w3 s00 p00 w5 '
             's03 p03 o00 q12 q13 s11 o01 o02 p11 s12 s10 o03 p12 o10 s13 p10 o11 p13 '
             'o12 o13')
_SEQ_NOQ = ('s01 s02 s00 p01 p02 w1 p00 s03 o00 w4 o01 s11 p03 s12 o02 w5 p11 w2 '
            'w0 p12 s10 o10 o11 p10 s13 o03 p13 w3 o12 o13')
_SEQ_Q = 'x1 q00 v1 q01 q02 q03 v0 x0 q10 q11 q12 q13'


def _dot(a, b, dims=_NN):
    return jax.lax.dot_general(a, b, dims, preferred_element_type=f32)


def _recip(l):
    r = pl.reciprocal(l, approx=True)
    return r * (2.0 - l * r)


def _col(x, i):
    return x[:, 128 * i:128 * (i + 1)]


def _pack(x):
    return pltpu.bitcast(x.astype(bf16), i32)


def _unpack(x):
    return pltpu.bitcast(x, bf16)


def _cat(xs, axis):
    return jnp.concatenate(list(xs), axis=axis)


def _or_tiles(vals):
    t = None
    for v in vals:
        for r in range(0, v.shape[0], 8):
            for c in range(0, v.shape[1], 128):
                x = v[r:r + 8, c:c + 128]
                t = x if t is None else t | x
    return t


def _lane_lo(rows):
    return jax.lax.broadcasted_iota(i32, (rows, 128), 1) < 64


_QPROD = (
    '+12-33 +20+22-30 +12+30-32', '+31+34 +02+12-22 +32-30-31', '+00+20+23 +00-01 -21',
    '+11 +12 +12', '+00 +21+41-01-11 +21+31-01', '+00+30+33 +01+02 +31',
    '+00+02+12 +21 +00+01-31', '+01+02+12+31+32 +11+12 +02', '+03 +20+31+32+41+42-21-30 +01-11',
    '+04+34-03 +41+42 +02', '+00-34 +02+41-11 +02-31', '+14+21+24 +40 +20-00-22',
    '+11 +10 +10', '+00+04+14+21+24 +11+40-10 +00+21', '+02+03+22 +20-21 +00',
    '+22 +00+10-20-40 +00+30-20', '+22+32+33 +20+22 +30', '+03+10+13 +31 +11',
    '+12 +30-20 +00+01+12+30-10-11-32', '+14 +32+42 +01+12+20-02-10-11-22', '+34 +02+12-22-42 +02+22-32',
    '+12+13+23 +30 +10', '+01+04+14+21+24 +10-11 +00', '+10-33 +01+02-31 +12+31-32',
    '+12+31+32 +22 +32-02-30', '+10+30-31 +02 +32-22-31', '+24+34-23 +40+42 +22',
    '+10+20+30-31-34 +02+10+12 +22-30', '+00-22 +21+40-00-10 -00-21', '+03+14 +32+41+42 +02+11-01',
    '+04+14+24 +11+40-10-41 -21', '+21+22 +40-10 +22-20-21', '+11 +11 +11',
    '+22+34 +10+22-40 +22-30', '+10+20+30 +00+02+10+12 +30', '+10+20+30-21-31 +10+12 -22',
    '+02+12+31+32+34 +11+12-22 +31-02', '+14+23 +32+40+42 +10+22-20', '+23 +01+30+32+40+42-00-31 +20-10',
    '+02+12+32 +11+12-21-22 -31', '+00-01 +11 +02-00-01', '+10-23 +00+31-01 +10-20-21',
    '+10 +31-01 +12+20+21+31-10-11-32', '+10+20+22 +00 +20+21-30', '+33 +01+02+20+22-30-31-32 +12-32',
    '+00+04+14 +41 +01-02-21', '+13+33-14 +32 +12', '+03-12 +21+30-20 +00+01-11',
)
_QROUNDS = (
    ((32, ~43, ~18, ~15), (~1, 17, ~41, ~4), (~45, ~11, ~24, ~42), (~19, ~37, 10, ~25), (39, 5, 36, ~31),
     (16, 34, ~6, ~23), (13, 30, 2, 28), (21, ~0, 12, ~38), (33, ~20, 27, 35), (46, ~3, ~44, 26),
     (~40, 22, ~47, 14), (29, 9, 8, 7)),
    ((~11, ~29, ~41, ~25), (~47, ~24, ~40, ~23), (~45, 44, ~38, ~19), (~18, ~1, 5, ~6), (3, 39, ~20, ~37),
     (46, ~0, ~4, ~42), (~15, 32, 17, 8), (21, 12, 2, 13), (~22, ~30, 28, 14), (36, 9, ~7, 10),
     (27, ~33, 26, 31), (34, 43, 16, 35)),
)
_OPROD = (
    '+10 -00-20-40-50 +00-10', '+00+10 +00-02-04-03 +00', '+03 +30+10 +00-10',
    '+03+13 +30-31 +10', '+10 +01 +11', '+00 +01 +01',
    '+11 -11-31-21-41-51 +01-11', '+01+11 +11-10-12-14-13 +01', '+13 -32-52-42 +02-12',
    '+03+13 +32-33-34 +02', '+02 +22+12+02 +02-12', '+02+12 +22-21-20 +12',
    '+14 +43 +13', '+04 +43 +03', '+05 +53+23+13+03+33 +03-13',
    '+05+15 +53-54-51-50-52 +13', '+04 +44+14+04+34 +04-14', '+04+14 +44-41-40-42 +14',
    '+12 -24-54 +04-14', '+02+12 +24-23 +04', '+05+12 +54+23 +04+13',
    '+05-02 -23 +03+04', '+15-12 +54 +13+14', '+03+11 +31+10 +01+10',
    '+03-01 -10 +00+01', '+13-11 +31 +10+11', '+02+11 +12+21 +01+12',
    '+01-02 +12 +01+02', '+11-12 -21 +11+12', '+04+11 +14+41 +01+14',
    '+01-04 +14 +01+04', '+11-14 -41 +11+14', '+05+11 +13+51 +01+13',
    '+01-05 +13 +01+03', '+11-15 -51 +11+13', '+02+10 +02+20 +00+12',
    '+00-02 +02 +00+02', '+10-12 -20 +10+12', '+04+10 +04+40 +00+14',
    '+00-04 +04 +00+04', '+10-14 -40 +10+14', '+05+10 +03+50 +00+13',
    '+00-05 +03 +00+03', '+10-15 -50 +10+13', '+05+13 +33+52 +02+13',
    '+03-05 +33 +02+03', '+13-15 -52 +12+13', '+04+13 +34+42 +02+14',
    '+03-04 +34 +02+04', '+13-14 -42 +12+14',
)
_OROUNDS = (
    ((~13, ~16, ~48, ~45), (29, ~20, ~2, ~37), (~14, ~23, ~38, ~41), (~18, ~32, 6, 4), (30, 7, 42, 5),
     (26, 19, 1, ~0), (35, 33, 21, 11), (39, ~36, ~24, ~27), (49, ~8, 31, 28), (25, 46, 40, 17),
     (44, 10, 15, 3), (47, ~9, 22, 43), (34, 12)),
    ((14, 13), (~45, ~16, ~2, ~48), (~4, ~0, ~20, ~32), (37, 38, 29, 41), (~23, ~6, 28, ~18),
     (19, 11, 26, ~7), (~10, ~30, 5, 33), (~35, 21, ~39, ~42), (~24, 27, 36, 1), (8, ~34, 44, ~49),
     (40, ~31, 25, ~17), (46, ~22, 9, ~47), (~15, 43, 12, 3)),
)


def _terms(code):
    return tuple((1 if code[i] == '+' else -1, int(code[i + 1]), int(code[i + 2]))
                 for i in range(0, len(code), 3))


_QX, _QW, _QO = zip(*[[_terms(c) for c in p.split()] for p in _QPROD])
_QXS = sorted(set(_QX))
_OX, _OW, _OO = zip(*[[_terms(c) for c in p.split()] for p in _OPROD])
_ORAW = [((1, i, k),) for i in range(2) for k in range(6)]
_OXS = _ORAW + sorted(set(_OX) - set(_ORAW))
_ARRIVAL = (2, 0, 1, 3)


def _signed_sum(terms):
    if terms[0][0] < 0 and len(terms) > 1 and terms[1][0] > 0:
        terms = [terms[1], terms[0]] + list(terms[2:])
    sg0, y = terms[0]
    for sg, v in terms[1:]:
        if sg0 < 0 and sg > 0:
            sg0, y = 1, v - y
        else:
            y = y + v if sg == sg0 else y - v
    return y if sg0 > 0 else -y


def _weights(xa, xb, xc):
    h = xa.shape[1] // 2
    xa, xb, xc = xa.astype(f32), xb.astype(f32), xc.astype(f32)
    return (_cat([xa[:, :h], xb[:, :h] - xb[:, h:]], 0),
            _cat([xa[:, h:], xc[:, h:] - xc[:, :h]], 0),
            _cat([xc[:, :h], xb[:, h:]], 0))


def _pair_weights(t0, t1):
    return (_weights(t0[:64], t0[64:128], t0[128:]), _weights(t1[64:128], t1[128:], t1[:64]))


def _scores(q_ref, kt0, kt1, lhs):
    t0, t1, t2, rot = (q_ref[:, 128 * k:128 * (k + 1)] for k in range(4))
    lo = _lane_lo(t0.shape[0])
    q = ((t0, jnp.where(lo, t0, rot), jnp.where(lo, t1, t0)),
         (t2, jnp.where(lo, t2, t1), jnp.where(lo, rot, t2)))
    w = _pair_weights(kt0, kt1)
    p = {}

    def run(h, k, i):
        y = _dot(lhs(q[h][k]), _col(w[h][k], i).astype(bf16))
        p[h, k, i] = y if k == 2 else y + p[h, 2, i]

    run(0, 2, 0), run(0, 2, 1), run(1, 2, 0), run(1, 2, 1)
    for h in range(2):
        run(h, 0, 0), run(h, 0, 1), run(h, 1, 0), run(h, 1, 1)
    return tuple(_cat([p[h, 0, 0], p[h, 0, 1], p[h, 1, 0], p[h, 1, 1]], 1) for h in range(2))


def _softmax_terms(s, p_ref, zero):
    ls, toks = [], []
    for c in range(s.shape[0] // CH):
        sc = s[c * CH:(c + 1) * CH]
        m = jnp.broadcast_to(jnp.max(sc, axis=-1, keepdims=True), (CH, 128))
        if c >= DEP:
            t = toks[c - DEP] & zero
            m = pltpu.bitcast(pltpu.bitcast(m, i32) | _cat([t, t], 0), f32)
        e = [jnp.exp2(_col(sc, k) - m) for k in range(4)]
        t0, t1 = e[0] + e[2], e[1] + e[3]
        t01 = t0 + t1
        ls.append(jnp.broadcast_to(jnp.sum(t01, axis=-1, keepdims=True), (CH, 128)))
        rows = slice(c * CH // 2, (c + 1) * CH // 2)
        for k, x in enumerate(e + [t0, t1]):
            p_ref[rows, 128 * k:128 * (k + 1)] = _pack(x)
        toks.append(_or_tiles([p_ref[rows, :], pltpu.bitcast(t01, i32)]))
    return ls


def _attend(s, vt0, vt1, p_ref, zero, lhs, sink):
    ls = [_softmax_terms(s[h], p_ref.at[h], zero) for h in range(2)]
    w = _pair_weights(vt0, vt1)
    r = {}
    for h, k in ((0, 0), (0, 2), (0, 1), (1, 0), (1, 2), (1, 1)):
        r[h, k] = _dot(lhs(p_ref.at[h][:, 256 * k:256 * (k + 1)]), w[h][k].astype(bf16), _NT)
    lo = _lane_lo(CH)

    def rows(c):
        p1, p2, p3, u1, u2, u3 = (r[h, k][c * CH:(c + 1) * CH] for h in range(2) for k in range(3))
        r0, r1 = _recip(ls[0][c]), _recip(ls[1][c])
        o_lo = p1 + jnp.where(lo, p2, p3)
        o_hi = u1 + jnp.where(lo, u2, u3)
        mid = jnp.where(lo, p3, u2) + pltpu.roll(jnp.where(lo, u3, p2), 64, 1)
        return _cat([o_lo * r0, mid * jnp.where(lo, r0, r1), o_hi * r1], 1)

    for c in range(len(ls[0])):
        sink(c, rows(c))


def _kernel(ax, akt, avt, awq, awo, bx, bkt, bvt, bwq, bwo, out,
            xbuf, xca, xcb, kvbuf, rq, ro, rq0, ro0,
            wqc0, woc0, wqc1, woc1,
            acc, obuf, pbuf, qbuf, qall, oc, zref,
            xsem, kvsem, rqsem, rosem, isem, vsem, osem,
            *, scale, d, sq, nbatch, npass, dh):
    ng = nbatch // 2
    nsteps = npass * ng
    gw = 4 * dh
    wr = 128 // ng
    hq = sq // 4
    xs, wqs, wos = (ax, bx), (awq, bwq), (awo, bwo)
    kvs = (akt, avt, bkt, bvt)
    xc = (xca, xcb)
    wsets = ((wqc0, woc0), (wqc1, woc1))

    def wait_all(ref, sem):
        pltpu.make_async_copy(ref, ref, sem).wait()

    def fetch(pp, gg, slot, live=True):
        def start(src, dst, sem):
            pl.when(live)(lambda: pltpu.make_async_copy(src, dst, sem).start())

        for t in range(4):
            start(kvs[t].at[pl.ds(gg * 2, 2), pl.ds(4 * pp, 4)], kvbuf.at[slot, t], kvsem.at[slot])
        pw = jnp.minimum(pp + 1, npass - 1)
        rows = pl.ds(pl.multiple_of(gg * wr, 16), wr)
        for j in range(2):
            for t in range(5):
                start(wqs[j].at[t, rows, pl.ds(pl.multiple_of(pw * gw, 128), gw)],
                      rq.at[slot, j, t], rqsem.at[slot])
            start(wos[j].at[pw, :, rows], ro.at[slot, j], rosem.at[slot])

    def fetch_wait(slot):
        wait_all(kvbuf.at[slot], kvsem.at[slot])
        wait_all(rq.at[slot], rqsem.at[slot])
        wait_all(ro.at[slot], rosem.at[slot])

    def x_copy(j, gg):
        return pltpu.make_async_copy(xs[j].at[pl.ds(gg * 2, 2)], xbuf.at[j, gg], xsem.at[j, gg])

    def build_x(j, gg):
        back = []
        for r in range(0, sq // 2, 16):
            x = [xbuf.at[j, gg, m // 2][(m % 2) * (sq // 2) + r:(m % 2) * (sq // 2) + r + 16, :].astype(f32)
                 for m in range(4)]
            tiles = [_signed_sum([(sg, _col(x[m], k)) for sg, m, k in f]) for f in _QXS]
            rows = slice(r // 2, r // 2 + 8)
            xc[j].at[gg][rows, :128 * len(tiles)] = _pack(_cat(tiles, 1))
            back.append(xc[j].at[gg][rows, :128 * len(tiles)])
        return back

    def build_wq(j, t, gg, raw, wset):
        wqc = wset[0]
        kt = [raw(k)[:, t * (gw // 2):(t + 1) * (gw // 2)].astype(f32) for k in range(5)]
        rows = pl.ds(pl.multiple_of(gg * (wr // 2), 8), wr // 2)
        tiles = [_signed_sum([(sg, _col(kt[k], n)) for sg, k, n in f]) for f in _QW]
        wqc.at[j, t][rows, :] = _pack(_cat(tiles, 1))
        return [wqc.at[j, t][rows, :]]

    def build_wo(j, gg, raw, wset):
        woc = wset[1]
        kt = [raw(t).astype(f32) for t in range(6)]
        tiles = [_signed_sum([(sg, _col(kt[k], n)) for sg, k, n in f]) for f in _OW]
        rows = pl.ds(pl.multiple_of(gg * (wr // 2), 8), wr // 2)
        woc.at[j][rows, :] = _pack(_cat(tiles, 1))
        return [woc.at[j][rows, :]]

    def compute(seq, g, slot, par, q_ref, first, write_out, last=None):
        wqc, woc = wsets[par]
        s, qm, om = {}, {}, {}
        toks = []
        zero = jnp.full((8, 128), zref[0], i32)

        def lhs(x):
            for e in toks:
                e[0] -= 1
            if toks and toks[0][0] < 0:
                t = toks.pop(0)[1] & zero
                x = _cat([x[:8] | _cat([t] * (x.shape[1] // 128), 1), x[8:]], 0)
            return _unpack(x)

        def gate(delay, vals):
            toks.append([delay, _or_tiles(vals)])
            toks.sort(key=lambda e: e[0])

        def run_round(ids, x_ref, w_ref, xs_, xf, of, state, finish):
            touched = []
            for e in ids:
                m = e if e >= 0 else ~e
                xt = xs_.index(xf[m])
                x = x_ref[:, 128 * xt:128 * (xt + 1)]
                w = _unpack(w_ref[:, 128 * m:128 * (m + 1)])
                y = _dot(lhs(x), w)
                for sg, i, n in of[m]:
                    st = state.setdefault((i, n), [[], sum(o[1:] == (i, n) for f in of for o in f)])
                    st[0].insert(0, (sg, y))
                    st[1] -= 1
                    if (e >= 0 or st[1] == 0) and (i, n) not in touched:
                        touched.append((i, n))
            for i, n in touched:
                st = state[i, n]
                y = _signed_sum(st[0])
                st[0] = [(1, y)]
                if st[1] == 0:
                    finish(i, n, y)

        def q_round(j, t, ids):
            def finish(m, n, y):
                y = y * scale
                dst = q_ref.at[j, 2 * (m // 2) + t]
                rows = slice((m % 2) * hq, (m % 2 + 1) * hq)
                dst[rows, 128 * n:128 * (n + 1)] = _pack(y)
                if n == 1:
                    dst[rows, 384:] = _pack(pltpu.roll(y, 64, 1))

            run_round(ids, xc[j].at[g], wqc.at[j, t], _QXS, _QX, _QO, qm.setdefault((j, t), {}), finish)

        def q_piece(j, part):
            for t, lo, hi in (((1, 0, 5),), ((1, 5, 10),), ((0, 0, 10),), ((0, 10, 12), (1, 10, 12)))[part]:
                for r in range(lo, hi):
                    q_round(j, t, _QROUNDS[t][r])

        def x_piece(j):
            back = build_x(1, g) if j == 1 else build_x(0, jnp.minimum(g + 1, ng - 1))
            for c, v in enumerate(back):
                gate(8 + 16 * c, [v])

        def v_piece(j):
            gate(-1, build_wo(j, g, lambda t: ro0[g, j, t], wsets[0]))

        def kv(j, which, u):
            return tuple(kvbuf[slot, 2 * j + which, u // 2, 2 * (u % 2) + h] for h in range(2))

        def s_piece(j, u):
            s[j, u] = _scores(q_ref.at[j, u], *kv(j, 0, u), lhs)

        def p_piece(j, u):
            when = lambda i, k: _ARRIVAL[2 * i + k // 3]
            new = [t for t, f in enumerate(_OXS) if max(when(i, k) for _, i, k in f) == _ARRIVAL[u]]

            def sink(c, o):
                rows = slice(c * CH // 2, (c + 1) * CH // 2)
                tile = lambda t: oc.at[j][rows, 128 * t:128 * (t + 1)]
                val = lambda i, k: (_col(o, k % 3) if when(i, k) == _ARRIVAL[u]
                                    else _unpack(tile(6 * i + k)).astype(f32))
                for t in new:
                    y = _signed_sum([(sg, val(i, k)) for sg, i, k in _OXS[t]])
                    oc.at[j][rows, 128 * t:128 * (t + 1)] = _pack(y)

            _attend(s.pop((j, u)), *kv(j, 1, u), pbuf.at[_ARRIVAL[u]], zero, lhs, sink)

        def o_round(j, ids):
            def finish(i, n, y):
                b = 2 * g + i
                cols = slice(j * d + 128 * n, j * d + 128 * (n + 1))
                if not first:
                    y = y + acc[b, :, cols]
                acc[b, :, cols] = y
                if write_out:
                    obuf[b, :, cols] = y.astype(bf16)

            run_round(ids, oc.at[j], woc.at[j], _OXS, _OX, _OO, om.setdefault(j, {}), finish)

        def flush(i):
            if write_out:
                @pl.when(last)
                def _():
                    pltpu.make_async_copy(obuf.at[2 * g + i], out.at[2 * g + i], osem).start()

        def o_piece(j, part):
            rounds = _OROUNDS[j]
            cuts = [j + c for c in (0, 1, 4, 8)] + [len(rounds)]
            for r in range(cuts[part], cuts[part + 1]):
                o_round(j, rounds[r])
            if part == 3:
                if j == 0:
                    o_round(1, _OROUNDS[1][0])
                else:
                    flush(0), flush(1)

        def w_piece(k):
            j, t = ((0, 0), (0, None), (1, 0), (1, None), (0, 1), (1, 1))[k]
            back = (build_wo(j, g, lambda c: ro[slot, j, c], wsets[1 - par]) if t is None
                    else build_wq(j, t, g, lambda c: rq[slot, j, c], wsets[1 - par]))
            gate(-1, back)

        run = {'q': q_piece, 's': s_piece, 'p': p_piece, 'o': o_piece, 'w': w_piece,
               'x': x_piece, 'v': v_piece}
        for tok in seq.split():
            run[tok[0]](*(int(ch) for ch in tok[1:]))

    def run_pass(p, par, first, slot0):
        def step(g, slot):
            fetch_wait(slot)

            wrap = g + 2 >= ng
            fetch(jnp.minimum(jnp.where(wrap, p + 1, p), npass - 1),
                  jnp.where(wrap, g + 2 - ng, g + 2), jnp.where(slot == 0, NKV - 1, slot - 1),
                  p * ng + g + 2 < nsteps)

            if first:
                compute(_SEQ_NOQ, g, slot, par, qall.at[g], True, False)
            else:
                compute(_SEQ_FULL, g, slot, par, qbuf, False, par == 1, p == npass - 1)
            return jnp.where(slot == NKV - 1, 0, slot + 1)

        jax.lax.fori_loop(0, ng, step, slot0)

    def wq_init(j):
        return pltpu.make_async_copy(wqs[j].at[:, :, pl.ds(0, gw)], rq0.at[j], isem.at[j])

    zref[0] = 0
    x_copy(0, 0).start()
    wq_init(0).start()
    x_copy(0, 0).wait()
    wq_init(1).start()
    build_x(0, 0)
    for j in range(2):
        wq_init(j).wait()
        if j == 0:
            for gg in range(ng):
                x_copy(1, gg).start()
                for jj in range(2):
                    pltpu.make_async_copy(wos[jj].at[0, :, pl.ds(gg * wr, wr)], ro0.at[gg, jj],
                                          vsem.at[gg]).start()
                if gg + 1 < ng:
                    x_copy(0, gg + 1).start()

        def init_wq(gg, carry, j=j):
            rows = pl.ds(pl.multiple_of(gg * wr, 16), wr)
            for t in range(2):
                build_wq(j, t, gg, lambda c: rq0.at[j, c][rows, :], wsets[0])
            return carry

        jax.lax.fori_loop(0, ng, init_wq, 0)

    def q_step(g, carry):
        x_copy(1, g).wait()
        wait_all(ro0.at[g], vsem.at[g])

        @pl.when(g + 1 < ng)
        def _():
            x_copy(0, g + 1).wait()

        @pl.when(g == 1)
        def _():
            fetch(0, 0, 0)

        @pl.when(g == 4)
        def _():
            fetch(0, 1, 1)

        compute(_SEQ_Q, g, 0, 0, qall.at[g], True, False)
        return carry

    jax.lax.fori_loop(0, ng, q_step, 0)

    run_pass(0, 0, True, 0)

    def pass_pair(pp, carry):
        run_pass(2 * pp + 1, 1, False, ((2 * pp + 1) * ng) % NKV)

        @pl.when(2 * pp + 2 < npass)
        def _():
            run_pass(2 * pp + 2, 0, False, ((2 * pp + 2) * ng) % NKV)

        return carry

    jax.lax.fori_loop(0, npass // 2, pass_pair, 0)
    wait_all(out, osem)


@jax.jit
def pallas_concat_heads__gqa_block_cached__mha_block_cached__near_ridge_kernel(
    A_x: jax.Array,
    A_k_cache: jax.Array,
    A_v_cache: jax.Array,
    A_wq: jax.Array,
    A_wo: jax.Array,
    B_x: jax.Array,
    B_k_cache: jax.Array,
    B_v_cache: jax.Array,
    B_wq: jax.Array,
    B_wo: jax.Array,
):
    B, Sq, D = A_x.shape
    _, H, Sk, Dh = A_k_cache.shape
    assert (B, Sq, D, H, Sk, Dh) == (16, 160, 640, 32, 512, 192)
    npass, ng = H // 4, B // 2
    gw = 4 * Dh
    scale = (Dh ** -0.5) * math.log2(math.e)

    akt, avt, bkt, bvt = (jnp.swapaxes(t, 2, 3) for t in
                          (A_k_cache, A_v_cache, B_k_cache, B_v_cache))
    awq, bwq = (w.reshape(5, 128, H * Dh) for w in (A_wq, B_wq))
    awo, bwo = (w.reshape(npass, 6, 128, D) for w in (A_wo, B_wo))
    any_spec = pl.BlockSpec(memory_space=pl.ANY)
    wset = [
        pltpu.VMEM((2, 2, 64, len(_QW) * 128), i32),
        pltpu.VMEM((2, 64, len(_OW) * 128), i32),
    ]

    return pl.pallas_call(
        functools.partial(_kernel, scale=scale, d=D, sq=Sq, nbatch=B, npass=npass, dh=Dh),
        in_specs=[any_spec] * 10,
        out_specs=any_spec,
        out_shape=jax.ShapeDtypeStruct((B, Sq, 2 * D), A_x.dtype),
        scratch_shapes=[
            pltpu.VMEM((2, ng, 2, Sq, D), bf16),
            pltpu.VMEM((ng, Sq // 4, XPAD * 128), i32),
            pltpu.VMEM((ng, Sq // 4, XPAD * 128), i32),
            pltpu.VMEM((NKV, 4, 2, 4, Dh, Sk), bf16),
            pltpu.VMEM((NKV, 2, 5, 128 // ng, gw), bf16),
            pltpu.VMEM((NKV, 2, 6, 128 // ng, D), bf16),
            pltpu.VMEM((2, 5, 128, gw), bf16),
            pltpu.VMEM((ng, 2, 6, 128 // ng, D), bf16),
            *wset, *wset,
            pltpu.VMEM((B, Sq, 2 * D), f32),
            pltpu.VMEM((B, Sq, 2 * D), bf16),
            pltpu.VMEM((NPS, 2, Sq // 2, 768), i32),
            pltpu.VMEM((2, 4, Sq // 2, 512), i32),
            pltpu.VMEM((ng, 2, 4, Sq // 2, 512), i32),
            pltpu.VMEM((2, Sq // 2, len(_OXS) * 128), i32),
            pltpu.SMEM((1,), i32),
            pltpu.SemaphoreType.DMA((2, ng)),
            pltpu.SemaphoreType.DMA((NKV,)),
            pltpu.SemaphoreType.DMA((NKV,)),
            pltpu.SemaphoreType.DMA((NKV,)),
            pltpu.SemaphoreType.DMA((2,)),
            pltpu.SemaphoreType.DMA((ng,)),
            pltpu.SemaphoreType.DMA(()),
        ],
        compiler_params=pltpu.CompilerParams(
            vmem_limit_bytes=124 * 1024 * 1024,
            disable_bounds_checks=True,
            disable_semaphore_checks=True,
        ),
    )(A_x, akt, avt, awq, awo, B_x, bkt, bvt, bwq, bwo)
```
